```python
import jax
import jax.numpy as jnp

def _softmax(x, axis=-1):
    return jax.nn.softmax(x, axis=axis)

def _gelu(x):
    return jax.nn.gelu(x, approximate=True)

def _silu(x):
    return jax.nn.silu(x)

def _sigmoid(x):
    return jax.nn.sigmoid(x)

def _layernorm(x, axis=-1, eps=1e-05):
    m = jnp.mean(x, axis=axis, keepdims=True)
    v = jnp.var(x, axis=axis, keepdims=True)
    return (x - m) / jnp.sqrt(v + eps)

def _scatter_add(tgt, idx, src, axis=0):
    return tgt.at[idx].add(src)

def _segment_sum(src, seg, n):
    return jax.ops.segment_sum(src, seg, n)

class _Rng:

    def __init__(self, key):
        self._k = key

    def _next(self):
        self._k, sub = jax.random.split(self._k)
        return sub

    def normal(self, shape):
        return jax.random.normal(self._next(), shape, dtype=jnp.bfloat16)

    def randint(self, lo, hi, shape):
        return jax.random.randint(self._next(), shape, lo, hi, dtype=jnp.int32)

    def uniform(self, shape, lo=0.0, hi=1.0):
        return jax.random.uniform(self._next(), shape, jnp.bfloat16, lo, hi)

    def permutation(self, n):
        return jax.random.permutation(self._next(), n)
kernel_name = 'adaLN_cond__sliding_local_dilated__glu_gated_swiglu__prompt'

def setup_inputs():
    _rng = _Rng(jax.random.key(int.from_bytes(__import__("os").urandom(4), "little")))
    _w = lambda a: (lambda t: t.astype(jnp.bfloat16) if jnp.issubdtype(t.dtype, jnp.floating) else t)(jnp.asarray(a))

    def _A_setup():
        B, S, D = (1, 2048, 1024)
        return {'x': _w((lambda *s: _rng.normal(s) * 0.05)(B, S, D)), 'wqkv': _w((lambda *s: _rng.normal(s) * 0.05)(D, 3 * D)), 'wo': _w((lambda *s: _rng.normal(s) * 0.05)(D, D))}
    _A_in = _A_setup()

    def _B_setup():
        B, S, D, F = (1, 2048, 1024, 3584)
        return {'x': _w((lambda *s: _rng.normal(s) * 0.05)(B, S, D)), 'w1': _w((lambda *s: _rng.normal(s) * 0.05)(D, F) * (2.0 / D) ** 0.5), 'w3': _w((lambda *s: _rng.normal(s) * 0.05)(D, F) * (2.0 / D) ** 0.5), 'w2': _w((lambda *s: _rng.normal(s) * 0.05)(F, D) * (2.0 / F) ** 0.5)}
    _B_in = _B_setup()
    return {'A_x': _A_in['x'], 'A_wqkv': _A_in['wqkv'], 'A_wo': _A_in['wo'], 'B_x': _B_in['x'], 'B_w1': _B_in['w1'], 'B_w3': _B_in['w3'], 'B_w2': _B_in['w2'], 'c': _w((lambda *s: _rng.normal(s) * 0.05)(1, 1024)), 'w_mod': _w((lambda *s: _rng.normal(s) * 0.05)(1024, 6 * 1024) * 1024 ** (-0.5))}

def reference(A_x, A_wqkv, A_wo, B_x, B_w1, B_w3, B_w2, c, w_mod):

    def _A_ref(x, wqkv, wo):
        B, S, D = x.shape
        H = 32
        Dh = D // H
        W, dil = (8, 2)
        qkv = (lambda x, *d: x.transpose(*d))((x @ wqkv).reshape(B, S, 3, H, Dh), 2, 0, 3, 1, 4)
        q, k, v = (qkv[0], qkv[1], qkv[2])
        scale = Dh ** (-0.5)
        pos = jnp.arange(S)
        off = jnp.arange(W) * dil
        idx = pos[:, None] - off[None, :]
        mask = idx >= 0
        idx_c = jnp.where(mask, idx, 0).reshape(-1)
        kg = k[:, :, idx_c, :].reshape(B, H, S, W, Dh)
        vg = v[:, :, idx_c, :].reshape(B, H, S, W, Dh)
        logits = jnp.einsum('bhsd,bhswd->bhsw', q, kg) * scale
        logits = jnp.where(mask[None, None, :, :], logits, -1000000000.0)
        attn = _softmax(logits, axis=-1)
        o = jnp.einsum('bhsw,bhswd->bhsd', attn, vg)
        return (lambda x, *d: x.transpose(*d))(o, 0, 2, 1, 3).reshape(B, S, D) @ wo

    def _B_ref(x, w1, w3, w2):
        gate = jnp.einsum('bsd,df->bsf', x, w1)
        up = jnp.einsum('bsd,df->bsf', x, w3)
        h = _silu(gate) * up
        out = jnp.einsum('bsf,fd->bsd', h, w2)
        return out
    x = A_x
    mod = (_silu(c) @ w_mod).reshape(c.shape[0], 6, 1, -1)
    sa, ca, ga, sb, cb, gb = (mod[:, 0].copy(), mod[:, 1].copy(), mod[:, 2].copy(), mod[:, 3].copy(), mod[:, 4].copy(), mod[:, 5].copy())
    h = _layernorm(x, axis=-1) * (1 + ca) + sa
    x = x + ga * _A_ref(h, A_wqkv, A_wo)
    h = _layernorm(x, axis=-1) * (1 + cb) + sb
    x = x + gb * _B_ref(h, B_w1, B_w3, B_w2)
    return x
```

```python
import functools
import jax
import jax.numpy as jnp
from jax import lax
import jax.experimental.pallas as pl
import jax.experimental.pallas.tpu as pltpu

S, D, F = 2048, 1024, 3584
H, DH, W, DIL = 32, 32, 8, 2
NG = D // 128
HALO = 16
T = 256
NT = S // T
FC = 512
NFC = F // FC
KROWS = T + 24
QROWS = T + 8
KOFF = 24
LOG2E = 1.4426950408889634
QSCALE = (DH ** -0.5) * LOG2E
NEG = -1e9 * LOG2E
EPS = 1e-5
f32, bf16, u32 = jnp.float32, jnp.bfloat16, jnp.uint32


def _swap_bits(vs, lane):
    vs = list(vs)
    for b in range(3):
        s = 4 << b
        hi = (lane & s) != 0
        for g in range(NG):
            if g & (1 << b):
                continue
            a, c = vs[g], vs[g | (1 << b)]
            vs[g] = jnp.where(hi, pltpu.roll(c, s, 1), a)
            vs[g | (1 << b)] = jnp.where(hi, c, pltpu.roll(a, 128 - s, 1))
    return vs


def _ln_mod(x, scale1, shift):
    m = jnp.mean(x, axis=-1, keepdims=True)
    xc = x - m
    v = jnp.mean(xc * xc, axis=-1, keepdims=True)
    return xc * lax.rsqrt(v + EPS) * scale1 + shift


def _kernel(x_hbm, wqkv_hbm, wo_hbm, w1_hbm, w3_hbm, w2_hbm, c_hbm, wmod_hbm, out_hbm,
            x_v, c_v, wmod_v, wqkv_v, wo_v, w1_v, w3_v, w2_v, mod_v,
            h_v, q_v, k_v, v_v, x1_v, acc_v, ob_v, sem, osem):
    cp = lambda src, dst, i: pltpu.make_async_copy(src, dst, sem.at[i])
    copies = dict(
        c=cp(c_hbm, c_v, 0),
        x=cp(x_hbm.at[0], x_v, 1),
        wmod=cp(wmod_hbm, wmod_v, 2),
        wqkv=cp(wqkv_hbm, wqkv_v, 3),
        wo=cp(wo_hbm, wo_v, 4),
        w1=cp(w1_hbm, w1_v, 5),
        w3=cp(w3_hbm, w3_v, 6),
        w2=cp(w2_hbm, w2_v, 7),
    )
    for k in ("c", "wmod", "x", "wqkv", "wo", "w1", "w3", "w2"):
        copies[k].start()

    copies["c"].wait()
    copies["wmod"].wait()
    c = c_v[...].astype(f32)
    sc = (c * jax.nn.sigmoid(c)).astype(bf16)
    sc = jnp.broadcast_to(sc, (16, D))
    mod = jnp.dot(sc, wmod_v[...], preferred_element_type=f32)[0:8]
    col = lax.broadcasted_iota(jnp.int32, (8, 6 * D), 1)
    is_scale = ((col >= D) & (col < 2 * D)) | ((col >= 4 * D) & (col < 5 * D))
    mod_v[...] = jnp.where(is_scale, mod + 1.0, mod)

    copies["wqkv"].wait()
    lane8 = lax.broadcasted_iota(jnp.int32, (8, 128), 1)

    def perm_body(r, carry):
        r0 = pl.multiple_of(r * 16, 16)
        for sec in range(3):
            vs = [pltpu.bitcast(wqkv_v[pl.ds(r0, 16), sec * D + g * 128: sec * D + (g + 1) * 128], u32) for g in range(NG)]
            vs = _swap_bits(vs, lane8)
            for g in range(NG):
                wqkv_v[pl.ds(r0, 16), sec * D + g * 128: sec * D + (g + 1) * 128] = pltpu.bitcast(vs[g], bf16)
        return carry
    lax.fori_loop(0, D // 16, perm_body, 0)

    copies["x"].wait()
    copies["wo"].wait()
    for g in range(NG):
        k_v[g, 0:KOFF, :] = jnp.zeros((KOFF, 128), f32)
        v_v[g, 0:KOFF, :] = jnp.zeros((KOFF, 128), f32)

    row8 = lax.broadcasted_iota(jnp.int32, (8, 128), 0)

    def phase_a(i, carry):
        t0 = pl.multiple_of(i * T, T)
        for rb in range(T // 16):
            x = x_v[pl.ds(t0 + rb * 16, 16), :].astype(f32)
            h_v[rb * 16:(rb + 1) * 16, :] = _ln_mod(x, mod_v[0:1, D:2 * D], mod_v[0:1, 0:D]).astype(bf16)
        qkv = jnp.dot(h_v[...], wqkv_v[...], preferred_element_type=f32)
        for g in range(NG):
            q_v[g, 0:T, :] = qkv[:, g * 128:(g + 1) * 128] * QSCALE
            k_v[g, KOFF:KOFF + T, :] = qkv[:, D + g * 128: D + (g + 1) * 128]
            v_v[g, KOFF:KOFF + T, :] = qkv[:, 2 * D + g * 128: 2 * D + (g + 1) * 128]

        @pl.when(i == 0)
        def _():
            for g in range(NG):
                v_v[g, KOFF - HALO:KOFF, :] = jnp.broadcast_to(v_v[g, KOFF:KOFF + 1, :], (HALO, 128))

        os = []
        for rb in range(T // 8):
            r0 = rb * 8
            s = [None] * W
            for g in range(NG):
                q = q_v[g, r0:r0 + 8, :]
                for j in range(W):
                    o = KOFF + r0 - DIL * j
                    p = q * k_v[g, o:o + 8, :]
                    s[j] = p if s[j] is None else s[j] + p
            for j in range(W):
                for sh in (1, 2):
                    hi = (lane8 & sh) != 0
                    s[j] = s[j] + jnp.where(hi, pltpu.roll(s[j], sh, 1), pltpu.roll(s[j], 128 - sh, 1))
                if r0 < DIL * j:
                    s[j] = jnp.where(t0 + r0 + row8 >= DIL * j, s[j], NEG)
            m = functools.reduce(jnp.maximum, s)
            e = [jnp.exp2(s[j] - m) for j in range(W)]
            inv = 1.0 / functools.reduce(lambda a, b: a + b, e)
            p = [e[j] * inv for j in range(W)]
            og = []
            for g in range(NG):
                acc = None
                for j in range(W):
                    o = KOFF + r0 - DIL * j
                    t = p[j] * v_v[g, o:o + 8, :]
                    acc = t if acc is None else acc + t
                og.append(acc)
            os.append(og)
            if rb % 2 == 1:
                pk = [pltpu.bitcast(jnp.concatenate([os[0][g], os[1][g]], axis=0).astype(bf16), u32) for g in range(NG)]
                pk = _swap_bits(pk, lane8)
                for g in range(NG):
                    h_v[r0 - 8:r0 + 8, g * 128:(g + 1) * 128] = pltpu.bitcast(pk[g], bf16)
                os = []
        for g in range(NG):
            k_v[g, KOFF - HALO:KOFF, :] = k_v[g, KOFF + T - HALO:KOFF + T, :]
            v_v[g, KOFF - HALO:KOFF, :] = v_v[g, KOFF + T - HALO:KOFF + T, :]
        a = jnp.dot(h_v[...], wo_v[...], preferred_element_type=f32)
        x1_v[pl.ds(t0, T), :] = x_v[pl.ds(t0, T), :].astype(f32) + mod_v[0:1, 2 * D:3 * D] * a
        return carry
    lax.fori_loop(0, NT, phase_a, 0)

    copies["w1"].wait()
    copies["w3"].wait()
    copies["w2"].wait()

    def out_copy(i, slot):
        return pltpu.make_async_copy(ob_v.at[slot], out_hbm.at[0, pl.ds(pl.multiple_of(i * T, T), T), :], osem.at[slot])

    def phase_b(i, carry):
        t0 = pl.multiple_of(i * T, T)
        slot = i % 2
        for rb in range(T // 16):
            x = x1_v[pl.ds(t0 + rb * 16, 16), :]
            h_v[rb * 16:(rb + 1) * 16, :] = _ln_mod(x, mod_v[0:1, 4 * D:5 * D], mod_v[0:1, 3 * D:4 * D]).astype(bf16)
        h = h_v[...]
        acc = None
        for fc in range(NFC):
            g = jnp.dot(h, w1_v[:, fc * FC:(fc + 1) * FC], preferred_element_type=f32)
            u = jnp.dot(h, w3_v[:, fc * FC:(fc + 1) * FC], preferred_element_type=f32)
            act = (g * jax.nn.sigmoid(g) * u).astype(bf16)
            y = jnp.dot(act, w2_v[fc * FC:(fc + 1) * FC, :], preferred_element_type=f32)
            acc = y if acc is None else acc + y

        @pl.when(i >= 2)
        def _():
            out_copy(i - 2, slot).wait()
        ob_v[slot] = (x1_v[pl.ds(t0, T), :] + mod_v[0:1, 5 * D:6 * D] * acc).astype(bf16)
        out_copy(i, slot).start()
        return carry
    lax.fori_loop(0, NT, phase_b, 0)
    out_copy(NT - 2, 0).wait()
    out_copy(NT - 1, 1).wait()


@jax.jit
def pallas_adaLN_cond__sliding_local_dilated__glu_gated_swiglu__prompt_kernel(
    A_x, A_wqkv, A_wo, B_x, B_w1, B_w3, B_w2, c, w_mod):
    del B_x
    any_spec = pl.BlockSpec(memory_space=pl.ANY)
    return pl.pallas_call(
        _kernel,
        out_shape=jax.ShapeDtypeStruct((1, S, D), bf16),
        in_specs=[any_spec] * 8,
        out_specs=any_spec,
        scratch_shapes=[
            pltpu.VMEM((S, D), bf16),
            pltpu.VMEM((1, D), bf16),
            pltpu.VMEM((D, 6 * D), bf16),
            pltpu.VMEM((D, 3 * D), bf16),
            pltpu.VMEM((D, D), bf16),
            pltpu.VMEM((D, F), bf16),
            pltpu.VMEM((D, F), bf16),
            pltpu.VMEM((F, D), bf16),
            pltpu.VMEM((8, 6 * D), f32),
            pltpu.VMEM((T, D), bf16),
            pltpu.VMEM((NG, QROWS, 128), f32),
            pltpu.VMEM((NG, KROWS, 128), f32),
            pltpu.VMEM((NG, KROWS, 128), f32),
            pltpu.VMEM((S, D), f32),
            pltpu.VMEM((T, D), f32),
            pltpu.VMEM((2, T, D), bf16),
            pltpu.SemaphoreType.DMA((8,)),
            pltpu.SemaphoreType.DMA((2,)),
        ],
        compiler_params=pltpu.CompilerParams(vmem_limit_bytes=110 * 2**20),
        name="adaln_fused",
    )(A_x, A_wqkv, A_wo, B_w1, B_w3, B_w2, c, w_mod)
```

```python
import functools
import jax
import jax.numpy as jnp
from jax import lax
import jax.experimental.pallas as pl
import jax.experimental.pallas.tpu as pltpu

S, D, F = 2048, 1024, 3584
H, DH, W, DIL = 32, 32, 8, 2
NG = D // 128
HALO = 16
T = 128
NT = S // T
SKEW = 3
M0 = SKEW * T
TB = 128
NTB = S // TB
FC = 512
NFC = F // FC
KOFF = 24
KROWS = T + KOFF
QROWS = T + 8
LOG2E = 1.4426950408889634
QSCALE = (DH ** -0.5) * LOG2E
NEG = -1e9 * LOG2E
EPS = 1e-5
UG = 4
f32, bf16, u32 = jnp.float32, jnp.bfloat16, jnp.uint32
scope = jax.named_scope


def _butterfly(vs):
    vs = list(vs)
    lane = lax.broadcasted_iota(jnp.int32, vs[0].shape, 1)
    for s in range(3):
        m = (lane & (4 << s)) != 0
        for g in range(NG):
            if g & (1 << s):
                continue
            a, b = vs[g], vs[g | (1 << s)]
            vs[g] = jnp.where(m, b, a)
            vs[g | (1 << s)] = jnp.where(m, a, b)
    return vs


def _to_head_lanes(vs):
    ys = _butterfly(vs)
    lane = lax.broadcasted_iota(jnp.int32, vs[0].shape, 1)
    head = lane & 31
    out = []
    for g in range(NG):
        src = ((head & 3) << 5) | (((head >> 2) ^ g) << 2) | (lane >> 5)
        out.append(jnp.take_along_axis(ys[g], src, axis=1))
    return out


def _from_head_lanes(zs):
    lane = lax.broadcasted_iota(jnp.int32, zs[0].shape, 1)
    ys = []
    for g in range(NG):
        src = ((lane & 3) << 5) | ((((lane >> 2) & 7) ^ g) << 2) | (lane >> 5)
        ys.append(jnp.take_along_axis(zs[g], src, axis=1))
    return _butterfly(ys)


def _add(a, b):
    return a + b


def _or(a, b):
    return a | b


def _after(x, dep):
    if dep is None:
        return x
    return pltpu.bitcast(pltpu.bitcast(x, u32) | dep, x.dtype)


def _ln8(xs, scale1, shift, dep):
    xs = [_after(xs[0], dep)] + list(xs[1:])
    m = jnp.sum(functools.reduce(_add, xs), axis=-1, keepdims=True) * (1.0 / D)
    xc = [v - m for v in xs]
    var = jnp.sum(functools.reduce(_add, [v * v for v in xc]), axis=-1, keepdims=True) * (1.0 / D)
    r = lax.rsqrt(var + EPS)
    return [xc[g] * r * scale1(g) + shift(g) for g in range(NG)]


def _kernel(x_hbm, wqkv_hbm, wo_hbm, w1_hbm, w3_hbm, w2_hbm, c_hbm, wmod_hbm, out_hbm,
            x_v, c_v, wmod_v, wraw_v, wp_v, wo_v, w1_v, w3_v, w2_v, mod_v,
            h0_v, h_v, h2_v, st_v, q0_v, k0_v, v0_v, q1_v, k1_v, v1_v, a_v, ob_v,
            zv_v, zs_s, sem, osem):
    X0 = M0 + T
    names = ["c", "wmod01", "x0", "wq", "wk", "wv", "wo", "xr", "wmodr", "w1", "w3", "w2"]
    srcdst = dict(
        c=(c_hbm, c_v),
        wmod01=(wmod_hbm.at[:, 0:2 * D], wmod_v.at[:, 0:2 * D]),
        x0=(x_hbm.at[0, 0:X0, :], x_v.at[0:X0, :]),
        wq=(wqkv_hbm.at[:, 0:D], wraw_v.at[:, 0:D]),
        wk=(wqkv_hbm.at[:, D:2 * D], wraw_v.at[:, D:2 * D]),
        wv=(wqkv_hbm.at[:, 2 * D:3 * D], wraw_v.at[:, 2 * D:3 * D]),
        wo=(wo_hbm, wo_v),
        xr=(x_hbm.at[0, X0:S, :], x_v.at[X0:S, :]),
        wmodr=(wmod_hbm.at[:, 2 * D:6 * D], wmod_v.at[:, 2 * D:6 * D]),
        w1=(w1_hbm, w1_v), w3=(w3_hbm, w3_v), w2=(w2_hbm, w2_v),
    )
    copies = {n: pltpu.make_async_copy(srcdst[n][0], srcdst[n][1], sem.at[i]) for i, n in enumerate(names)}
    for n in names:
        copies[n].start()
    zv_v[...] = jnp.zeros(zv_v.shape, u32)
    zs_s[0] = 0

    bufs = ((q0_v, k0_v, v0_v), (q1_v, k1_v, v1_v))
    mcol = lambda sec: (lambda g: mod_v[:, sec * D + g * 128:sec * D + (g + 1) * 128])
    groups = lambda x: [x[:, g * 128:(g + 1) * 128] for g in range(NG)]
    row8 = lax.broadcasted_iota(jnp.int32, (8, 128), 0)

    def silu_c():
        c = c_v[...].astype(f32)
        sc = (c * jax.nn.sigmoid(c)).astype(bf16)
        return jnp.broadcast_to(sc, (16, D))

    def mod_cols(sc, sec, add_one):
        m = jnp.dot(sc, wmod_v[:, sec * D:(sec + 1) * D], preferred_element_type=f32)[0:8]
        m = m + 1.0 if add_one else m
        mod_v[:, sec * D:(sec + 1) * D] = m
        return m

    def ln1_rows(row, dst, drow, dep):
        ys = _ln8(groups(x_v[pl.ds(row, 8), :].astype(f32)), mcol(1), mcol(0), dep)
        dst[drow:drow + 8, :] = jnp.concatenate(ys, axis=1).astype(bf16)
        return pltpu.bitcast(ys[NG - 1], u32)

    def x1_rows(row):
        x = groups(x_v[pl.ds(row, 8), :].astype(f32))
        a = groups(a_v[pl.ds(row, 8), :])
        return [x[g] + mcol(2)(g) * a[g] for g in range(NG)]

    def ln2_rows(row, drow, dep):
        ys = _ln8(x1_rows(row), mcol(4), mcol(3), dep)
        h2_v[drow:drow + 8, :] = jnp.concatenate(ys, axis=1).astype(bf16)
        return pltpu.bitcast(ys[NG - 1], u32)

    def perm_w(sec):
        def body(r, carry):
            r0 = pl.multiple_of(r * 64, 64)
            vs = [pltpu.bitcast(wraw_v[pl.ds(r0, 64), sec * D + g * 128: sec * D + (g + 1) * 128], u32) for g in range(NG)]
            vs = _to_head_lanes(vs)
            for g in range(NG):
                wp_v[pl.ds(pl.multiple_of(r * 32, 32), 32), sec * D + g * 128: sec * D + (g + 1) * 128] = vs[g]
            return carry
        lax.fori_loop(0, D // 64, body, 0)

    def attn8(src, t0, rb, dep):
        q_v, k_lo, k_hi, v_lo, v_hi = src
        r0 = rb * 8
        s = [None] * W
        for g in range(NG):
            q = q_v[g, r0:r0 + 8, :]
            if g == 0:
                q = _after(q, dep)
            for j in range(W):
                o = KOFF + r0 - DIL * j
                p = q * (k_lo if j < 4 else k_hi)[g, o:o + 8, :]
                s[j] = p if s[j] is None else s[j] + p
        for j in range(W):
            s[j] = s[j] + pltpu.roll(s[j], 64, 1)
            s[j] = s[j] + pltpu.roll(s[j], 32, 1)
            if t0 is not None and r0 < DIL * j:
                s[j] = jnp.where(t0 + r0 + row8 >= DIL * j, s[j], NEG)
        m = functools.reduce(jnp.maximum, s)
        e = [jnp.exp2(s[j] - m) for j in range(W)]
        den = functools.reduce(_add, e)
        r = pl.reciprocal(den, approx=True)
        inv = r * (2.0 - den * r)
        p = [e[j] * inv for j in range(W)]
        og = []
        for g in range(NG):
            acc = None
            for j in range(W):
                o = KOFF + r0 - DIL * j
                t = p[j] * (v_lo if j < 4 else v_hi)[g, o:o + 8, :]
                acc = t if acc is None else acc + t
            og.append(acc)
        return og

    def attention(par, slot, t0, dep_fn, extra_fn):
        q_v, k_v, v_v = bufs[par]
        slot2 = slot + zs_s[0]
        src = (q_v.at[slot], k_v.at[slot], k_v.at[slot2], v_v.at[slot], v_v.at[slot2])
        rows = []
        for pb in range(T // 16):
            d = dep_fn(pb)
            a = attn8(src, t0, 2 * pb, d)
            b = attn8(src, t0, 2 * pb + 1, d)
            for g in range(NG):
                st_v[pb * 8:(pb + 1) * 8, g * 128:(g + 1) * 128] = pltpu.bitcast(
                    jnp.concatenate([a[g], b[g]], axis=0).astype(bf16), u32)
            extra_fn(pb)
            if (pb + 1) % UG == 0:
                vs = _from_head_lanes(groups(st_v[(pb + 1 - UG) * 8:(pb + 1) * 8, :]))
                rows.append(jnp.concatenate([pltpu.bitcast(v, bf16) for v in vs], axis=1))
        return jnp.concatenate(rows, axis=0)

    with scope("p_mod"):
        copies["c"].wait()
        copies["wmod01"].wait()
        sc = silu_c()
        mod_cols(sc, 0, False)
        mod_cols(sc, 1, True)
        copies["x0"].wait()
        for rb in range(M0 // 8):
            ln1_rows(rb * 8, h0_v, rb * 8, None)
    for sec, n in enumerate(["wq", "wk", "wv"]):
        with scope("p_perm"):
            copies[n].wait()
            perm_w(sec)
        with scope("p_mm"):
            res = jnp.dot(h0_v[...], pltpu.bitcast(wp_v[:, sec * D:(sec + 1) * D], bf16), preferred_element_type=f32)
            for t in range(SKEW):
                dst = bufs[t % 2][sec]
                for g in range(NG):
                    blk = res[:, g * 128:(g + 1) * 128]
                    if sec == 0:
                        dst[t // 2, g, 0:T, :] = blk[t * T:(t + 1) * T] * QSCALE
                    elif t == 0:
                        dst[0, g, KOFF:KOFF + T, :] = blk[0:T]
                        dst[0, g, KOFF - HALO:KOFF, :] = jnp.broadcast_to(blk[0:1], (HALO, 128))
                    else:
                        dst[t // 2, g, KOFF - HALO:KOFF + T, :] = blk[t * T - HALO:(t + 1) * T]
            if sec == 2:
                for rb in range(T // 8):
                    ln1_rows(M0 + rb * 8, h_v, rb * 8, None)
    with scope("p_wait"):
        copies["wo"].wait()
        copies["xr"].wait()

    def step(s, par):
        zvec = zv_v[...]
        t0 = pl.multiple_of(s * T, T)
        slot = (s // 2) % 2
        dslot = ((s + SKEW) // 2) % 2
        pslot = ((s + SKEW - 1) // 2) % 2
        res = jnp.dot(h_v[...], pltpu.bitcast(wp_v[...], bf16), preferred_element_type=f32)
        tiles = [res[:, t * 128:(t + 1) * 128] for t in range(3 * NG)]
        qd, kd, vd = bufs[1 - par]
        _, kp, vp = bufs[par]
        for g in range(NG):
            qd[dslot, g, 0:T, :] = tiles[g] * QSCALE
            kd[dslot, g, KOFF:KOFF + T, :] = tiles[NG + g]
            vd[dslot, g, KOFF:KOFF + T, :] = tiles[2 * NG + g]
            kd[dslot, g, KOFF - HALO:KOFF, :] = kp[pslot, g, KOFF + T - HALO:KOFF + T, :]
            vd[dslot, g, KOFF - HALO:KOFF, :] = vp[pslot, g, KOFF + T - HALO:KOFF + T, :]
        t1 = pl.multiple_of(jnp.minimum(s + SKEW + 1, NT - 1) * T, T)
        NP = T // 16
        tile_dep = lambda pb: pltpu.bitcast(tiles[(20 * pb) // NP][T - 8:T, :], u32) & zvec
        links = []

        def dep_fn(pb):
            d = tile_dep(pb)
            if pb >= 2:
                d = d | ((links[2 * pb - 4] | links[2 * pb - 3]) & zvec)
            return d

        def extra_fn(pb):
            for rb in (2 * pb, 2 * pb + 1):
                links.append(ln1_rows(t1 + rb * 8, h_v, rb * 8, tile_dep(pb)))
        o = attention(par, slot, t0 if par == 0 else None, dep_fn, extra_fn)
        a_v[pl.ds(t0, T), :] = jnp.dot(o, wo_v[...], preferred_element_type=f32)

    NS = NT - SKEW

    def phase_a(i, carry):
        step(2 * i, 0)

        @pl.when(2 * i + 1 < NS)
        def _():
            step(2 * i + 1, 1)
        return carry
    with scope("phase_a"):
        lax.fori_loop(0, (NS + 1) // 2, phase_a, 0)

    with scope("tail_a"):
        copies["wmodr"].wait()
        zvec = zv_v[...]
        sc = silu_c()
        mods = [mod_cols(sc, sec, sec == 4) for sec in range(2, 6)]
        mt = [m[:, g * 128:(g + 1) * 128] for m in mods for g in range(NG)]
        gate = [pltpu.bitcast(mt[3 * pb], u32) & zvec for pb in range(T // 16)]
        for s in range(NS, NT):
            o = attention(s % 2, (s // 2) % 2, None, lambda pb: gate[pb], lambda pb: None)
            a = jnp.dot(o, wo_v[...], preferred_element_type=f32)
            a_v[s * T:(s + 1) * T, :] = a
            gate = [pltpu.bitcast(a[T - 8:T, ((6 * pb) // 8) * 128:((6 * pb) // 8 + 1) * 128], u32) & zvec
                    for pb in range(T // 16)]
        for rb in range(TB // 8):
            ln2_rows(rb * 8, rb * 8, gate[(rb * 8) // (TB // 8)])
        copies["w1"].wait()
        copies["w3"].wait()
        copies["w2"].wait()

    def out_copy(i, slot):
        return pltpu.make_async_copy(ob_v.at[slot], out_hbm.at[0, pl.ds(pl.multiple_of(i * TB, TB), TB), :], osem.at[slot])

    def phase_b(i, carry):
        t0 = pl.multiple_of(i * TB, TB)
        t1 = pl.multiple_of(jnp.minimum(i + 1, NTB - 1) * TB, TB)
        slot = i % 2

        @pl.when(i >= 2)
        def _():
            out_copy(i - 2, slot).wait()
        zvec = zv_v[...]
        h = h2_v[...]
        NRB = TB // 8
        per = -(-NRB // (NFC - 2))
        acc = act_prev = None
        links = []
        for fc in range(NFC + 1):
            if fc < NFC:
                g = jnp.dot(h, w1_v[:, fc * FC:(fc + 1) * FC], preferred_element_type=f32)
                u = jnp.dot(h, w3_v[:, fc * FC:(fc + 1) * FC], preferred_element_type=f32)
                lk = links[(fc - 2) * per:(fc - 1) * per] if fc >= 2 else []
                if lk:
                    u0 = _after(u[TB - 8:TB, FC - 128:FC], functools.reduce(_or, lk) & zvec)
                    u = jnp.concatenate([u[0:TB - 8, :], jnp.concatenate([u[TB - 8:TB, 0:FC - 128], u0], axis=1)], axis=0)
                hg = 0.5 * g
                act = (hg * (1.0 + jnp.tanh(hg)) * u).astype(bf16)
                for k in range(per):
                    rb = fc * per + k
                    if fc < NFC - 2 and rb < NRB:
                        ct = (k * (FC // 128)) // per
                        dep = pltpu.bitcast(u[TB - 16:TB - 8, ct * 128:(ct + 1) * 128], u32) & zvec
                        links.append(ln2_rows(t1 + rb * 8, rb * 8, dep))
            if fc >= 1:
                y = jnp.dot(act_prev, w2_v[(fc - 1) * FC:fc * FC, :], preferred_element_type=f32)
                acc = y if acc is None else acc + y
            act_prev = act
        for rb in range(NRB):
            xs = x1_rows(t0 + rb * 8)
            row = [xs[g] + mcol(5)(g) * acc[rb * 8:(rb + 1) * 8, g * 128:(g + 1) * 128] for g in range(NG)]
            ob_v[slot, rb * 8:(rb + 1) * 8, :] = jnp.concatenate(row, axis=1).astype(bf16)
        out_copy(i, slot).start()
        return carry
    with scope("phase_b"):
        lax.fori_loop(0, NTB, phase_b, 0)
    out_copy(NTB - 2, 0).wait()
    out_copy(NTB - 1, 1).wait()


@jax.jit
def pallas_adaLN_cond__sliding_local_dilated__glu_gated_swiglu__prompt_kernel(
    A_x, A_wqkv, A_wo, B_x, B_w1, B_w3, B_w2, c, w_mod):
    del B_x
    any_spec = pl.BlockSpec(memory_space=pl.ANY)
    qbuf = pltpu.VMEM((2, NG, QROWS, 128), f32)
    kbuf = pltpu.VMEM((2, NG, KROWS, 128), f32)
    return pl.pallas_call(
        _kernel,
        out_shape=jax.ShapeDtypeStruct((1, S, D), bf16),
        in_specs=[any_spec] * 8,
        out_specs=any_spec,
        scratch_shapes=[
            pltpu.VMEM((S, D), bf16),
            pltpu.VMEM((1, D), bf16),
            pltpu.VMEM((D, 6 * D), bf16),
            pltpu.VMEM((D, 3 * D), bf16),
            pltpu.VMEM((D // 2, 3 * D), u32),
            pltpu.VMEM((D, D), bf16),
            pltpu.VMEM((D, F), bf16),
            pltpu.VMEM((D, F), bf16),
            pltpu.VMEM((F, D), bf16),
            pltpu.VMEM((8, 6 * D), f32),
            pltpu.VMEM((M0, D), bf16),
            pltpu.VMEM((T, D), bf16),
            pltpu.VMEM((TB, D), bf16),
            pltpu.VMEM((T // 2, D), u32),
            qbuf, kbuf, kbuf, qbuf, kbuf, kbuf,
            pltpu.VMEM((S, D), f32),
            pltpu.VMEM((2, TB, D), bf16),
            pltpu.VMEM((8, 128), u32),
            pltpu.SMEM((1,), jnp.int32),
            pltpu.SemaphoreType.DMA((12,)),
            pltpu.SemaphoreType.DMA((2,)),
        ],
        compiler_params=pltpu.CompilerParams(vmem_limit_bytes=110 * 2**20),
        name="adaln_fused",
    )(A_x, A_wqkv, A_wo, B_w1, B_w3, B_w2, c, w_mod)
```

```python
import functools
import jax
import jax.numpy as jnp
from jax import lax
import jax.experimental.pallas as pl
import jax.experimental.pallas.tpu as pltpu

S, D, F = 2048, 1024, 3584
H, DH, W, DIL = 32, 32, 8, 2
NG = D // 128
HALO = 16
T = 128
NT = S // T
NP = T // 16
SKEW = 3
M0 = SKEW * T
NS = NT - SKEW
TB = 128
NTB = S // TB
FC = 512
NFC = F // FC
KOFF = 24
KROWS = T + KOFF
LOG2E = 1.4426950408889634
QSCALE = (DH ** -0.5) * LOG2E
NEG = -1e9 * DH ** 0.5
KC = 128
NKC = D // KC
EPS = 1e-5
UG = 4
TCHAIN = 3
f32, bf16, u32 = jnp.float32, jnp.bfloat16, jnp.uint32
scope = jax.named_scope


def _butterfly(vs):
    vs = list(vs)
    lane = lax.broadcasted_iota(jnp.int32, vs[0].shape, 1)
    for s in range(3):
        m = (lane & (4 << s)) != 0
        for g in range(NG):
            if g & (1 << s):
                continue
            a, b = vs[g], vs[g | (1 << s)]
            vs[g] = jnp.where(m, b, a)
            vs[g | (1 << s)] = jnp.where(m, a, b)
    return vs


def _to_head_lanes(vs):
    ys = _butterfly(vs)
    lane = lax.broadcasted_iota(jnp.int32, vs[0].shape, 1)
    head = lane & 31
    out = []
    for g in range(NG):
        src = ((head & 3) << 5) | (((head >> 2) ^ g) << 2) | (lane >> 5)
        out.append(jnp.take_along_axis(ys[g], src, axis=1))
    return out


def _from_head_lanes(zs):
    lane = lax.broadcasted_iota(jnp.int32, zs[0].shape, 1)
    ys = []
    for g in range(NG):
        src = ((lane & 3) << 5) | ((((lane >> 2) & 7) ^ g) << 2) | (lane >> 5)
        ys.append(jnp.take_along_axis(zs[g], src, axis=1))
    return _butterfly(ys)


def _add(a, b):
    return a + b


def _or(a, b):
    return a | b


def _bits(x):
    return pltpu.bitcast(x, u32)


def _after(x, dep):
    if dep is None:
        return x
    return pltpu.bitcast(_bits(x) | dep, x.dtype)


def _norm8(xs, dep=None):
    xs = [_after(xs[0], dep)] + list(xs[1:])
    m = jnp.sum(functools.reduce(_add, xs), axis=-1, keepdims=True) * (1.0 / D)
    xc = [v - m for v in xs]
    var = jnp.sum(functools.reduce(_add, [v * v for v in xc]), axis=-1, keepdims=True) * (1.0 / D)
    r = lax.rsqrt(var + EPS)
    return [v * r for v in xc]


def _groups(x):
    return [x[:, g * 128:(g + 1) * 128] for g in range(x.shape[1] // 128)]


def _kernel(x_hbm, wqkv_hbm, wo_hbm, w1_hbm, w3_hbm, w2_hbm, c_hbm, wmod_hbm, out_hbm,
            x_v, c_v, sc_v, wm_v, wmod_v, wraw_v, wpe_v, wpo_v, wo_v, w1_v, w3_v, w2_v, mod_v,
            xn_v, he_v, ho_v, h_v, h2_v, st_v, p0_v, p1_v, a_v, ob_v,
            zv_v, sem, osem):
    names = ["c", "x0", "wo", "wmodr", "w1", "w3", "w2"]
    srcdst = dict(
        c=(c_hbm, c_v),
        x0=(x_hbm.at[0, 0:M0, :], x_v.at[0:M0, :]),
        wo=(wo_hbm, wo_v),
        wmodr=(wmod_hbm.at[:, 2 * D:6 * D], wmod_v),
        w1=(w1_hbm, w1_v), w3=(w3_hbm, w3_v), w2=(w2_hbm, w2_v),
    )
    copies = {n: pltpu.make_async_copy(srcdst[n][0], srcdst[n][1], sem.at[i]) for i, n in enumerate(names)}

    def chunk_copies(c):
        col = pl.multiple_of(c * KC, KC)
        s0 = len(names) + 3 * c
        return [
            pltpu.make_async_copy(wmod_hbm.at[:, pl.ds(col, KC)], wm_v.at[c], sem.at[s0]),
            pltpu.make_async_copy(wmod_hbm.at[:, pl.ds(D + col, KC)], wm_v.at[NKC + c], sem.at[s0 + 1]),
            pltpu.make_async_copy(wqkv_hbm.at[pl.ds(col, KC), :], wraw_v.at[pl.ds(col, KC), :], sem.at[s0 + 2]),
        ]

    def x_copy(t):
        rows = pl.ds(pl.multiple_of(t * T, T), T)
        return pltpu.make_async_copy(x_hbm.at[0, rows, :], x_v.at[rows, :], sem.at[len(names) + 3 * NKC + t])

    copies["c"].start()
    copies["x0"].start()
    for c in range(NKC):
        for cp in chunk_copies(c):
            cp.start()
    x_copy(SKEW).start()
    x_copy(SKEW + 1).start()
    copies["wo"].start()
    for t in range(SKEW + 2, NT):
        x_copy(t).start()
    for n in ("wmodr", "w1", "w3", "w2"):
        copies[n].start()
    zv_v[...] = jnp.zeros(zv_v.shape, u32)

    proj = (p0_v, p1_v)
    mcol = lambda sec, g: mod_v[sec * NG + g]
    row8 = lax.broadcasted_iota(jnp.int32, (8, 128), 0)

    def mod_cols(sec, add_one):
        m = jnp.dot(sc_v[...], wmod_v[:, (sec - 2) * D:(sec - 1) * D], preferred_element_type=f32)[0:8]
        m = _groups(m + 1.0 if add_one else m)
        for g in range(NG):
            mod_v[sec * NG + g] = m[g]
        return m

    def wperm():
        w = [(wpe_v, wpo_v)[c % 2][c // 2] for c in range(NKC)]
        return pltpu.bitcast(jnp.concatenate(w, axis=0), bf16)

    def ln1_rows(row, drow, dep):
        xn = _norm8(_groups(x_v[pl.ds(row, 8), :].astype(f32)), dep)
        ys = [xn[g] * mcol(1, g) + mcol(0, g) for g in range(NG)]
        h_v[drow:drow + 8, :] = jnp.concatenate(ys, axis=1).astype(bf16)
        return _bits(ys[NG - 1])

    def x1_rows(row):
        x = _groups(x_v[pl.ds(row, 8), :].astype(f32))
        return [x[g] + mcol(2, g) * a_v[g, pl.ds(row, 8), :] for g in range(NG)]

    def ln2_rows(row, drow, dep):
        xn = _norm8(x1_rows(row), dep)
        ys = [xn[g] * mcol(4, g) + mcol(3, g) for g in range(NG)]
        h2_v[drow:drow + 8, :] = jnp.concatenate(ys, axis=1).astype(bf16)
        return _bits(ys[NG - 1])

    def attn8(src, t0, pb, par, dep):
        r0 = KOFF + 16 * pb + par
        rows = lambda j: pl.ds(r0 - DIL * j, 8, stride=DIL)
        s = [None] * W
        for g in range(NG):
            q = src[g, rows(0), :]
            if g == 0:
                q = _after(q, dep)
            for j in range(W):
                p = q * src[NG + g, rows(j), :]
                s[j] = p if s[j] is None else s[j] + p
        for j in range(W):
            s[j] = s[j] + pltpu.roll(s[j], 64, 1)
            s[j] = s[j] + pltpu.roll(s[j], 32, 1)
            if t0 is not None and pb == 0 and j > 0:
                s[j] = jnp.where(t0 + par + DIL * row8 >= DIL * j, s[j], NEG)
        m = functools.reduce(jnp.maximum, s)
        e = [jnp.exp2((s[j] - m) * QSCALE) for j in range(W)]
        den = functools.reduce(_add, e)
        r = pl.reciprocal(den, approx=True)
        inv = r * (2.0 - den * r)
        p = [e[j] * inv for j in range(W)]
        og = []
        for g in range(NG):
            acc = None
            for j in range(W):
                t = p[j] * src[2 * NG + g, rows(j), :]
                acc = t if acc is None else acc + t
            og.append(acc)
        return og

    def attention(src, t0, dep_fn, extra_fn):
        rows = []
        for pb in range(NP):
            d = dep_fn(pb)
            a = attn8(src, t0, pb, 0, d)
            b = attn8(src, t0, pb, 1, d)
            for g in range(NG):
                st_v[pb * 8:(pb + 1) * 8, g * 128:(g + 1) * 128] = _bits(
                    jnp.concatenate([a[g], b[g]], axis=0).astype(bf16))
            extra_fn(pb, _bits(a[NG - 1]) | _bits(b[NG - 1]))
            if (pb + 1) % UG == 0:
                vs = _from_head_lanes(_groups(st_v[(pb + 1 - UG) * 8:(pb + 1) * 8, :]))
                rows.append(jnp.concatenate([pltpu.bitcast(v, bf16) for v in vs], axis=1))
        return jnp.concatenate(rows, axis=0)

    def out_proj(o, t0):
        a = jnp.dot(o, wo_v[...], preferred_element_type=f32)
        for g in range(NG):
            for rb in range(T // 8):
                a_v[g, pl.ds(t0 + (rb // 2) * 16 + rb % 2, 8, stride=2), :] = a[rb * 8:(rb + 1) * 8, g * 128:(g + 1) * 128]
        return a

    def chunk_block(c, par, do_prep, do_mm, extra=None):
        zvec = zv_v[...]
        links = {}

        def link(ct, v):
            links[ct] = (links[ct] | v) if ct in links else v
        if do_prep:
            sc = sc_v[...]
            sh = jnp.dot(sc, wm_v[c], preferred_element_type=f32)[0:8]
            s1 = jnp.dot(sc, wm_v[NKC + c], preferred_element_type=f32)[0:8] + 1.0
        if do_mm:
            wprev = pltpu.bitcast((wpe_v, wpo_v)[1 - par][(c - 1) >> 1], bf16)
            res = jnp.dot((he_v, ho_v)[1 - par][...], wprev, preferred_element_type=f32)
        if do_prep:
            mod_v[c] = sh
            mod_v[NG + c] = s1
            hc = (xn_v[c].reshape(M0 // 8, 8, 128) * s1 + sh).reshape(M0, 128)
            (he_v, ho_v)[par][...] = hc.astype(bf16)
            link(8, _bits(hc[M0 - 8:M0]))
            wp = (wpe_v, wpo_v)[par]
            for b in range(6):
                sec, half = b // 2, b % 2
                r0 = pl.multiple_of(c * KC + half * 64, 64)
                vs = _groups(_bits(wraw_v[pl.ds(r0, 64), sec * D:(sec + 1) * D]))
                if do_mm:
                    d = _bits(res[M0 - 8:M0, 3 * b * 128:(3 * b + 1) * 128]) & zvec
                    vs[0] = jnp.concatenate([vs[0][0:8] | d, vs[0][8:32]], axis=0)
                vs = _to_head_lanes(vs)
                wp[c >> 1, half * 32:(half + 1) * 32, sec * D:(sec + 1) * D] = jnp.concatenate(vs, axis=1)
                link(3 * b + 7, vs[NG - 1][24:32])
        if extra is not None:
            extra(res, link, zvec)
        if do_mm:
            for ct in range(3 * NG):
                for t in range(SKEW):
                    blk = res[t * T:(t + 1) * T, ct * 128:(ct + 1) * 128]
                    if t == SKEW - 1 and ct in links:
                        blk = jnp.concatenate([blk[0:T - 8], _after(blk[T - 8:T], links[ct] & zvec)], axis=0)
                    proj[t % 2][t // 2, ct, KOFF:KOFF + T, :] += blk

    with scope("p_first"):
        for t in range(SKEW):
            proj[t % 2][t // 2, :, KOFF:KOFF + T, :] = jnp.zeros((3 * NG, T, 128), f32)
        copies["c"].wait()
        c32 = c_v[...].astype(f32)
        sc_v[...] = jnp.broadcast_to((c32 * jax.nn.sigmoid(c32)).astype(bf16), (16, D))
        copies["x0"].wait()
        for rb in range(M0 // 8):
            xn = _norm8(_groups(x_v[rb * 8:(rb + 1) * 8, :].astype(f32)))
            for g in range(NG):
                xn_v[g, rb * 8:(rb + 1) * 8, :] = xn[g]
        for cp in chunk_copies(0):
            cp.wait()
        chunk_block(0, 0, True, False)

    def kloop(i, carry):
        for cp in chunk_copies(2 * i + 1):
            cp.wait()
        chunk_block(2 * i + 1, 1, True, True)

        @pl.when(2 * i + 2 < NKC)
        def _():
            for cp in chunk_copies(2 * i + 2):
                cp.wait()
            chunk_block(2 * i + 2, 0, True, True)
        return carry
    with scope("p_kloop"):
        lax.fori_loop(0, NKC // 2, kloop, 0)

    with scope("p_last"):
        x_copy(SKEW).wait()

        def ln_next(res, link, zvec):
            for rb in range(T // 8):
                dep = _bits(res[M0 - 8:M0, rb * 128:(rb + 1) * 128]) & zvec
                link(rb + 6, ln1_rows(M0 + rb * 8, rb * 8, dep))
        chunk_block(NKC, 0, False, True, ln_next)
        for t in range(SKEW):
            for sg in range(NG, 3 * NG):
                if t == 0:
                    halo = jnp.broadcast_to(p0_v[0, sg, KOFF:KOFF + 1, :], (HALO, 128))
                else:
                    halo = proj[(t - 1) % 2][(t - 1) // 2, sg, KOFF + T - HALO:KOFF + T, :]
                proj[t % 2][t // 2, sg, KOFF - HALO:KOFF, :] = halo
        copies["wo"].wait()

    def step(s, par):
        @pl.when(s + SKEW + 1 < NT)
        def _():
            x_copy(s + SKEW + 1).wait()
        zvec = zv_v[...]
        t0 = pl.multiple_of(s * T, T)
        slot = (s >> 1) & 1
        dst = proj[1 - par].at[((s + SKEW) >> 1) & 1]
        prev = proj[par].at[1 - slot]
        tiles = _groups(jnp.dot(h_v[...], wperm(), preferred_element_type=f32))
        for ct in range(3 * NG):
            dst[ct, KOFF:KOFF + T, :] = tiles[ct]
            if ct >= NG:
                dst[ct, KOFF - HALO:KOFF, :] = prev[ct, KOFF + T - HALO:KOFF + T, :]
        t1 = pl.multiple_of(jnp.minimum(s + SKEW + 1, NT - 1) * T, T)
        tile_dep = lambda pb: _bits(tiles[(20 * pb) // NP][T - 8:T, :]) & zvec
        links = []

        def dep_fn(pb):
            d = tile_dep(pb)
            if pb >= 2:
                d = d | ((links[2 * pb - 4] | links[2 * pb - 3]) & zvec)
            return d

        def extra_fn(pb, _):
            for rb in (2 * pb, 2 * pb + 1):
                links.append(ln1_rows(t1 + rb * 8, rb * 8, tile_dep(pb)))
        o = attention(proj[par].at[slot], t0 if par == 0 else None, dep_fn, extra_fn)
        out_proj(o, t0)

    def phase_a(i, carry):
        step(2 * i, 0)

        @pl.when(2 * i + 1 < NS)
        def _():
            step(2 * i + 1, 1)
        return carry
    with scope("phase_a"):
        lax.fori_loop(0, (NS + 1) // 2, phase_a, 0)

    with scope("tail_a"):
        copies["wmodr"].wait()
        zvec = zv_v[...]
        for sec in range(2, 6):
            mod_cols(sec, sec == 4)
        chain = []
        for s in range(NS, NT):
            dep_fn = lambda pb: (chain[-TCHAIN] & zvec) if len(chain) >= TCHAIN else None
            o = attention(proj[s % 2].at[(s // 2) % 2], None, dep_fn, lambda pb, lk: chain.append(lk))
            a = out_proj(o, s * T)
        for rb in range(TB // 8):
            ct = (6 * rb) // (TB // 8)
            ln2_rows(rb * 8, rb * 8, _bits(a[T - 8:T, ct * 128:(ct + 1) * 128]) & zvec)
        copies["w1"].wait()
        copies["w3"].wait()
        copies["w2"].wait()

    def out_copy(i, slot):
        return pltpu.make_async_copy(ob_v.at[slot], out_hbm.at[0, pl.ds(pl.multiple_of(i * TB, TB), TB), :], osem.at[slot])

    def phase_b(i, carry):
        t0 = pl.multiple_of(i * TB, TB)
        t1 = pl.multiple_of(jnp.minimum(i + 1, NTB - 1) * TB, TB)
        slot = i & 1

        @pl.when(i >= 2)
        def _():
            out_copy(i - 2, slot).wait()
        zvec = zv_v[...]
        h = h2_v[...]
        NRB = TB // 8
        per = -(-NRB // (NFC - 2))
        acc = act_prev = None
        links = []
        for fc in range(NFC + 1):
            if fc < NFC:
                g = jnp.dot(h, w1_v[:, fc * FC:(fc + 1) * FC], preferred_element_type=f32)
                u = jnp.dot(h, w3_v[:, fc * FC:(fc + 1) * FC], preferred_element_type=f32)
                lk = links[(fc - 2) * per:(fc - 1) * per] if fc >= 2 else []
                if lk:
                    u0 = _after(u[TB - 8:TB, FC - 128:FC], functools.reduce(_or, lk) & zvec)
                    u = jnp.concatenate([u[0:TB - 8, :], jnp.concatenate([u[TB - 8:TB, 0:FC - 128], u0], axis=1)], axis=0)
                hg = 0.5 * g
                act = (hg * (1.0 + jnp.tanh(hg)) * u).astype(bf16)
                for k in range(per):
                    rb = fc * per + k
                    if fc < NFC - 2 and rb < NRB:
                        ct = (k * (FC // 128)) // per
                        dep = _bits(u[TB - 16:TB - 8, ct * 128:(ct + 1) * 128]) & zvec
                        links.append(ln2_rows(t1 + rb * 8, rb * 8, dep))
            if fc >= 1:
                y = jnp.dot(act_prev, w2_v[(fc - 1) * FC:fc * FC, :], preferred_element_type=f32)
                acc = y if acc is None else acc + y
            act_prev = act
        for rb in range(NRB):
            xs = x1_rows(t0 + rb * 8)
            row = [xs[g] + mcol(5, g) * acc[rb * 8:(rb + 1) * 8, g * 128:(g + 1) * 128] for g in range(NG)]
            ob_v[slot, rb * 8:(rb + 1) * 8, :] = jnp.concatenate(row, axis=1).astype(bf16)
        out_copy(i, slot).start()
        return carry
    with scope("phase_b"):
        lax.fori_loop(0, NTB, phase_b, 0)
    out_copy(NTB - 2, 0).wait()
    out_copy(NTB - 1, 1).wait()


@jax.jit
def pallas_adaLN_cond__sliding_local_dilated__glu_gated_swiglu__prompt_kernel(
    A_x, A_wqkv, A_wo, B_x, B_w1, B_w3, B_w2, c, w_mod):
    del B_x
    any_spec = pl.BlockSpec(memory_space=pl.ANY)
    return pl.pallas_call(
        _kernel,
        out_shape=jax.ShapeDtypeStruct((1, S, D), bf16),
        in_specs=[any_spec] * 8,
        out_specs=any_spec,
        scratch_shapes=[
            pltpu.VMEM((S, D), bf16),
            pltpu.VMEM((1, D), bf16),
            pltpu.VMEM((16, D), bf16),
            pltpu.VMEM((2 * NKC, D, KC), bf16),
            pltpu.VMEM((D, 4 * D), bf16),
            pltpu.VMEM((D, 3 * D), bf16),
            pltpu.VMEM((NKC // 2, KC // 2, 3 * D), u32),
            pltpu.VMEM((NKC // 2, KC // 2, 3 * D), u32),
            pltpu.VMEM((D, D), bf16),
            pltpu.VMEM((D, F), bf16),
            pltpu.VMEM((D, F), bf16),
            pltpu.VMEM((F, D), bf16),
            pltpu.VMEM((6 * NG, 8, 128), f32),
            pltpu.VMEM((NG, M0, 128), f32),
            pltpu.VMEM((M0, KC), bf16),
            pltpu.VMEM((M0, KC), bf16),
            pltpu.VMEM((T, D), bf16),
            pltpu.VMEM((TB, D), bf16),
            pltpu.VMEM((T // 2, D), u32),
            pltpu.VMEM((2, 3 * NG, KROWS, 128), f32),
            pltpu.VMEM((2, 3 * NG, KROWS, 128), f32),
            pltpu.VMEM((NG, S + 8, 128), f32),
            pltpu.VMEM((2, TB, D), bf16),
            pltpu.VMEM((8, 128), u32),
            pltpu.SemaphoreType.DMA((7 + 3 * NKC + NT,)),
            pltpu.SemaphoreType.DMA((2,)),
        ],
        compiler_params=pltpu.CompilerParams(vmem_limit_bytes=110 * 2**20),
        name="adaln_fused",
    )(A_x, A_wqkv, A_wo, B_w1, B_w3, B_w2, c, w_mod)
```

```python
import functools
import jax
import jax.numpy as jnp
from jax import lax
import jax.experimental.pallas as pl
import jax.experimental.pallas.tpu as pltpu

S, D, F = 2048, 1024, 3584
H, DH, W, DIL = 32, 32, 8, 2
NG = D // 128
HALO = 16
T = 128
NT = S // T
NP = T // 16
SKEW = 3
M0 = SKEW * T
NS = NT - SKEW
TB = 128
NTB = S // TB
FC = 512
NFC = F // FC
KOFF = 24
KROWS = T + KOFF
LOG2E = 1.4426950408889634
QSCALE = (DH ** -0.5) * LOG2E
NEG = -1e9 * DH ** 0.5
KC = 128
NKC = D // KC
NMOD = 6 * NG
MPS = 3
MLAG = 2
EPS = 1e-5
G0, GN = 3, 5
UG = 4
f32, bf16, u32 = jnp.float32, jnp.bfloat16, jnp.uint32
scope = jax.named_scope


def _butterfly(vs):
    vs = list(vs)
    lane = lax.broadcasted_iota(jnp.int32, vs[0].shape, 1)
    for s in range(3):
        m = (lane & (4 << s)) != 0
        for g in range(NG):
            if g & (1 << s):
                continue
            a, b = vs[g], vs[g | (1 << s)]
            vs[g] = jnp.where(m, b, a)
            vs[g | (1 << s)] = jnp.where(m, a, b)
    return vs


def _to_head_lanes(vs):
    ys = _butterfly(vs)
    lane = lax.broadcasted_iota(jnp.int32, vs[0].shape, 1)
    head = lane & 31
    out = []
    for g in range(NG):
        src = ((head & 3) << 5) | (((head >> 2) ^ g) << 2) | (lane >> 5)
        out.append(jnp.take_along_axis(ys[g], src, axis=1))
    return out


def _from_head_lanes(zs):
    lane = lax.broadcasted_iota(jnp.int32, zs[0].shape, 1)
    ys = []
    for g in range(NG):
        src = ((lane & 3) << 5) | ((((lane >> 2) & 7) ^ g) << 2) | (lane >> 5)
        ys.append(jnp.take_along_axis(zs[g], src, axis=1))
    return _butterfly(ys)


def _add(a, b):
    return a + b


def _or(a, b):
    return a | b


def _bits(x):
    return pltpu.bitcast(x, u32)


def _dot(a, b):
    return jnp.dot(a, b, preferred_element_type=f32)


def _after(x, dep):
    if dep is None:
        return x
    return pltpu.bitcast(_bits(x) | dep, x.dtype)


def _norm8(xs, dep=None):
    xs = [_after(xs[0], dep)] + list(xs[1:])
    m = jnp.sum(functools.reduce(_add, xs), axis=-1, keepdims=True) * (1.0 / D)
    xc = [v - m for v in xs]
    var = jnp.sum(functools.reduce(_add, [v * v for v in xc]), axis=-1, keepdims=True) * (1.0 / D)
    r = lax.rsqrt(var + EPS)
    return [v * r for v in xc]


def _groups(x):
    return [x[:, g * 128:(g + 1) * 128] for g in range(x.shape[1] // 128)]


def _kernel(x_hbm, wqkv_hbm, wo_hbm, w1_hbm, w3_hbm, w2_hbm, c_hbm, wmod_hbm, out_hbm,
            x_v, c_v, sc_v, wm_v, wraw_v, wpe_v, wpo_v, wo_v, w1_v, w3_v, w2_v, mod_v, modr_v,
            xn_v, he_v, ho_v, h_v, h2_v, st_v, o_v, p0_v, p1_v, a_v, ob_v,
            zv_v, sem, osem):
    names = ["c", "x0", "wo", "w1", "w3", "w2"]
    srcdst = dict(
        c=(c_hbm, c_v),
        x0=(x_hbm.at[0, 0:M0, :], x_v.at[0:M0, :]),
        wo=(wo_hbm, wo_v),
        w1=(w1_hbm, w1_v), w3=(w3_hbm, w3_v), w2=(w2_hbm, w2_v),
    )
    copies = {n: pltpu.make_async_copy(srcdst[n][0], srcdst[n][1], sem.at[i]) for i, n in enumerate(names)}
    SEM_C = len(names)
    SEM_X = SEM_C + NKC
    SEM_M = SEM_X + NT

    def slab_copy(j, s):
        return pltpu.make_async_copy(wmod_hbm.at[:, pl.ds(pl.multiple_of(j * 128, 128), 128)], wm_v.at[j], sem.at[s])

    def chunk_copies(c):
        rows = pl.ds(pl.multiple_of(c * KC, KC), KC)
        return [slab_copy(c, SEM_C + c), slab_copy(NG + c, SEM_C + c),
                pltpu.make_async_copy(wqkv_hbm.at[rows, :], wraw_v.at[rows, :], sem.at[SEM_C + c])]

    def x_copy(t):
        rows = pl.ds(pl.multiple_of(t * T, T), T)
        return pltpu.make_async_copy(x_hbm.at[0, rows, :], x_v.at[rows, :], sem.at[SEM_X + t])

    copies["c"].start()
    copies["x0"].start()
    for c in range(NKC):
        for cp in chunk_copies(c):
            cp.start()
    x_copy(SKEW).start()
    x_copy(SKEW + 1).start()
    copies["wo"].start()
    for t in range(SKEW + 2, NT):
        x_copy(t).start()
    for j in range(2 * NG, NMOD):
        slab_copy(j, SEM_M + (j - 2 * NG) // MPS).start()
    for n in ("w1", "w3", "w2"):
        copies[n].start()
    zv_v[...] = jnp.zeros(zv_v.shape, u32)

    proj = (p0_v, p1_v)
    mcol = lambda sec, g: (mod_v if sec < 2 else modr_v)[sec * NG + g]
    row8 = lax.broadcasted_iota(jnp.int32, (8, 128), 0)

    def mod_round(j, kh):
        ks = slice(kh * 512, (kh + 1) * 512)
        return _dot(sc_v[:, ks], wm_v[j, ks, :])[0:8]

    def ln1_rows(row, drow, dep):
        xn = _norm8(_groups(x_v[pl.ds(row, 8), :].astype(f32)), dep)
        ys = [xn[g] * mcol(1, g) + mcol(0, g) for g in range(NG)]
        h_v[drow:drow + 8, :] = jnp.concatenate(ys, axis=1).astype(bf16)
        return _bits(ys[NG - 1])

    def x1_rows(row):
        x = _groups(x_v[pl.ds(row, 8), :].astype(f32))
        return [x[g] + mcol(2, g) * a_v[g, pl.ds(row, 8), :] for g in range(NG)]

    def ln2_rows(row, drow, dep):
        xn = _norm8(x1_rows(row), dep)
        ys = [xn[g] * mcol(4, g) + mcol(3, g) for g in range(NG)]
        h2_v[drow:drow + 8, :] = jnp.concatenate(ys, axis=1).astype(bf16)
        return _bits(ys[NG - 1])

    def attn8(src, t0, pb, par, dep):
        r0 = KOFF + 16 * pb + par
        rows = lambda j: pl.ds(r0 - DIL * j, 8, stride=DIL)
        s = [None] * W
        for g in range(NG):
            q = src[g, rows(0), :]
            if g == 0:
                q = _after(q, dep)
            for j in range(W):
                p = q * src[NG + g, rows(j), :]
                s[j] = p if s[j] is None else s[j] + p
        for j in range(W):
            s[j] = s[j] + pltpu.roll(s[j], 64, 1)
            s[j] = s[j] + pltpu.roll(s[j], 32, 1)
            if t0 is not None and pb == 0 and j > 0:
                s[j] = jnp.where(t0 + par + DIL * row8 >= DIL * j, s[j], NEG)
        m = functools.reduce(jnp.maximum, s)
        e = [jnp.exp2((s[j] - m) * QSCALE) for j in range(W)]
        den = functools.reduce(_add, e)
        r = pl.reciprocal(den, approx=True)
        inv = r * (2.0 - den * r)
        p = [e[j] * inv for j in range(W)]
        og = []
        for g in range(NG):
            acc = None
            for j in range(W):
                t = p[j] * src[2 * NG + g, rows(j), :]
                acc = t if acc is None else acc + t
            og.append(acc)
        return og

    def attn16(src, t0, pb, srow, dep):
        a = attn8(src, t0, pb, 0, dep)
        b = attn8(src, t0, pb, 1, dep)
        for g in range(NG):
            st_v[srow:srow + 8, g * 128:(g + 1) * 128] = _bits(jnp.concatenate([a[g], b[g]], axis=0).astype(bf16))
        return _bits(a[NG - 1]) | _bits(b[NG - 1])

    def unstage(r0, r1):
        return jnp.concatenate(_from_head_lanes(_groups(st_v[r0:r1, :])), axis=1)

    def out_proj(o, t0):
        a = _dot(o, wo_v[...])
        for g in range(NG):
            for rb in range(a.shape[0] // 8):
                a_v[g, pl.ds(t0 + (rb // 2) * 16 + rb % 2, 8, stride=2), :] = a[rb * 8:(rb + 1) * 8, g * 128:(g + 1) * 128]

    def chunk_block(c, par, do_prep, do_mm, extra=None):
        zvec = zv_v[...]
        links = {}

        def link(ct, v):
            links[ct] = (links[ct] | v) if ct in links else v
        res, mr = [], []
        if do_mm:
            hprev = (he_v, ho_v)[1 - par][...]
            wprev = (wpe_v, wpo_v)[1 - par].at[(c - 1) >> 1]
        for r in range(6):
            if do_mm:
                res += _groups(_dot(hprev, pltpu.bitcast(wprev[:, r * 512:(r + 1) * 512], bf16)))
            if do_prep and r < 4:
                mr.append(mod_round(c + NG * (r // 2), r % 2))
        if do_prep:
            sh = mr[0] + mr[1]
            s1 = mr[2] + mr[3] + 1.0
            mod_v[c] = sh
            mod_v[NG + c] = s1
            hc = (xn_v[c].reshape(M0 // 8, 8, 128) * s1 + sh).reshape(M0, 128)
            (he_v, ho_v)[par][...] = hc.astype(bf16)
            link(22, _bits(hc[M0 - 8:M0]))
            wp = (wpe_v, wpo_v)[par]
            for b in range(6):
                sec, half = b // 2, b % 2
                r0 = pl.multiple_of(c * KC + half * 64, 64)
                vs = _groups(_bits(wraw_v[pl.ds(r0, 64), sec * D:(sec + 1) * D]))
                if do_mm:
                    d = _bits(res[3 * b][M0 - 8:M0]) & zvec
                    vs[0] = jnp.concatenate([vs[0][0:8] | d, vs[0][8:32]], axis=0)
                vs = _to_head_lanes(vs)
                wp[c >> 1, half * 32:(half + 1) * 32, sec * D:(sec + 1) * D] = jnp.concatenate(vs, axis=1)
                link(3 * b + 7, vs[NG - 1][24:32])
        if extra is not None:
            extra(res, link, zvec)
        if do_mm:
            for ct in range(3 * NG):
                for t in range(SKEW):
                    blk = res[ct][t * T:(t + 1) * T]
                    if t == SKEW - 1 and ct in links:
                        blk = jnp.concatenate([blk[0:T - 8], _after(blk[T - 8:T], links[ct] & zvec)], axis=0)
                    proj[t % 2][t // 2, ct, KOFF:KOFF + T, :] += blk

    with scope("p_first"):
        for t in range(SKEW):
            proj[t % 2][t // 2, :, KOFF:KOFF + T, :] = jnp.zeros((3 * NG, T, 128), f32)
        copies["c"].wait()
        c32 = c_v[...].astype(f32)
        sc_v[...] = jnp.broadcast_to((c32 * jax.nn.sigmoid(c32)).astype(bf16), (16, D))
        copies["x0"].wait()
        for rb in range(M0 // 8):
            xn = _norm8(_groups(x_v[rb * 8:(rb + 1) * 8, :].astype(f32)))
            for g in range(NG):
                xn_v[g, rb * 8:(rb + 1) * 8, :] = xn[g]
        for cp in chunk_copies(0):
            cp.wait()
        chunk_block(0, 0, True, False)

    def kloop(i, carry):
        for cp in chunk_copies(2 * i + 1):
            cp.wait()
        chunk_block(2 * i + 1, 1, True, True)

        @pl.when(2 * i + 2 < NKC)
        def _():
            for cp in chunk_copies(2 * i + 2):
                cp.wait()
            chunk_block(2 * i + 2, 0, True, True)
        return carry
    with scope("p_kloop"):
        lax.fori_loop(0, NKC // 2, kloop, 0)

    with scope("p_last"):
        x_copy(SKEW).wait()

        def ln_next(res, link, zvec):
            for rb in range(T // 8):
                link(rb + 6, ln1_rows(M0 + rb * 8, rb * 8, _bits(res[rb][M0 - 8:M0]) & zvec))
        chunk_block(NKC, 0, False, True, ln_next)
        for t in range(SKEW):
            for sg in range(NG, 3 * NG):
                if t == 0:
                    halo = jnp.broadcast_to(p0_v[0, sg, KOFF:KOFF + 1, :], (HALO, 128))
                else:
                    halo = proj[(t - 1) % 2][(t - 1) // 2, sg, KOFF + T - HALO:KOFF + T, :]
                proj[t % 2][t // 2, sg, KOFF - HALO:KOFF, :] = halo
        copies["wo"].wait()

    def step(s, par):
        @pl.when(s + SKEW + 1 < NT)
        def _():
            x_copy(s + SKEW + 1).wait()
        jn = 2 * NG + MPS * (s - MLAG)
        for k in range(MPS):
            @pl.when((s >= MLAG) & (jn + k < NMOD))
            def _():
                slab_copy(jn + k, SEM_M + s - MLAG).wait()
        j0 = jnp.where(s >= MLAG, jnp.minimum(jn, NMOD - MPS), 0)
        zvec = zv_v[...]
        t0 = pl.multiple_of(s * T, T)
        slot = (s >> 1) & 1
        dst = proj[1 - par].at[((s + SKEW) >> 1) & 1]
        prev = proj[par].at[1 - slot]
        h = h_v[...]
        tiles, mr = [], []
        for r in range(8):
            cols = slice(r * 384, (r + 1) * 384)
            w = jnp.concatenate([(wpe_v, wpo_v)[c % 2][c // 2, :, cols] for c in range(NKC)], axis=0)
            tiles += _groups(_dot(h, pltpu.bitcast(w, bf16)))
            if r < 2 * MPS:
                mr.append(mod_round(j0 + r // 2, r % 2))
        for k in range(MPS):
            one = jnp.where((j0 + k) >> 3 == 4, 1.0, 0.0)
            modr_v[j0 + k] = mr[2 * k] + mr[2 * k + 1] + one
        for ct in range(3 * NG):
            dst[ct, KOFF:KOFF + T, :] = tiles[ct]
            if ct >= NG:
                dst[ct, KOFF - HALO:KOFF, :] = prev[ct, KOFF + T - HALO:KOFF + T, :]
        t1 = pl.multiple_of(jnp.minimum(s + SKEW + 1, NT - 1) * T, T)
        src = proj[par].at[slot]
        links, rows = [], []
        for pb in range(NP):
            gate = _bits(tiles[(20 * pb) // NP][T - 8:T, :]) & zvec
            d = gate if pb < 2 else gate | ((links[2 * pb - 4] | links[2 * pb - 3]) & zvec)
            attn16(src, t0 if par == 0 else None, pb, pb * 8, d)
            for rb in (2 * pb, 2 * pb + 1):
                links.append(ln1_rows(t1 + rb * 8, rb * 8, gate))
            if (pb + 1) % UG == 0:
                rows.append(pltpu.bitcast(unstage((pb + 1 - UG) * 8, (pb + 1) * 8), bf16))
        out_proj(jnp.concatenate(rows, axis=0), t0)

    def phase_a(i, carry):
        step(2 * i, 0)

        @pl.when(2 * i + 1 < NS)
        def _():
            step(2 * i + 1, 1)
        return carry
    with scope("phase_a"):
        lax.fori_loop(0, (NS + 1) // 2, phase_a, 0)

    moved = pltpu.make_async_copy(p0_v.at[1], p1_v.at[2], osem.at[2])
    with scope("mid"):
        moved.start()
        for rb in range(TB // 8):
            ln2_rows(rb * 8, rb * 8, None)
        copies["w1"].wait()
        copies["w3"].wait()
        copies["w2"].wait()

    def out_copy(i, slot):
        return pltpu.make_async_copy(ob_v.at[slot], out_hbm.at[0, pl.ds(pl.multiple_of(i * TB, TB), TB), :], osem.at[slot])

    def phase_b(i, carry):
        t0 = pl.multiple_of(i * TB, TB)
        t1 = pl.multiple_of(jnp.minimum(i + 1, NTB - 1) * TB, TB)
        slot = i & 1

        @pl.when(i == 3 * NP // 2)
        def _():
            out_proj(pltpu.bitcast(o_v[...], bf16), NS * T)

        @pl.when(i == NP)
        def _():
            moved.wait()

        @pl.when(i >= 2)
        def _():
            out_copy(i - 2, slot).wait()
        zvec = zv_v[...]
        sl = (i >> 2) % 3
        ra = pl.multiple_of((i & 3) * 32, 32)
        src = p1_v.at[sl, :, pl.ds(ra, KOFF + 32), :]
        orow = jnp.where(sl == 0, 0, jnp.where(sl == 1, T, T // 2)) + (i & 3) * 16

        def fin(dep):
            o = unstage(0, 16)
            o_v[pl.ds(pl.multiple_of(orow, 16), 16), :] = o
            return o[8:16, D - 128:D]
        side = [[lambda d, r=r: ln2_rows(t1 + r * 8, r * 8, d) for r in range(4 * k, 4 * k + 4)] for k in range(4)]
        side[0].insert(0, lambda d: attn16(src, None, 0, 0, d))
        side[1].insert(0, lambda d: attn16(src, None, 1, 8, d))
        side[3].append(fin)
        h = h2_v[...]
        acc = act_prev = None
        links = []
        for fc in range(NFC + 1):
            if fc < NFC:
                g = _dot(h, w1_v[:, fc * FC:(fc + 1) * FC])
                u = _dot(h, w3_v[:, fc * FC:(fc + 1) * FC])
                if 2 <= fc < len(side) + 2:
                    u0 = _after(u[TB - 8:TB, FC - 128:FC], functools.reduce(_or, links[fc - 2]) & zvec)
                    u = jnp.concatenate([u[0:TB - 8, :], jnp.concatenate([u[TB - 8:TB, 0:FC - 128], u0], axis=1)], axis=0)
                hg = 0.5 * g
                act = (hg * (1.0 + jnp.tanh(hg)) * u).astype(bf16)
                if fc < len(side):
                    gates = _groups(g) + _groups(u)
                    n = len(side[fc])
                    links.append([fn(_bits(gates[G0 + (k * GN) // n][TB - 16:TB - 8]) & zvec) for k, fn in enumerate(side[fc])])
            if fc >= 1:
                y = _dot(act_prev, w2_v[(fc - 1) * FC:fc * FC, :])
                acc = y if acc is None else acc + y
            act_prev = act
        for rb in range(TB // 8):
            xs = x1_rows(t0 + rb * 8)
            row = [xs[g] + mcol(5, g) * acc[rb * 8:(rb + 1) * 8, g * 128:(g + 1) * 128] for g in range(NG)]
            ob_v[slot, rb * 8:(rb + 1) * 8, :] = jnp.concatenate(row, axis=1).astype(bf16)
        out_copy(i, slot).start()
        return carry
    with scope("phase_b"):
        lax.fori_loop(0, NTB, phase_b, 0)
    out_copy(NTB - 2, 0).wait()
    out_copy(NTB - 1, 1).wait()


@jax.jit
def pallas_adaLN_cond__sliding_local_dilated__glu_gated_swiglu__prompt_kernel(
    A_x, A_wqkv, A_wo, B_x, B_w1, B_w3, B_w2, c, w_mod):
    del B_x
    any_spec = pl.BlockSpec(memory_space=pl.ANY)
    return pl.pallas_call(
        _kernel,
        out_shape=jax.ShapeDtypeStruct((1, S, D), bf16),
        in_specs=[any_spec] * 8,
        out_specs=any_spec,
        scratch_shapes=[
            pltpu.VMEM((S, D), bf16),
            pltpu.VMEM((1, D), bf16),
            pltpu.VMEM((16, D), bf16),
            pltpu.VMEM((NMOD, D, 128), bf16),
            pltpu.VMEM((D, 3 * D), bf16),
            pltpu.VMEM((NKC // 2, KC // 2, 3 * D), u32),
            pltpu.VMEM((NKC // 2, KC // 2, 3 * D), u32),
            pltpu.VMEM((D, D), bf16),
            pltpu.VMEM((D, F), bf16),
            pltpu.VMEM((D, F), bf16),
            pltpu.VMEM((F, D), bf16),
            pltpu.VMEM((2 * NG, 8, 128), f32),
            pltpu.VMEM((NMOD, 8, 128), f32),
            pltpu.VMEM((NG, M0, 128), f32),
            pltpu.VMEM((M0, KC), bf16),
            pltpu.VMEM((M0, KC), bf16),
            pltpu.VMEM((T, D), bf16),
            pltpu.VMEM((TB, D), bf16),
            pltpu.VMEM((T // 2, D), u32),
            pltpu.VMEM((M0 // 2, D), u32),
            pltpu.VMEM((2, 3 * NG, KROWS, 128), f32),
            pltpu.VMEM((3, 3 * NG, KROWS, 128), f32),
            pltpu.VMEM((NG, S + 8, 128), f32),
            pltpu.VMEM((2, TB, D), bf16),
            pltpu.VMEM((8, 128), u32),
            pltpu.SemaphoreType.DMA((6 + NKC + NT + NS,)),
            pltpu.SemaphoreType.DMA((3,)),
        ],
        compiler_params=pltpu.CompilerParams(vmem_limit_bytes=110 * 2**20, disable_bounds_checks=True,
                                             disable_semaphore_checks=True),
        name="adaln_fused",
    )(A_x, A_wqkv, A_wo, B_w1, B_w3, B_w2, c, w_mod)
```

```python
import functools
import jax
import jax.numpy as jnp
from jax import lax
import jax.experimental.pallas as pl
import jax.experimental.pallas.tpu as pltpu

S, D, F = 2048, 1024, 3584
KOFF0 = 24
H, DH, W, DIL = 32, 32, 8, 2
NG = D // 128
HALO = 16
T = 128
NT = S // T
NP = T // 16
SKEW = 3
M0 = SKEW * T
NS = NT - SKEW
TB = 128
NTB = S // TB
PPI = TB // 64
WROWS = KOFF0 + 16 * PPI
FC = 512
NFC = F // FC
KOFF = 24
KROWS = T + KOFF
LOG2E = 1.4426950408889634
QSCALE = (DH ** -0.5) * LOG2E
NEG = -1e9 * DH ** 0.5
KC = 128
NKC = D // KC
NMOD = 6 * NG
MPS = 3
MLAG = 2
EPS = 1e-5
G0, GN = 3, 5
WR = 3
MR = 2
UG = 4
f32, bf16, u32 = jnp.float32, jnp.bfloat16, jnp.uint32
scope = jax.named_scope


def _butterfly(vs):
    vs = list(vs)
    lane = lax.broadcasted_iota(jnp.int32, vs[0].shape, 1)
    for s in range(3):
        m = (lane & (4 << s)) != 0
        for g in range(NG):
            if g & (1 << s):
                continue
            a, b = vs[g], vs[g | (1 << s)]
            vs[g] = jnp.where(m, b, a)
            vs[g | (1 << s)] = jnp.where(m, a, b)
    return vs


def _to_head_lanes(vs):
    ys = _butterfly(vs)
    lane = lax.broadcasted_iota(jnp.int32, vs[0].shape, 1)
    head = lane & 31
    out = []
    for g in range(NG):
        src = ((head & 3) << 5) | (((head >> 2) ^ g) << 2) | (lane >> 5)
        out.append(jnp.take_along_axis(ys[g], src, axis=1))
    return out


def _from_head_lanes(zs):
    lane = lax.broadcasted_iota(jnp.int32, zs[0].shape, 1)
    ys = []
    for g in range(NG):
        src = ((lane & 3) << 5) | ((((lane >> 2) & 7) ^ g) << 2) | (lane >> 5)
        ys.append(jnp.take_along_axis(zs[g], src, axis=1))
    return _butterfly(ys)


def _add(a, b):
    return a + b


def _or(a, b):
    return a | b


def _bits(x):
    return pltpu.bitcast(x, u32)


def _dot(a, b):
    return jnp.dot(a, b, preferred_element_type=f32)


def _after(x, dep):
    if dep is None:
        return x
    return pltpu.bitcast(_bits(x) | dep, x.dtype)


def _norm8(xs, dep=None):
    xs = [_after(xs[0], dep)] + list(xs[1:])
    m = jnp.sum(functools.reduce(_add, xs), axis=-1, keepdims=True) * (1.0 / D)
    xc = [v - m for v in xs]
    var = jnp.sum(functools.reduce(_add, [v * v for v in xc]), axis=-1, keepdims=True) * (1.0 / D)
    r = lax.rsqrt(var + EPS)
    return [v * r for v in xc]


def _groups(x):
    return [x[:, g * 128:(g + 1) * 128] for g in range(x.shape[1] // 128)]


def _kernel(x_hbm, wqkv_hbm, wo_hbm, w1_hbm, w3_hbm, w2_hbm, c_hbm, wmod_hbm, out_hbm,
            x_v, c_v, sc_v, wm_v, wraw_v, wpe_v, wpo_v, wo_v, w1_v, w3_v, w2_v, mod_v, modr_v,
            xn_v, he_v, ho_v, h_v, h2_v, x1_v, win_v, st_v, o_v, p0_v, p1_v, a_v, ob_v,
            zv_v, sem, osem):
    names = ["c", "x0", "wo", "w1", "w3", "w2"]
    srcdst = dict(
        c=(c_hbm, c_v),
        x0=(x_hbm.at[0, 0:M0, :], x_v.at[0:M0, :]),
        wo=(wo_hbm, wo_v),
        w1=(w1_hbm, w1_v), w3=(w3_hbm, w3_v), w2=(w2_hbm, w2_v),
    )
    copies = {n: pltpu.make_async_copy(srcdst[n][0], srcdst[n][1], sem.at[i]) for i, n in enumerate(names)}
    SEM_C = len(names)
    SEM_W = SEM_C + NKC
    SEM_X = SEM_W + NKC
    SEM_M = SEM_X + NT

    def slab_copy(j, s):
        return pltpu.make_async_copy(wmod_hbm.at[:, pl.ds(pl.multiple_of(j * 128, 128), 128)], wm_v.at[j], sem.at[s])

    def chunk_copies(c):
        rows = pl.ds(pl.multiple_of(c * KC, KC), KC)
        return [slab_copy(c, SEM_C + c), slab_copy(NG + c, SEM_C + c),
                pltpu.make_async_copy(wqkv_hbm.at[rows, :], wraw_v.at[rows, :], sem.at[SEM_W + c])]

    def x_copy(t):
        rows = pl.ds(pl.multiple_of(t * T, T), T)
        return pltpu.make_async_copy(x_hbm.at[0, rows, :], x_v.at[rows, :], sem.at[SEM_X + t])

    copies["c"].start()
    copies["x0"].start()
    for c in range(NKC):
        for cp in chunk_copies(c):
            cp.start()
    x_copy(SKEW).start()
    x_copy(SKEW + 1).start()
    copies["wo"].start()
    for t in range(SKEW + 2, NT):
        x_copy(t).start()
    for j in range(2 * NG, NMOD):
        slab_copy(j, SEM_M + (j - 2 * NG) // MPS).start()
    for n in ("w1", "w3", "w2"):
        copies[n].start()
    zv_v[...] = jnp.zeros(zv_v.shape, u32)

    proj = (p0_v, p1_v)
    mcol = lambda sec, g: (mod_v if sec < 2 else modr_v)[sec * NG + g]
    row8 = lax.broadcasted_iota(jnp.int32, (8, 128), 0)

    def mod_round(j, kh):
        ks = slice(kh * 512, (kh + 1) * 512)
        return _dot(sc_v[:, ks], wm_v[j, ks, :])[0:8]

    def ln1_rows(row, drow, dep):
        xn = _norm8(_groups(x_v[pl.ds(row, 8), :].astype(f32)), dep)
        ys = [xn[g] * mcol(1, g) + mcol(0, g) for g in range(NG)]
        h_v[drow:drow + 8, :] = jnp.concatenate(ys, axis=1).astype(bf16)
        return _bits(ys[NG - 1])

    def ln2_rows(row, drow, dep):
        x = _groups(x_v[pl.ds(row, 8), :].astype(f32))
        x1 = [x[g] + mcol(2, g) * a_v[g, pl.ds(row, 8), :] for g in range(NG)]
        x1_v[drow:drow + 8, :] = jnp.concatenate(x1, axis=1)
        xn = _norm8(x1, dep)
        ys = [xn[g] * mcol(4, g) + mcol(3, g) for g in range(NG)]
        h2_v[drow:drow + 8, :] = jnp.concatenate(ys, axis=1).astype(bf16)
        return _bits(ys[NG - 1])

    def attn8(src, t0, pb, par, dep):
        r0 = KOFF + 16 * pb + par
        rows = lambda j: pl.ds(r0 - DIL * j, 8, stride=DIL)
        s = [None] * W
        for g in range(NG):
            q = src[g, rows(0), :]
            if g == 0:
                q = _after(q, dep)
            for j in range(W):
                p = q * src[NG + g, rows(j), :]
                s[j] = p if s[j] is None else s[j] + p
        for j in range(W):
            s[j] = s[j] + pltpu.roll(s[j], 64, 1)
            s[j] = s[j] + pltpu.roll(s[j], 32, 1)
            if t0 is not None and pb == 0 and j > 0:
                s[j] = jnp.where(t0 + par + DIL * row8 >= DIL * j, s[j], NEG)
        m = functools.reduce(jnp.maximum, s)
        e = [jnp.exp2((s[j] - m) * QSCALE) for j in range(W)]
        den = functools.reduce(_add, e)
        r = pl.reciprocal(den, approx=True)
        inv = r * (2.0 - den * r)
        p = [e[j] * inv for j in range(W)]
        og = []
        for g in range(NG):
            acc = None
            for j in range(W):
                t = p[j] * src[2 * NG + g, rows(j), :]
                acc = t if acc is None else acc + t
            og.append(acc)
        return og

    def attn16(src, t0, pb, srow, dep):
        a = attn8(src, t0, pb, 0, dep)
        b = attn8(src, t0, pb, 1, dep)
        for g in range(NG):
            st_v[srow:srow + 8, g * 128:(g + 1) * 128] = _bits(jnp.concatenate([a[g], b[g]], axis=0).astype(bf16))
        return _bits(a[NG - 1]) | _bits(b[NG - 1])

    def unstage(r0, r1):
        return jnp.concatenate(_from_head_lanes(_groups(st_v[r0:r1, :])), axis=1)

    def out_proj(o, t0):
        a = _dot(o, wo_v[...])
        for g in range(NG):
            for rb in range(a.shape[0] // 8):
                a_v[g, pl.ds(t0 + (rb // 2) * 16 + rb % 2, 8, stride=2), :] = a[rb * 8:(rb + 1) * 8, g * 128:(g + 1) * 128]

    def chunk_block(c, par, do_prep, do_mm, extra=None):
        zvec = zv_v[...]
        links = {}

        def link(ct, v):
            links[ct] = (links[ct] | v) if ct in links else v

        def rounds(hc, wp, rs, between=None):
            res = {}
            for k, r in enumerate(rs):
                out = _groups(_dot(hc, pltpu.bitcast(wp[:, r * 512:(r + 1) * 512], bf16)))
                for n in range(4):
                    res[4 * r + n] = out[n]
                if between is not None:
                    between(k)
            return res

        def accumulate(res):
            for ct in res:
                for t in range(SKEW):
                    blk = res[ct][t * T:(t + 1) * T]
                    if t == SKEW - 1 and ct in links:
                        blk = jnp.concatenate([blk[0:T - 8], _after(blk[T - 8:T], links.pop(ct) & zvec)], axis=0)
                    proj[t % 2][t // 2, ct, KOFF:KOFF + T, :] += blk
        mr = []

        def mods(k):
            todo = range(len(mr), 4) if k is None else range(len(mr), min(4, (4 * (k + 1)) // MR))
            for r in todo:
                mr.append(mod_round(c + NG * (r // 2), r % 2))
        if do_prep:
            for cp in chunk_copies(c):
                cp.wait()
        if do_mm:
            res = rounds((he_v, ho_v)[1 - par][...], (wpe_v, wpo_v)[1 - par].at[(c - 1) >> 1], range(WR, 6),
                         mods if do_prep else None)
        if do_prep:
            mods(None)
            sh = mr[0] + mr[1]
            s1 = mr[2] + mr[3] + 1.0
            mod_v[c] = sh
            mod_v[NG + c] = s1
            hc = (xn_v[c].reshape(M0 // 8, 8, 128) * s1 + sh).reshape(M0, 128).astype(bf16)
            (he_v, ho_v)[par][...] = hc
            wp = (wpe_v, wpo_v)[par].at[c >> 1]
            for b in range(6):
                sec, half = b // 2, b % 2
                r0 = pl.multiple_of(c * KC + half * 64, 64)
                vs = _groups(_bits(wraw_v[pl.ds(r0, 64), sec * D:(sec + 1) * D]))
                vs = _to_head_lanes(vs)
                wp[half * 32:(half + 1) * 32, sec * D:(sec + 1) * D] = jnp.concatenate(vs, axis=1)
                if 2 * sec + 2 > WR:
                    link(4 * WR - 2 + half - 2 * (2 - sec), vs[NG - 1][24:32])
        if extra is not None:
            extra(res, link, zvec)
        if do_mm:
            accumulate(res)
        if do_prep:
            accumulate(rounds(hc, wp, range(WR)))

    with scope("p_first"):
        def zero(ct, carry):
            for t in range(SKEW):
                proj[t % 2][t // 2, ct, KOFF:KOFF + T, :] = jnp.zeros((T, 128), f32)
            return carry
        lax.fori_loop(0, 3 * NG, zero, 0)
        copies["c"].wait()
        c32 = c_v[...].astype(f32)
        sc_v[...] = jnp.broadcast_to((c32 * jax.nn.sigmoid(c32)).astype(bf16), (16, D))
        copies["x0"].wait()

        def stats(i, carry):
            for rb in range(12):
                rows = pl.ds(pl.multiple_of(i * 96, 32) + rb * 8, 8)
                xn = _norm8(_groups(x_v[rows, :].astype(f32)))
                for g in range(NG):
                    xn_v[g, rows, :] = xn[g]
            return carry
        lax.fori_loop(0, M0 // 96, stats, 0)
        chunk_block(0, 0, True, False)

    def kloop(i, carry):
        chunk_block(2 * i + 1, 1, True, True)

        @pl.when(2 * i + 2 < NKC)
        def _():
            chunk_block(2 * i + 2, 0, True, True)
        return carry
    with scope("p_kloop"):
        lax.fori_loop(0, NKC // 2, kloop, 0)

    with scope("p_last"):
        x_copy(SKEW).wait()

        def ln_next(res, link, zvec):
            for rb in range(T // 8):
                ct = 4 * WR + (rb * (20 - 4 * WR)) // (T // 8)
                link(ct + 3, ln1_rows(M0 + rb * 8, rb * 8, _bits(res[ct][M0 - 8:M0]) & zvec))
        chunk_block(NKC, 0, False, True, ln_next)
        for t in range(SKEW):
            for sg in range(NG, 3 * NG):
                if t == 0:
                    halo = jnp.broadcast_to(p0_v[0, sg, KOFF:KOFF + 1, :], (HALO, 128))
                else:
                    halo = proj[(t - 1) % 2][(t - 1) // 2, sg, KOFF + T - HALO:KOFF + T, :]
                proj[t % 2][t // 2, sg, KOFF - HALO:KOFF, :] = halo
        copies["wo"].wait()

    def step(s, par):
        @pl.when(s + SKEW + 1 < NT)
        def _():
            x_copy(s + SKEW + 1).wait()
        jn = 2 * NG + MPS * (s - MLAG)
        for k in range(MPS):
            @pl.when((s >= MLAG) & (jn + k < NMOD))
            def _():
                slab_copy(jn + k, SEM_M + s - MLAG).wait()
        j0 = jnp.where(s >= MLAG, jnp.minimum(jn, NMOD - MPS), 0)
        zvec = zv_v[...]
        t0 = pl.multiple_of(s * T, T)
        slot = (s >> 1) & 1
        dst = proj[1 - par].at[((s + SKEW) >> 1) & 1]
        prev = proj[par].at[1 - slot]
        h = h_v[...]
        tiles, mr = [], []
        for r in range(8):
            cols = slice(r * 384, (r + 1) * 384)
            w = jnp.concatenate([(wpe_v, wpo_v)[c % 2][c // 2, :, cols] for c in range(NKC)], axis=0)
            tiles += _groups(_dot(h, pltpu.bitcast(w, bf16)))
            if r < 2 * MPS:
                mr.append(mod_round(j0 + r // 2, r % 2))
        for k in range(MPS):
            one = jnp.where((j0 + k) >> 3 == 4, 1.0, 0.0)
            modr_v[j0 + k] = mr[2 * k] + mr[2 * k + 1] + one
        for ct in range(3 * NG):
            dst[ct, KOFF:KOFF + T, :] = tiles[ct]
            if ct >= NG:
                dst[ct, KOFF - HALO:KOFF, :] = prev[ct, KOFF + T - HALO:KOFF + T, :]
        t1 = pl.multiple_of(jnp.minimum(s + SKEW + 1, NT - 1) * T, T)
        src = proj[par].at[slot]
        links, rows = [], []
        for pb in range(NP):
            gate = _bits(tiles[(20 * pb) // NP][T - 8:T, :]) & zvec
            d = gate if pb < 2 else gate | ((links[2 * pb - 4] | links[2 * pb - 3]) & zvec)
            attn16(src, t0 if par == 0 else None, pb, pb * 8, d)
            for rb in (2 * pb, 2 * pb + 1):
                links.append(ln1_rows(t1 + rb * 8, rb * 8, gate))
            if (pb + 1) % UG == 0:
                rows.append(pltpu.bitcast(unstage((pb + 1 - UG) * 8, (pb + 1) * 8), bf16))
        out_proj(jnp.concatenate(rows, axis=0), t0)

    def phase_a(i, carry):
        step(2 * i, 0)

        @pl.when(2 * i + 1 < NS)
        def _():
            step(2 * i + 1, 1)
        return carry
    with scope("phase_a"):
        lax.fori_loop(0, (NS + 1) // 2, phase_a, 0)

    IPT = NP // PPI

    def fill_window(i, sgs, dep):
        src = p1_v.at[(i // IPT) % 3, :, pl.ds(pl.multiple_of((i % IPT) * 16 * PPI, 16 * PPI), WROWS), :]
        for sg in sgs:
            lo = KOFF if sg < NG else KOFF - HALO
            v = src[sg, lo:WROWS, :]
            if dep is not None:
                v = jnp.concatenate([_after(v[0:8], dep), v[8:]], axis=0)
            win_v[sg, lo:WROWS, :] = v
        return _bits(v[0:8])

    with scope("mid"):
        for sg in range(3 * NG):
            lo = KOFF if sg < NG else KOFF - HALO
            p1_v[2, sg, lo:KROWS, :] = p0_v[1, sg, lo:KROWS, :]
        fill_window(0, range(3 * NG), None)
        for rb in range(TB // 8):
            ln2_rows(rb * 8, rb * 8, None)
        copies["w1"].wait()
        copies["w3"].wait()
        copies["w2"].wait()

    def out_copy(i, slot):
        return pltpu.make_async_copy(ob_v.at[slot], out_hbm.at[0, pl.ds(pl.multiple_of(i * TB, TB), TB), :], osem.at[slot])

    def phase_b(i, carry):
        t1 = pl.multiple_of(jnp.minimum(i + 1, NTB - 1) * TB, TB)
        slot = i & 1

        def late_proj(t, carry):
            rows = pl.ds(pl.multiple_of(t * (T // 2), T // 2), T // 2)
            out_proj(pltpu.bitcast(o_v[rows, :], bf16), pl.multiple_of((NS + t) * T, T))
            return carry
        if TB == T:
            @pl.when(i == SKEW * IPT)
            def _():
                out_proj(pltpu.bitcast(o_v[...], bf16), NS * T)
        else:
            lax.fori_loop(jnp.where(i == NTB - 2, 1, 0), jnp.where(i == NTB - 3, 1, jnp.where(i == NTB - 2, SKEW, 0)),
                          late_proj, 0)

        @pl.when(i >= 2)
        def _():
            out_copy(i - 2, slot).wait()
        zvec = zv_v[...]
        sl = (i // IPT) % 3
        orow = jnp.where(sl == 0, 0, jnp.where(sl == 1, T, T // 2)) + (i % IPT) * 8 * PPI

        def fin(dep):
            o = unstage(0, 8 * PPI)
            o_v[pl.ds(pl.multiple_of(orow, 8 * PPI), 8 * PPI), :] = o
            return o[8 * PPI - 8:8 * PPI, D - 128:D]
        NRB = TB // 8
        side = [[] for _ in range(NFC - 1)]
        for k in range(PPI):
            side[(k * 2) // PPI].append(lambda d, k=k: attn16(win_v, None, k, 8 * k, d))
        side[2].append(fin)
        for r in range(NRB):
            side[2 + (r * 4) // NRB].append(lambda d, r=r: ln2_rows(t1 + r * 8, r * 8, d))
        for k in range(4):
            side[3 + k // 2].append(lambda d, k=k: fill_window(i + 1, range(6 * k, 6 * k + 6), d))
        h = h2_v[...]
        gb = jnp.concatenate([mcol(5, g) for g in range(NG)], axis=1)
        scaled = lambda y: (y.reshape(NRB, 8, D) * gb).reshape(TB, D)
        acc = act_prev = None
        links = []
        for fc in range(NFC + 1):
            if fc < NFC:
                g = _dot(h, w1_v[:, fc * FC:(fc + 1) * FC])
                u = _dot(h, w3_v[:, fc * FC:(fc + 1) * FC])
                if fc >= 1:
                    u0 = _after(u[TB - 8:TB, FC - 128:FC], functools.reduce(_or, links[fc - 1]) & zvec)
                    u = jnp.concatenate([u[0:TB - 8, :], jnp.concatenate([u[TB - 8:TB, 0:FC - 128], u0], axis=1)], axis=0)
                hg = 0.5 * g
                act = (hg * (1.0 + jnp.tanh(hg)) * u).astype(bf16)
                if fc < len(side):
                    gates = _groups(g) + _groups(u)
                    n = len(side[fc])
                    links.append([fn(_bits(gates[G0 + (k * GN) // n][TB - 16:TB - 8]) & zvec) for k, fn in enumerate(side[fc])])
            if fc >= 1:
                y = scaled(_dot(act_prev, w2_v[(fc - 1) * FC:fc * FC, :]))
                acc = (x1_v[...] if acc is None else acc) + y
            act_prev = act
        ob_v[slot] = acc.astype(bf16)
        out_copy(i, slot).start()
        return carry
    with scope("phase_b"):
        lax.fori_loop(0, NTB, phase_b, 0)
    out_copy(NTB - 2, 0).wait()
    out_copy(NTB - 1, 1).wait()


@jax.jit
def pallas_adaLN_cond__sliding_local_dilated__glu_gated_swiglu__prompt_kernel(
    A_x, A_wqkv, A_wo, B_x, B_w1, B_w3, B_w2, c, w_mod):
    del B_x
    any_spec = pl.BlockSpec(memory_space=pl.ANY)
    return pl.pallas_call(
        _kernel,
        out_shape=jax.ShapeDtypeStruct((1, S, D), bf16),
        in_specs=[any_spec] * 8,
        out_specs=any_spec,
        scratch_shapes=[
            pltpu.VMEM((S, D), bf16),
            pltpu.VMEM((1, D), bf16),
            pltpu.VMEM((16, D), bf16),
            pltpu.VMEM((NMOD, D, 128), bf16),
            pltpu.VMEM((D, 3 * D), bf16),
            pltpu.VMEM((NKC // 2, KC // 2, 3 * D), u32),
            pltpu.VMEM((NKC // 2, KC // 2, 3 * D), u32),
            pltpu.VMEM((D, D), bf16),
            pltpu.VMEM((D, F), bf16),
            pltpu.VMEM((D, F), bf16),
            pltpu.VMEM((F, D), bf16),
            pltpu.VMEM((2 * NG, 8, 128), f32),
            pltpu.VMEM((NMOD, 8, 128), f32),
            pltpu.VMEM((NG, M0, 128), f32),
            pltpu.VMEM((M0, KC), bf16),
            pltpu.VMEM((M0, KC), bf16),
            pltpu.VMEM((T, D), bf16),
            pltpu.VMEM((TB, D), bf16),
            pltpu.VMEM((TB, D), f32),
            pltpu.VMEM((3 * NG, WROWS, 128), f32),
            pltpu.VMEM((T // 2, D), u32),
            pltpu.VMEM((M0 // 2, D), u32),
            pltpu.VMEM((2, 3 * NG, KROWS, 128), f32),
            pltpu.VMEM((3, 3 * NG, KROWS, 128), f32),
            pltpu.VMEM((NG, S + 8, 128), f32),
            pltpu.VMEM((2, TB, D), bf16),
            pltpu.VMEM((8, 128), u32),
            pltpu.SemaphoreType.DMA((6 + 2 * NKC + NT + NS,)),
            pltpu.SemaphoreType.DMA((2,)),
        ],
        compiler_params=pltpu.CompilerParams(vmem_limit_bytes=110 * 2**20, disable_bounds_checks=True,
                                             disable_semaphore_checks=True),
        name="adaln_fused",
    )(A_x, A_wqkv, A_wo, B_w1, B_w3, B_w2, c, w_mod)
```

```python
import functools
import jax
import jax.numpy as jnp
from jax import lax
import jax.experimental.pallas as pl
import jax.experimental.pallas.tpu as pltpu

S, D, F = 2048, 1024, 3584
KOFF0 = 24
H, DH, W, DIL = 32, 32, 8, 2
NG = D // 128
HALO = 16
T = 128
NT = S // T
NP = T // 16
SKEW = 3
M0 = SKEW * T
NS = NT - SKEW
TB = 128
NTB = S // TB
PPI = TB // 64
WROWS = KOFF0 + 16 * PPI
FC = 512
NFC = F // FC
KOFF = 24
KROWS = T + KOFF
LOG2E = 1.4426950408889634
QSCALE = (DH ** -0.5) * LOG2E
NEG = -1e9 * DH ** 0.5
KC = 128
NKC = D // KC
NMOD = 6 * NG
MPS = 3
MLAG = 2
EPS = 1e-5
G0, GN = 3, 5
PAD = "wp,wo,w2,h,w1"
padw = lambda k: 128 if k in PAD.split(",") else 0
WR = 3
MR = 2
UG = 4
f32, bf16, u32 = jnp.float32, jnp.bfloat16, jnp.uint32
scope = jax.named_scope


def _butterfly(vs):
    vs = list(vs)
    lane = lax.broadcasted_iota(jnp.int32, vs[0].shape, 1)
    for s in range(3):
        m = (lane & (4 << s)) != 0
        for g in range(NG):
            if g & (1 << s):
                continue
            a, b = vs[g], vs[g | (1 << s)]
            vs[g] = jnp.where(m, b, a)
            vs[g | (1 << s)] = jnp.where(m, a, b)
    return vs


def _to_head_lanes(vs):
    ys = _butterfly(vs)
    lane = lax.broadcasted_iota(jnp.int32, vs[0].shape, 1)
    head = lane & 31
    out = []
    for g in range(NG):
        src = ((head & 3) << 5) | (((head >> 2) ^ g) << 2) | (lane >> 5)
        out.append(jnp.take_along_axis(ys[g], src, axis=1))
    return out


def _from_head_lanes(zs):
    lane = lax.broadcasted_iota(jnp.int32, zs[0].shape, 1)
    ys = []
    for g in range(NG):
        src = ((lane & 3) << 5) | ((((lane >> 2) & 7) ^ g) << 2) | (lane >> 5)
        ys.append(jnp.take_along_axis(zs[g], src, axis=1))
    return _butterfly(ys)


def _add(a, b):
    return a + b


def _or(a, b):
    return a | b


def _bits(x):
    return pltpu.bitcast(x, u32)


def _dot(a, b):
    return jnp.dot(a, b, preferred_element_type=f32)


def _after(x, dep):
    if dep is None:
        return x
    return pltpu.bitcast(_bits(x) | dep, x.dtype)


def _norm8(xs, dep=None):
    xs = [_after(xs[0], dep)] + list(xs[1:])
    m = jnp.sum(functools.reduce(_add, xs), axis=-1, keepdims=True) * (1.0 / D)
    xc = [v - m for v in xs]
    var = jnp.sum(functools.reduce(_add, [v * v for v in xc]), axis=-1, keepdims=True) * (1.0 / D)
    r = lax.rsqrt(var + EPS)
    return [v * r for v in xc]


def _groups(x):
    return [x[:, g * 128:(g + 1) * 128] for g in range(x.shape[1] // 128)]


def _kernel(x_hbm, wqkv_hbm, wo_hbm, w1_hbm, w3_hbm, w2_hbm, c_hbm, wmod_hbm, out_hbm,
            x_v, c_v, sc_v, cb_v, wm_v, wraw_v, wpe_v, wpo_v, wo_v, w1_v, w3_v, w2_v, mod_v, modr_v,
            xn_v, he_v, ho_v, h_v, h2_v, x1_v, win_v, st_v, o_v, p0_v, p1_v, a_v, ob_v,
            zv_v, sem, osem):
    names = ["c", "x0", "wo", "w1", "w3", "w2"]
    srcdst = dict(
        c=(c_hbm, c_v),
        x0=(x_hbm.at[0, 0:M0, :], x_v.at[0:M0, :]),
        wo=(wo_hbm, wo_v.at[:, 0:D]),
        w1=(w1_hbm, w1_v.at[:, 0:F]), w3=(w3_hbm, w3_v.at[:, 0:F]), w2=(w2_hbm, w2_v.at[:, 0:D]),
    )
    copies = {n: pltpu.make_async_copy(srcdst[n][0], srcdst[n][1], sem.at[i]) for i, n in enumerate(names)}
    SEM_C = len(names)
    SEM_W = SEM_C + NKC
    SEM_X = SEM_W + NKC
    SEM_M = SEM_X + NT

    def slab_copy(j, s):
        return pltpu.make_async_copy(wmod_hbm.at[:, pl.ds(pl.multiple_of(j * 128, 128), 128)], wm_v.at[j], sem.at[s])

    def chunk_copies(c):
        rows = pl.ds(pl.multiple_of(c * KC, KC), KC)
        return [slab_copy(c, SEM_C + c), slab_copy(NG + c, SEM_C + c),
                pltpu.make_async_copy(wqkv_hbm.at[rows, :], wraw_v.at[rows, :], sem.at[SEM_W + c])]

    def x_copy(t):
        rows = pl.ds(pl.multiple_of(t * T, T), T)
        return pltpu.make_async_copy(x_hbm.at[0, rows, :], x_v.at[rows, :], sem.at[SEM_X + t])

    copies["c"].start()
    copies["x0"].start()
    for c in range(NKC):
        for cp in chunk_copies(c):
            cp.start()
    x_copy(SKEW).start()
    x_copy(SKEW + 1).start()
    copies["wo"].start()
    for t in range(SKEW + 2, NT):
        x_copy(t).start()
    for j in range(2 * NG, NMOD):
        slab_copy(j, SEM_M + (j - 2 * NG) // MPS).start()
    for n in ("w1", "w3", "w2"):
        copies[n].start()
    zv_v[...] = jnp.zeros(zv_v.shape, u32)

    proj = (p0_v, p1_v)
    mcol = lambda sec, g: (mod_v if sec < 2 else modr_v)[sec * NG + g]
    row8 = lax.broadcasted_iota(jnp.int32, (8, 128), 0)

    def mod_round(j, kh):
        ks = slice(kh * 512, (kh + 1) * 512)
        return _dot(sc_v[:, ks], wm_v[j, ks, :])[0:8]

    def ln1_rows(row, drow, dep):
        xn = _norm8(_groups(x_v[pl.ds(row, 8), :].astype(f32)), dep)
        ys = [xn[g] * mcol(1, g) + mcol(0, g) for g in range(NG)]
        h_v[drow:drow + 8, 0:D] = jnp.concatenate(ys, axis=1).astype(bf16)
        return _bits(ys[NG - 1])

    def ln2_rows(row, drow, dep):
        x = _groups(x_v[pl.ds(row, 8), :].astype(f32))
        x1 = [x[g] + mcol(2, g) * a_v[g, pl.ds(row, 8), :] for g in range(NG)]
        x1_v[drow:drow + 8, :] = jnp.concatenate(x1, axis=1)
        xn = _norm8(x1, dep)
        ys = [xn[g] * mcol(4, g) + mcol(3, g) for g in range(NG)]
        h2_v[drow:drow + 8, 0:D] = jnp.concatenate(ys, axis=1).astype(bf16)
        return _bits(ys[NG - 1])

    def attn8(src, t0, pb, par, dep):
        r0 = KOFF + 16 * pb + par
        rows = lambda j: pl.ds(r0 - DIL * j, 8, stride=DIL)
        s = [None] * W
        for g in range(NG):
            q = src[g, rows(0), :]
            if g == 0:
                q = _after(q, dep)
            for j in range(W):
                p = q * src[NG + g, rows(j), :]
                s[j] = p if s[j] is None else s[j] + p
        for j in range(W):
            s[j] = s[j] + pltpu.roll(s[j], 64, 1)
            s[j] = s[j] + pltpu.roll(s[j], 32, 1)
            if t0 is not None and pb == 0 and j > 0:
                s[j] = jnp.where(t0 + par + DIL * row8 >= DIL * j, s[j], NEG)
        m = functools.reduce(jnp.maximum, s)
        e = [jnp.exp2((s[j] - m) * QSCALE) for j in range(W)]
        den = functools.reduce(_add, e)
        r = pl.reciprocal(den, approx=True)
        inv = r * (2.0 - den * r)
        p = [e[j] * inv for j in range(W)]
        og = []
        for g in range(NG):
            acc = None
            for j in range(W):
                t = p[j] * src[2 * NG + g, rows(j), :]
                acc = t if acc is None else acc + t
            og.append(acc)
        return og

    def attn16(src, t0, pb, srow, dep):
        a = attn8(src, t0, pb, 0, dep)
        b = attn8(src, t0, pb, 1, dep)
        for g in range(NG):
            st_v[srow:srow + 8, g * 128:(g + 1) * 128] = _bits(jnp.concatenate([a[g], b[g]], axis=0).astype(bf16))
        return _bits(a[NG - 1]) | _bits(b[NG - 1])

    def unstage(r0, r1):
        return jnp.concatenate(_from_head_lanes(_groups(st_v[r0:r1, :])), axis=1)

    def out_proj(o, t0, side=None):
        a = _groups(_dot(o, wo_v[:, 0:D]))
        links = side(a) if side is not None else {}
        for g in range(NG):
            for rb in range(a[g].shape[0] // 8):
                v = a[g][rb * 8:(rb + 1) * 8]
                if rb == 0 and g in links:
                    v = _after(v, links[g])
                a_v[g, pl.ds(t0 + (rb // 2) * 16 + rb % 2, 8, stride=2), :] = v

    def mod_vpu(j, part, nparts, dep):
        n = D // nparts
        acc = [None] * 4
        for i in range(n // 8):
            rows = slice(part * n + i * 8, part * n + (i + 1) * 8)
            cb = cb_v[rows, :]
            if i == 0:
                cb = _after(cb, dep)
            t = wm_v[j, rows, :].astype(f32) * cb
            acc[i % 4] = t if acc[i % 4] is None else acc[i % 4] + t
        return (acc[0] + acc[1]) + (acc[2] + acc[3])

    def chunk_block(c, par, do_prep, do_mm, extra=None):
        zvec = zv_v[...]
        links = {}

        def link(ct, v):
            links[ct] = (links[ct] | v) if ct in links else v

        def rounds(hc, wp, rs, between=None):
            res = {}
            for k, r in enumerate(rs):
                out = _groups(_dot(hc, pltpu.bitcast(wp[:, r * 512:(r + 1) * 512], bf16)))
                for n in range(4):
                    res[4 * r + n] = out[n]
                if between is not None:
                    between(k)
            return res

        def accumulate(res):
            for ct in res:
                for t in range(SKEW):
                    blk = res[ct][t * T:(t + 1) * T]
                    if t == SKEW - 1 and ct in links:
                        blk = jnp.concatenate([blk[0:T - 8], _after(blk[T - 8:T], links.pop(ct) & zvec)], axis=0)
                    proj[t % 2][t // 2, ct, KOFF:KOFF + T, :] += blk
        mr = []

        def mods(k):
            todo = range(len(mr), 4) if k is None else range(len(mr), min(4, (4 * (k + 1)) // MR))
            for r in todo:
                mr.append(mod_round(c + NG * (r // 2), r % 2))
        if do_prep:
            for cp in chunk_copies(c):
                cp.wait()
        if do_mm:
            res = rounds((he_v, ho_v)[1 - par][...], (wpe_v, wpo_v)[1 - par].at[(c - 1) >> 1], range(WR, 6),
                         mods if do_prep else None)
        if do_prep:
            mods(None)
            sh = mr[0] + mr[1]
            s1 = mr[2] + mr[3] + 1.0
            mod_v[c] = sh
            mod_v[NG + c] = s1
            hc = (xn_v[c].reshape(M0 // 8, 8, 128) * s1 + sh).reshape(M0, 128).astype(bf16)
            (he_v, ho_v)[par][...] = hc
            wp = (wpe_v, wpo_v)[par].at[c >> 1]
            for b in range(6):
                sec, half = b // 2, b % 2
                r0 = pl.multiple_of(c * KC + half * 64, 64)
                vs = _groups(_bits(wraw_v[pl.ds(r0, 64), sec * D:(sec + 1) * D]))
                vs = _to_head_lanes(vs)
                wp[half * 32:(half + 1) * 32, sec * D:(sec + 1) * D] = jnp.concatenate(vs, axis=1)
                if 2 * sec + 2 > WR:
                    link(4 * WR - 2 + half - 2 * (2 - sec), vs[NG - 1][24:32])
        if extra is not None:
            extra(res, link, zvec)
        if do_mm:
            accumulate(res)
        if do_prep:
            accumulate(rounds(hc, wp, range(WR)))

    with scope("p_first"):
        def zero(ct, carry):
            for t in range(SKEW):
                proj[t % 2][t // 2, ct, KOFF:KOFF + T, :] = jnp.zeros((T, 128), f32)
            return carry
        lax.fori_loop(0, 3 * NG, zero, 0)
        copies["c"].wait()
        c32 = c_v[...].astype(f32)
        sc = (c32 * jax.nn.sigmoid(c32)).astype(bf16)
        sc_v[...] = jnp.broadcast_to(sc, (16, D))
        diag = lax.broadcasted_iota(jnp.int32, (128, 128), 0) == lax.broadcasted_iota(jnp.int32, (128, 128), 1)
        for g, row in enumerate(_groups(sc.astype(f32))):
            col = jnp.sum(jnp.where(diag, row, 0.0), axis=1, keepdims=True)
            cb_v[g * 128:(g + 1) * 128, :] = jnp.broadcast_to(col, (128, 128))
        copies["x0"].wait()

        def stats(i, carry):
            for rb in range(12):
                rows = pl.ds(pl.multiple_of(i * 96, 32) + rb * 8, 8)
                xn = _norm8(_groups(x_v[rows, :].astype(f32)))
                for g in range(NG):
                    xn_v[g, rows, :] = xn[g]
            return carry
        lax.fori_loop(0, M0 // 96, stats, 0)
        chunk_block(0, 0, True, False)

    def kloop(i, carry):
        chunk_block(2 * i + 1, 1, True, True)

        @pl.when(2 * i + 2 < NKC)
        def _():
            chunk_block(2 * i + 2, 0, True, True)
        return carry
    with scope("p_kloop"):
        lax.fori_loop(0, NKC // 2, kloop, 0)

    with scope("p_last"):
        x_copy(SKEW).wait()

        def ln_next(res, link, zvec):
            for rb in range(T // 8):
                ct = 4 * WR + (rb * (20 - 4 * WR)) // (T // 8)
                link(ct + 3, ln1_rows(M0 + rb * 8, rb * 8, _bits(res[ct][M0 - 8:M0]) & zvec))
        chunk_block(NKC, 0, False, True, ln_next)
        for t in range(SKEW):
            for sg in range(NG, 3 * NG):
                if t == 0:
                    halo = jnp.broadcast_to(p0_v[0, sg, KOFF:KOFF + 1, :], (HALO, 128))
                else:
                    halo = proj[(t - 1) % 2][(t - 1) // 2, sg, KOFF + T - HALO:KOFF + T, :]
                proj[t % 2][t // 2, sg, KOFF - HALO:KOFF, :] = halo
        copies["wo"].wait()

    def step(s, par):
        @pl.when(s + SKEW + 1 < NT)
        def _():
            x_copy(s + SKEW + 1).wait()
        jn = 2 * NG + MPS * (s - MLAG)
        for k in range(MPS):
            @pl.when((s >= MLAG) & (jn + k < NMOD))
            def _():
                slab_copy(jn + k, SEM_M + s - MLAG).wait()
        j0 = jnp.where(s >= MLAG, jnp.minimum(jn, NMOD - MPS), 0)
        zvec = zv_v[...]
        t0 = pl.multiple_of(s * T, T)
        slot = (s >> 1) & 1
        dst = proj[1 - par].at[((s + SKEW) >> 1) & 1]
        prev = proj[par].at[1 - slot]
        w = jnp.concatenate([(wpe_v, wpo_v)[c % 2][c // 2, :, 0:3 * D] for c in range(NKC)], axis=0)
        tiles = _groups(_dot(h_v[:, 0:D], pltpu.bitcast(w, bf16)))
        for ct in range(3 * NG):
            dst[ct, KOFF:KOFF + T, :] = tiles[ct]
            if ct >= NG:
                dst[ct, KOFF - HALO:KOFF, :] = prev[ct, KOFF + T - HALO:KOFF + T, :]
        t1 = pl.multiple_of(jnp.minimum(s + SKEW + 1, NT - 1) * T, T)
        src = proj[par].at[slot]
        links, rows = [], []
        for pb in range(NP):
            gate = _bits(tiles[(20 * pb) // NP][T - 8:T, :]) & zvec
            d = gate if pb < 2 else gate | ((links[2 * pb - 4] | links[2 * pb - 3]) & zvec)
            attn16(src, t0 if par == 0 else None, pb, pb * 8, d)
            for rb in (2 * pb, 2 * pb + 1):
                links.append(ln1_rows(t1 + rb * 8, rb * 8, gate))
            if (pb + 1) % UG == 0:
                rows.append(pltpu.bitcast(unstage((pb + 1 - UG) * 8, (pb + 1) * 8), bf16))

        def mods(a):
            links = {}
            for k in range(MPS):
                gates = [tiles[3 * NG - 1][T - 8:T] if 2 * k + h == 0 else a[2 * k + h - 1][T - 8:T] for h in range(2)]
                part = [mod_vpu(j0 + k, h, 2, _bits(gates[h]) & zvec) for h in range(2)]
                m = jnp.sum(part[0] + part[1], axis=0, keepdims=True) + jnp.where((j0 + k) >> 3 == 4, 1.0, 0.0)
                m = jnp.broadcast_to(m, (8, 128))
                modr_v[j0 + k] = m
                links[2 * k + 3] = _bits(m) & zvec
            return links
        out_proj(jnp.concatenate(rows, axis=0), t0, mods)

    def phase_a(i, carry):
        step(2 * i, 0)

        @pl.when(2 * i + 1 < NS)
        def _():
            step(2 * i + 1, 1)
        return carry
    with scope("phase_a"):
        lax.fori_loop(0, (NS + 1) // 2, phase_a, 0)

    IPT = NP // PPI

    def fill_window(i, sgs, dep):
        src = p1_v.at[(i // IPT) % 3, :, pl.ds(pl.multiple_of((i % IPT) * 16 * PPI, 16 * PPI), WROWS), :]
        for sg in sgs:
            lo = KOFF if sg < NG else KOFF - HALO
            v = src[sg, lo:WROWS, :]
            if dep is not None:
                v = jnp.concatenate([_after(v[0:8], dep), v[8:]], axis=0)
            win_v[sg, lo:WROWS, :] = v
        return _bits(v[0:8])

    with scope("mid"):
        for sg in range(3 * NG):
            lo = KOFF if sg < NG else KOFF - HALO
            p1_v[2, sg, lo:KROWS, :] = p0_v[1, sg, lo:KROWS, :]
        fill_window(0, range(3 * NG), None)
        for rb in range(TB // 8):
            ln2_rows(rb * 8, rb * 8, None)
        copies["w1"].wait()
        copies["w3"].wait()
        copies["w2"].wait()

    def out_copy(i, slot):
        return pltpu.make_async_copy(ob_v.at[slot], out_hbm.at[0, pl.ds(pl.multiple_of(i * TB, TB), TB), :], osem.at[slot])

    def phase_b(i, carry):
        t1 = pl.multiple_of(jnp.minimum(i + 1, NTB - 1) * TB, TB)
        slot = i & 1

        def late_proj(t, carry):
            rows = pl.ds(pl.multiple_of(t * (T // 2), T // 2), T // 2)
            out_proj(pltpu.bitcast(o_v[rows, :], bf16), pl.multiple_of((NS + t) * T, T))
            return carry
        if TB == T:
            @pl.when(i == SKEW * IPT)
            def _():
                out_proj(pltpu.bitcast(o_v[...], bf16), NS * T)
        else:
            lax.fori_loop(jnp.where(i == NTB - 2, 1, 0), jnp.where(i == NTB - 3, 1, jnp.where(i == NTB - 2, SKEW, 0)),
                          late_proj, 0)

        @pl.when(i >= 2)
        def _():
            out_copy(i - 2, slot).wait()
        zvec = zv_v[...]
        sl = (i // IPT) % 3
        orow = jnp.where(sl == 0, 0, jnp.where(sl == 1, T, T // 2)) + (i % IPT) * 8 * PPI

        def fin(dep):
            o = unstage(0, 8 * PPI)
            o_v[pl.ds(pl.multiple_of(orow, 8 * PPI), 8 * PPI), :] = o
            return o[8 * PPI - 8:8 * PPI, D - 128:D]
        NRB = TB // 8
        side = [[] for _ in range(NFC - 1)]
        for k in range(PPI):
            side[(k * 2) // PPI].append(lambda d, k=k: attn16(win_v, None, k, 8 * k, d))
        side[2].append(fin)
        for r in range(NRB):
            side[2 + (r * 4) // NRB].append(lambda d, r=r: ln2_rows(t1 + r * 8, r * 8, d))
        for k in range(4):
            side[3 + k // 2].append(lambda d, k=k: fill_window(i + 1, range(6 * k, 6 * k + 6), d))
        h = h2_v[:, 0:D]
        gb = jnp.concatenate([mcol(5, g) for g in range(NG)], axis=1)
        scaled = lambda y: (y.reshape(NRB, 8, D) * gb).reshape(TB, D)
        acc = act_prev = None
        links = []
        for fc in range(NFC + 1):
            if fc < NFC:
                g = _dot(h, w1_v[:, fc * FC:(fc + 1) * FC])
                u = _dot(h, w3_v[:, fc * FC:(fc + 1) * FC])
                if fc >= 1:
                    u0 = _after(u[TB - 8:TB, FC - 128:FC], functools.reduce(_or, links[fc - 1]) & zvec)
                    u = jnp.concatenate([u[0:TB - 8, :], jnp.concatenate([u[TB - 8:TB, 0:FC - 128], u0], axis=1)], axis=0)
                hg = 0.5 * g
                act = (hg * (1.0 + jnp.tanh(hg)) * u).astype(bf16)
                if fc < len(side):
                    gates = _groups(g) + _groups(u)
                    n = len(side[fc])
                    links.append([fn(_bits(gates[G0 + (k * GN) // n][TB - 16:TB - 8]) & zvec) for k, fn in enumerate(side[fc])])
            if fc >= 1:
                y = scaled(_dot(act_prev, w2_v[(fc - 1) * FC:fc * FC, 0:D]))
                acc = (x1_v[...] if acc is None else acc) + y
            act_prev = act
        ob_v[slot] = acc.astype(bf16)
        out_copy(i, slot).start()
        return carry
    with scope("phase_b"):
        lax.fori_loop(0, NTB, phase_b, 0)
    out_copy(NTB - 2, 0).wait()
    out_copy(NTB - 1, 1).wait()


@jax.jit
def pallas_adaLN_cond__sliding_local_dilated__glu_gated_swiglu__prompt_kernel(
    A_x, A_wqkv, A_wo, B_x, B_w1, B_w3, B_w2, c, w_mod):
    del B_x
    any_spec = pl.BlockSpec(memory_space=pl.ANY)
    return pl.pallas_call(
        _kernel,
        out_shape=jax.ShapeDtypeStruct((1, S, D), bf16),
        in_specs=[any_spec] * 8,
        out_specs=any_spec,
        scratch_shapes=[
            pltpu.VMEM((S, D), bf16),
            pltpu.VMEM((1, D), bf16),
            pltpu.VMEM((16, D), bf16),
            pltpu.VMEM((D, 128), f32),
            pltpu.VMEM((NMOD, D, 128), bf16),
            pltpu.VMEM((D, 3 * D), bf16),
            pltpu.VMEM((NKC // 2, KC // 2, 3 * D + padw('wp')), u32),
            pltpu.VMEM((NKC // 2, KC // 2, 3 * D + padw('wp')), u32),
            pltpu.VMEM((D, D + padw('wo')), bf16),
            pltpu.VMEM((D, F + padw('w1')), bf16),
            pltpu.VMEM((D, F + padw('w1')), bf16),
            pltpu.VMEM((F, D + padw('w2')), bf16),
            pltpu.VMEM((2 * NG, 8, 128), f32),
            pltpu.VMEM((NMOD, 8, 128), f32),
            pltpu.VMEM((NG, M0, 128), f32),
            pltpu.VMEM((M0, KC), bf16),
            pltpu.VMEM((M0, KC), bf16),
            pltpu.VMEM((T, D + padw('h')), bf16),
            pltpu.VMEM((TB, D + padw('h')), bf16),
            pltpu.VMEM((TB, D), f32),
            pltpu.VMEM((3 * NG, WROWS, 128), f32),
            pltpu.VMEM((T // 2, D), u32),
            pltpu.VMEM((M0 // 2, D), u32),
            pltpu.VMEM((2, 3 * NG, KROWS, 128), f32),
            pltpu.VMEM((3, 3 * NG, KROWS, 128), f32),
            pltpu.VMEM((NG, S + 8, 128), f32),
            pltpu.VMEM((2, TB, D), bf16),
            pltpu.VMEM((8, 128), u32),
            pltpu.SemaphoreType.DMA((6 + 2 * NKC + NT + NS,)),
            pltpu.SemaphoreType.DMA((2,)),
        ],
        compiler_params=pltpu.CompilerParams(vmem_limit_bytes=110 * 2**20, disable_bounds_checks=True,
                                             disable_semaphore_checks=True),
        name="adaln_fused",
    )(A_x, A_wqkv, A_wo, B_w1, B_w3, B_w2, c, w_mod)
```

```python
import functools
import jax
import jax.numpy as jnp
from jax import lax
import jax.experimental.pallas as pl
import jax.experimental.pallas.tpu as pltpu

S, D, F = 2048, 1024, 3584
H, DH, W, DIL = 32, 32, 8, 2
NG = D // 128
HALO = 16
T = 128
NT = S // T
NP = T // 16
SKEW = 3
M0 = SKEW * T
NS = NT - SKEW
TB = 128
NTB = S // TB
PPI = TB // 64
WROWS = HALO + 16 * PPI
FC = 512
NFC = F // FC
KOFF = HALO
KROWS = KOFF + T + 8
LOG2E = 1.4426950408889634
QSCALE = (DH ** -0.5) * LOG2E
NEG = -1e9 * DH ** 0.5
KC = 128
NKC = D // KC
NMOD = 6 * NG
MPS = 4
MLAG = 3
EPS = 1e-5
G0, GN = 3, 5
GS = 22.0; GA = 0.0; STG = 1
CQ = 1; CP = 1
E0 = 3; EN = 5; PLAN = 0
PAD = "wp,wo,w2,h,w1"
padw = lambda k: 128 if k in PAD.split(",") else 0
WR = 3
MR = 2
UG = 4
f32, bf16, u32 = jnp.float32, jnp.bfloat16, jnp.uint32
scope = jax.named_scope


def _butterfly(vs):
    vs = list(vs)
    lane = lax.broadcasted_iota(jnp.int32, vs[0].shape, 1)
    for s in range(3):
        m = (lane & (4 << s)) != 0
        for g in range(NG):
            if g & (1 << s):
                continue
            a, b = vs[g], vs[g | (1 << s)]
            vs[g] = jnp.where(m, b, a)
            vs[g | (1 << s)] = jnp.where(m, a, b)
    return vs


def _to_head_lanes(vs):
    ys = _butterfly(vs)
    lane = lax.broadcasted_iota(jnp.int32, vs[0].shape, 1)
    head = lane & 31
    out = []
    for g in range(NG):
        src = ((head & 3) << 5) | (((head >> 2) ^ g) << 2) | (lane >> 5)
        out.append(jnp.take_along_axis(ys[g], src, axis=1))
    return out


def _from_head_lanes(zs):
    lane = lax.broadcasted_iota(jnp.int32, zs[0].shape, 1)
    ys = []
    for g in range(NG):
        src = ((lane & 3) << 5) | ((((lane >> 2) & 7) ^ g) << 2) | (lane >> 5)
        ys.append(jnp.take_along_axis(zs[g], src, axis=1))
    return _butterfly(ys)


def _add(a, b):
    return a + b


def _or(a, b):
    return a | b


def _bits(x):
    return pltpu.bitcast(x, u32)


def _dot(a, b):
    return jnp.dot(a, b, preferred_element_type=f32)


def _after(x, dep):
    if dep is None:
        return x
    return pltpu.bitcast(_bits(x) | dep, x.dtype)


def _norm8(xs, dep=None):
    xs = [_after(xs[0], dep)] + list(xs[1:])
    m = jnp.sum(functools.reduce(_add, xs), axis=-1, keepdims=True) * (1.0 / D)
    xc = [v - m for v in xs]
    var = jnp.sum(functools.reduce(_add, [v * v for v in xc]), axis=-1, keepdims=True) * (1.0 / D)
    r = lax.rsqrt(var + EPS)
    return [v * r for v in xc]


def _groups(x):
    return [x[:, g * 128:(g + 1) * 128] for g in range(x.shape[1] // 128)]


def _kernel(x_hbm, wqkv_hbm, wo_hbm, w1_hbm, w3_hbm, w2_hbm, c_hbm, wmod_hbm, out_hbm,
            x_v, c_v, sc_v, cb_v, wm_v, wraw_v, wpe_v, wpo_v, wo_v, w1_v, w3_v, w2_v, mod_v, modr_v,
            xn_v, he_v, ho_v, h_v, h2_v, x1_v, win_v, st_v, o_v, p0_v, p1_v, a_v, ob_v,
            zv_v, sem, osem):
    names = ["c", "x0", "x1", "x2", "xr", "wo", "w1", "w3", "w2", "wm"]
    srcdst = dict(
        c=(c_hbm, c_v),
        x0=(x_hbm.at[0, 0:M0, :], x_v.at[0:M0, :]),
        x1=(x_hbm.at[0, M0:M0 + T, :], x_v.at[M0:M0 + T, :]),
        x2=(x_hbm.at[0, M0 + T:M0 + 2 * T, :], x_v.at[M0 + T:M0 + 2 * T, :]),
        xr=(x_hbm.at[0, M0 + 2 * T:S, :], x_v.at[M0 + 2 * T:S, :]),
        wo=(wo_hbm, wo_v.at[:, 0:D]),
        wm=(wm_v.at[2 * NG:NMOD], wm_v.at[2 * NG:NMOD]),
        w1=(w1_hbm, w1_v.at[:, 0:F]), w3=(w3_hbm, w3_v.at[:, 0:F]), w2=(w2_hbm, w2_v.at[:, 0:D]),
    )
    copies = {n: pltpu.make_async_copy(srcdst[n][0], srcdst[n][1], sem.at[i]) for i, n in enumerate(names)}
    SEM_C = len(names)
    SEM_W = SEM_C + NKC

    def slab_copy(j, s):
        return pltpu.make_async_copy(wmod_hbm.at[:, pl.ds(pl.multiple_of(j * 128, 128), 128)], wm_v.at[j], sem.at[s])

    def chunk_copies(c):
        rows = pl.ds(pl.multiple_of(c * KC, KC), KC)
        return [slab_copy(c, SEM_C + c), slab_copy(NG + c, SEM_C + c),
                pltpu.make_async_copy(wqkv_hbm.at[rows, :], wraw_v.at[rows, :], sem.at[SEM_W + c])]

    copies["c"].start()
    copies["x0"].start()
    for c in range(NKC):
        for cp in chunk_copies(c):
            cp.start()
    for n in ("x1", "x2", "wo", "xr"):
        copies[n].start()
    for j in range(2 * NG, NMOD):
        slab_copy(j, names.index("wm")).start()
    for n in ("w1", "w3", "w2"):
        copies[n].start()
    zv_v[...] = jnp.zeros(zv_v.shape, u32)

    proj = (p0_v, p1_v)
    mcol = lambda sec, g: (mod_v if sec < 2 else modr_v)[sec * NG + g]
    row8 = lax.broadcasted_iota(jnp.int32, (8, 128), 0)

    def mod_round(j, kh):
        ks = slice(kh * 512, (kh + 1) * 512)
        return _dot(sc_v[:, ks], wm_v[j, ks, :])[0:8]

    def ln1_rows(row, drow, dep):
        xn = _norm8(_groups(x_v[pl.ds(row, 8), :].astype(f32)), dep)
        ys = [xn[g] * mcol(1, g) + mcol(0, g) for g in range(NG)]
        h_v[drow:drow + 8, 0:D] = jnp.concatenate(ys, axis=1).astype(bf16)
        return _bits(ys[NG - 1])

    def ln2_rows(row, drow, dep):
        x = _groups(x_v[pl.ds(row, 8), :].astype(f32))
        x1 = [x[g] + mcol(2, g) * a_v[g, pl.ds(row, 8), :] for g in range(NG)]
        x1_v[drow:drow + 8, :] = jnp.concatenate(x1, axis=1)
        xn = _norm8(x1, dep)
        ys = [xn[g] * mcol(4, g) + mcol(3, g) for g in range(NG)]
        h2_v[drow:drow + 8, 0:D] = jnp.concatenate(ys, axis=1).astype(bf16)
        return _bits(ys[NG - 1])

    def attn8(src, t0, pb, par, dep):
        r0 = KOFF + 16 * pb + par
        rows = lambda j: pl.ds(r0 - DIL * j, 8, stride=DIL)
        zvec = zv_v[...]
        s = [None] * W
        for g in range(NG):
            q = src[g, rows(0), :]
            if g == 0:
                q = _after(q, dep)
            elif CQ and g % CQ == 0:
                q = _after(q, _bits(s[W - 1]) & zvec)
            for j in range(W):
                p = q * src[NG + g, rows(j), :]
                s[j] = p if s[j] is None else s[j] + p
        for j in range(W):
            s[j] = s[j] + pltpu.roll(s[j], 64, 1)
            s[j] = s[j] + pltpu.roll(s[j], 32, 1)
            if t0 is not None and pb == 0 and j > 0:
                s[j] = jnp.where(t0 + par + DIL * row8 >= DIL * j, s[j], NEG)
        m = functools.reduce(jnp.maximum, s)
        e = [jnp.exp2((s[j] - m) * QSCALE) for j in range(W)]
        den = functools.reduce(_add, e)
        r = pl.reciprocal(den, approx=True)
        inv = r * (2.0 - den * r)
        og = [None] * NG
        for j in range(W):
            p = e[j] * inv
            if CP and j and j % CP == 0:
                p = _after(p, _bits(og[NG - 1]) & zvec)
            for g in range(NG):
                t = p * src[2 * NG + g, rows(j), :]
                og[g] = t if og[g] is None else og[g] + t
        return og

    def attn16(src, t0, pb, srow, dep, dep2=None):
        a = attn8(src, t0, pb, 0, dep)
        b = attn8(src, t0, pb, 1, dep if dep2 is None else dep2)
        for g in range(NG):
            st_v[srow:srow + 8, g * 128:(g + 1) * 128] = _bits(jnp.concatenate([a[g], b[g]], axis=0).astype(bf16))
        return _bits(a[NG - 1]) | _bits(b[NG - 1])

    def unstage(r0, r1):
        return jnp.concatenate(_from_head_lanes(_groups(st_v[r0:r1, :])), axis=1)

    def out_proj(o, t0, side=None):
        a = _groups(_dot(o, wo_v[:, 0:D]))
        links = side(a) if side is not None else {}
        for g in range(NG):
            for rb in range(a[g].shape[0] // 8):
                v = a[g][rb * 8:(rb + 1) * 8]
                if rb == 0 and g in links:
                    v = _after(v, links[g])
                a_v[g, pl.ds(t0 + (rb // 2) * 16 + rb % 2, 8, stride=2), :] = v

    def mod_vpu(j, part, nparts, dep):
        n = D // nparts
        acc = [None] * 4
        for i in range(n // 8):
            rows = slice(part * n + i * 8, part * n + (i + 1) * 8)
            cb = cb_v[rows, :]
            if i == 0:
                cb = _after(cb, dep)
            t = wm_v[j, rows, :].astype(f32) * cb
            acc[i % 4] = t if acc[i % 4] is None else acc[i % 4] + t
        return (acc[0] + acc[1]) + (acc[2] + acc[3])

    def chunk_block(c, par, do_prep, do_mm, extra=None):
        zvec = zv_v[...]
        links = {}

        def link(ct, v):
            links[ct] = (links[ct] | v) if ct in links else v

        def rounds(hc, wp, rs, between=None):
            res = {}
            for k, r in enumerate(rs):
                out = _groups(_dot(hc, pltpu.bitcast(wp[:, r * 512:(r + 1) * 512], bf16)))
                for n in range(4):
                    res[4 * r + n] = out[n]
                if between is not None:
                    between(k)
            return res

        def accumulate(res):
            for ct in res:
                for t in range(SKEW):
                    blk = res[ct][t * T:(t + 1) * T]
                    if t == SKEW - 1 and ct in links:
                        blk = jnp.concatenate([blk[0:T - 8], _after(blk[T - 8:T], links.pop(ct) & zvec)], axis=0)
                    proj[t % 2][t // 2, ct, KOFF:KOFF + T, :] += blk
        mr = []

        def mods(k):
            todo = range(len(mr), 4) if k is None else range(len(mr), min(4, (4 * (k + 1)) // MR))
            for r in todo:
                mr.append(mod_round(c + NG * (r // 2), r % 2))
        if do_prep:
            for cp in chunk_copies(c):
                cp.wait()
        if do_mm:
            res = rounds((he_v, ho_v)[1 - par][...], (wpe_v, wpo_v)[1 - par].at[(c - 1) >> 1], range(WR, 6),
                         mods if do_prep else None)
        if do_prep:
            mods(None)
            sh = mr[0] + mr[1]
            s1 = mr[2] + mr[3] + 1.0
            mod_v[c] = sh
            mod_v[NG + c] = s1
            hc = (xn_v[c].reshape(M0 // 8, 8, 128) * s1 + sh).reshape(M0, 128).astype(bf16)
            (he_v, ho_v)[par][...] = hc
            wp = (wpe_v, wpo_v)[par].at[c >> 1]
            for b in range(6):
                sec, half = b // 2, b % 2
                r0 = pl.multiple_of(c * KC + half * 64, 64)
                vs = _groups(_bits(wraw_v[pl.ds(r0, 64), sec * D:(sec + 1) * D]))
                vs = _to_head_lanes(vs)
                wp[half * 32:(half + 1) * 32, sec * D:(sec + 1) * D] = jnp.concatenate(vs, axis=1)
                if 2 * sec + 2 > WR:
                    link(4 * WR - 2 + half - 2 * (2 - sec), vs[NG - 1][24:32])
        if extra is not None:
            extra(res, link, zvec)
        if do_mm:
            accumulate(res)
        if do_prep:
            accumulate(rounds(hc, wp, range(WR)))

    with scope("p_first"):
        def zero(ct, carry):
            for t in range(SKEW):
                proj[t % 2][t // 2, ct, KOFF:KOFF + T, :] = jnp.zeros((T, 128), f32)
            return carry
        lax.fori_loop(0, 3 * NG, zero, 0)
        copies["c"].wait()
        c32 = c_v[...].astype(f32)
        sc = (c32 * jax.nn.sigmoid(c32)).astype(bf16)
        sc_v[...] = jnp.broadcast_to(sc, (16, D))
        diag = lax.broadcasted_iota(jnp.int32, (128, 128), 0) == lax.broadcasted_iota(jnp.int32, (128, 128), 1)
        for g, row in enumerate(_groups(sc.astype(f32))):
            col = jnp.sum(jnp.where(diag, row, 0.0), axis=1, keepdims=True)
            cb_v[g * 128:(g + 1) * 128, :] = jnp.broadcast_to(col, (128, 128))
        copies["x0"].wait()

        def stats(i, carry):
            for rb in range(12):
                rows = pl.ds(pl.multiple_of(i * 96, 32) + rb * 8, 8)
                xn = _norm8(_groups(x_v[rows, :].astype(f32)))
                for g in range(NG):
                    xn_v[g, rows, :] = xn[g]
            return carry
        lax.fori_loop(0, M0 // 96, stats, 0)
        chunk_block(0, 0, True, False)

    def kloop(i, carry):
        chunk_block(2 * i + 1, 1, True, True)

        @pl.when(2 * i + 2 < NKC)
        def _():
            chunk_block(2 * i + 2, 0, True, True)
        return carry
    with scope("p_kloop"):
        lax.fori_loop(0, NKC // 2, kloop, 0)

    with scope("p_last"):
        copies["x1"].wait()

        def ln_next(res, link, zvec):
            for rb in range(T // 8):
                ct = 4 * WR + (rb * (20 - 4 * WR)) // (T // 8)
                link(ct + 3, ln1_rows(M0 + rb * 8, rb * 8, _bits(res[ct][M0 - 8:M0]) & zvec))
        chunk_block(NKC, 0, False, True, ln_next)
        for t in range(SKEW):
            for sg in range(NG, 3 * NG):
                if t == 0:
                    halo = jnp.broadcast_to(p0_v[0, sg, KOFF:KOFF + 1, :], (HALO, 128))
                else:
                    halo = proj[(t - 1) % 2][(t - 1) // 2, sg, KOFF + T - HALO:KOFF + T, :]
                proj[t % 2][t // 2, sg, KOFF - HALO:KOFF, :] = halo
        copies["x2"].wait()
        copies["wo"].wait()

    def step(s, par):
        if par == 1:
            @pl.when(s == 1)
            def _():
                copies["xr"].wait()

            @pl.when(s == MLAG)
            def _():
                copies["wm"].wait()
        jn = 2 * NG + MPS * (s - MLAG)
        j0 = jnp.where((s >= MLAG) & (jn < NMOD), jn, 0)
        zvec = zv_v[...]
        t0 = pl.multiple_of(s * T, T)
        slot = (s >> 1) & 1
        dst = proj[1 - par].at[((s + SKEW) >> 1) & 1]
        prev = proj[par].at[1 - slot]
        w = jnp.concatenate([(wpe_v, wpo_v)[c % 2][c // 2, :, 0:3 * D] for c in range(NKC)], axis=0)
        tiles = _groups(_dot(h_v[:, 0:D], pltpu.bitcast(w, bf16)))
        for ct in range(3 * NG):
            dst[ct, KOFF:KOFF + T, :] = tiles[ct]
            if ct >= NG:
                dst[ct, KOFF - HALO:KOFF, :] = prev[ct, KOFF + T - HALO:KOFF + T, :]
        t1 = pl.multiple_of(jnp.minimum(s + SKEW + 1, NT - 1) * T, T)
        src = proj[par].at[slot]
        links, rows = [], []
        def gate(pos):
            ct = int(pos)
            rb = min(T // 8 - 1, int((pos - ct) * (T // 8)))
            return _bits(tiles[ct][rb * 8:(rb + 1) * 8, :]) & zvec
        for pb in range(NP):
            ds = []
            for p2 in range(2):
                k = 2 * pb + (p2 if STG else 0)
                d = gate(GA + GS * k / (2 * NP))
                if pb >= 2:
                    d = d | (links[2 * pb + p2 - 4] & zvec)
                ds.append(d)
            attn16(src, t0 if par == 0 else None, pb, pb * 8, ds[0], ds[1])
            for rb in (2 * pb, 2 * pb + 1):
                links.append(ln1_rows(t1 + rb * 8, rb * 8, gate(GA + GS * (rb if STG else 2 * pb) / (2 * NP))))
            if (pb + 1) % UG == 0:
                rows.append(pltpu.bitcast(unstage((pb + 1 - UG) * 8, (pb + 1) * 8), bf16))

        def mods(a):
            links = {}
            for k in range(MPS):
                gates = [(tiles[3 * NG - 2:] + a)[(7 * (2 * k + h)) // (2 * MPS)][T - 8:T] for h in range(2)]
                part = [mod_vpu(j0 + k, h, 2, _bits(gates[h]) & zvec) for h in range(2)]
                m = jnp.sum(part[0] + part[1], axis=0, keepdims=True) + jnp.where((j0 + k) >> 3 == 4, 1.0, 0.0)
                m = jnp.broadcast_to(m, (8, 128))
                modr_v[j0 + k] = m
                links[min(2 * k + 3, NG - 1)] = (_bits(m) & zvec) | links.get(min(2 * k + 3, NG - 1), jnp.uint32(0))
            return links
        out_proj(jnp.concatenate(rows, axis=0), t0, mods)

    def phase_a(i, carry):
        step(2 * i, 0)

        @pl.when(2 * i + 1 < NS)
        def _():
            step(2 * i + 1, 1)
        return carry
    with scope("phase_a"):
        lax.fori_loop(0, (NS + 1) // 2, phase_a, 0)

    IPT = NP // PPI

    def fill_window(i, sgs, dep):
        src = p1_v.at[(i // IPT) % 3, :, pl.ds(pl.multiple_of((i % IPT) * 16 * PPI, 16 * PPI), WROWS), :]
        for sg in sgs:
            lo = KOFF if sg < NG else KOFF - HALO
            v = src[sg, lo:WROWS, :]
            if dep is not None:
                v = jnp.concatenate([_after(v[0:8], dep), v[8:]], axis=0)
            win_v[sg, lo:WROWS, :] = v
        return _bits(v[0:8])

    with scope("mid"):
        for sg in range(3 * NG):
            lo = KOFF if sg < NG else KOFF - HALO
            p1_v[2, sg, lo:KOFF + T, :] = p0_v[1, sg, lo:KOFF + T, :]
        fill_window(0, range(3 * NG), None)
        for rb in range(TB // 8):
            ln2_rows(rb * 8, rb * 8, None)
        copies["w1"].wait()
        copies["w3"].wait()
        copies["w2"].wait()

    def out_copy(i, slot):
        return pltpu.make_async_copy(ob_v.at[slot], out_hbm.at[0, pl.ds(pl.multiple_of(i * TB, TB), TB), :], osem.at[slot])

    def phase_b(i, carry):
        t1 = pl.multiple_of(jnp.minimum(i + 1, NTB - 1) * TB, TB)
        slot = i & 1

        def late_proj(t, carry):
            rows = pl.ds(pl.multiple_of(t * (T // 2), T // 2), T // 2)
            out_proj(pltpu.bitcast(o_v[rows, :], bf16), pl.multiple_of((NS + t) * T, T))
            return carry
        if TB == T:
            @pl.when(i == SKEW * IPT)
            def _():
                out_proj(pltpu.bitcast(o_v[...], bf16), NS * T)
        else:
            lax.fori_loop(jnp.where(i == NTB - 2, 1, 0), jnp.where(i == NTB - 3, 1, jnp.where(i == NTB - 2, SKEW, 0)),
                          late_proj, 0)

        @pl.when(i >= 2)
        def _():
            out_copy(i - 2, slot).wait()
        zvec = zv_v[...]
        sl = (i // IPT) % 3
        orow = jnp.where(sl == 0, 0, jnp.where(sl == 1, T, T // 2)) + (i % IPT) * 8 * PPI

        def fin(dep):
            o = unstage(0, 8 * PPI)
            o_v[pl.ds(pl.multiple_of(orow, 8 * PPI), 8 * PPI), :] = o
            return o[8 * PPI - 8:8 * PPI, D - 128:D]
        NRB = TB // 8
        halves = {}

        def att(k, par):
            def run(d):
                halves[(k, par)] = attn8(win_v, None, k, par, d)
                if par == 1:
                    a, b = halves[(k, 0)], halves[(k, 1)]
                    for g in range(NG):
                        st_v[8 * k:8 * k + 8, g * 128:(g + 1) * 128] = _bits(jnp.concatenate([a[g], b[g]], axis=0).astype(bf16))
                return _bits(halves[(k, par)][NG - 1])
            return run
        ln = lambda r: (lambda d: ln2_rows(t1 + r * 8, r * 8, d))
        fw = lambda k: (lambda d: fill_window(i + 1, range(6 * k, 6 * k + 6), d))
        if PLAN == 0:
            side = [[att(0, 0), att(0, 1)], [att(1, 0), att(1, 1)], [fin] + [ln(r) for r in range(0, 4)],
                    [ln(r) for r in range(4, 8)] + [fw(0), fw(1)], [ln(r) for r in range(8, 12)] + [fw(2), fw(3)],
                    [ln(r) for r in range(12, 16)]]
        elif PLAN == 1:
            side = [[att(0, 0), att(0, 1), att(1, 0)], [att(1, 1), ln(0), ln(1)], [fin, ln(2), ln(3), ln(4), fw(0)],
                    [ln(5), ln(6), ln(7), ln(8), fw(1)], [ln(9), ln(10), ln(11), ln(12), fw(2)],
                    [ln(13), ln(14), ln(15), fw(3)]]
        h = h2_v[:, 0:D]
        gb = jnp.concatenate([mcol(5, g) for g in range(NG)], axis=1)
        scaled = lambda y: (y.reshape(NRB, 8, D) * gb).reshape(TB, D)
        acc = act_prev = None
        links = []
        for fc in range(NFC + 1):
            ev = []
            if fc < NFC:
                g = _dot(h, w1_v[:, fc * FC:(fc + 1) * FC])
                u = _dot(h, w3_v[:, fc * FC:(fc + 1) * FC])
                ev = _groups(g) + _groups(u)
                if 1 <= fc <= len(side):
                    u0 = _after(u[TB - 8:TB, FC - 128:FC], functools.reduce(_or, links[fc - 1]) & zvec)
                    u = jnp.concatenate([u[0:TB - 8, :], jnp.concatenate([u[TB - 8:TB, 0:FC - 128], u0], axis=1)], axis=0)
                hg = 0.5 * g
                act = (hg * (1.0 + jnp.tanh(hg)) * u).astype(bf16)
            if fc >= 1:
                y = _dot(act_prev, w2_v[(fc - 1) * FC:fc * FC, 0:D])
                ev = ev + _groups(y)
                acc = (x1_v[...] if acc is None else acc) + scaled(y)
            if fc < len(side):
                n = len(side[fc])
                pos = [min(E0 + (k * EN) // n, len(ev) - 1) if fc else min(G0 + (k * GN) // n, 7) for k in range(n)]
                links.append([fn(_bits(ev[p][TB - 16:TB - 8]) & zvec) for p, fn in zip(pos, side[fc])])
            act_prev = act
        ob_v[slot] = acc.astype(bf16)
        out_copy(i, slot).start()
        return carry
    with scope("phase_b"):
        lax.fori_loop(0, NTB, phase_b, 0)
    out_copy(NTB - 2, 0).wait()
    out_copy(NTB - 1, 1).wait()


@jax.jit
def pallas_adaLN_cond__sliding_local_dilated__glu_gated_swiglu__prompt_kernel(
    A_x, A_wqkv, A_wo, B_x, B_w1, B_w3, B_w2, c, w_mod):
    del B_x
    any_spec = pl.BlockSpec(memory_space=pl.ANY)
    return pl.pallas_call(
        _kernel,
        out_shape=jax.ShapeDtypeStruct((1, S, D), bf16),
        in_specs=[any_spec] * 8,
        out_specs=any_spec,
        scratch_shapes=[
            pltpu.VMEM((S, D), bf16),
            pltpu.VMEM((1, D), bf16),
            pltpu.VMEM((16, D), bf16),
            pltpu.VMEM((D, 128), f32),
            pltpu.VMEM((NMOD, D, 128), bf16),
            pltpu.VMEM((D, 3 * D), bf16),
            pltpu.VMEM((NKC // 2, KC // 2, 3 * D + padw('wp')), u32),
            pltpu.VMEM((NKC // 2, KC // 2, 3 * D + padw('wp')), u32),
            pltpu.VMEM((D, D + padw('wo')), bf16),
            pltpu.VMEM((D, F + padw('w1')), bf16),
            pltpu.VMEM((D, F + padw('w1')), bf16),
            pltpu.VMEM((F, D + padw('w2')), bf16),
            pltpu.VMEM((2 * NG, 8, 128), f32),
            pltpu.VMEM((NMOD, 8, 128), f32),
            pltpu.VMEM((NG, M0, 128), f32),
            pltpu.VMEM((M0, KC), bf16),
            pltpu.VMEM((M0, KC), bf16),
            pltpu.VMEM((T, D + padw('h')), bf16),
            pltpu.VMEM((TB, D + padw('h')), bf16),
            pltpu.VMEM((TB, D), f32),
            pltpu.VMEM((3 * NG, WROWS + 8, 128), f32),
            pltpu.VMEM((T // 2, D), u32),
            pltpu.VMEM((M0 // 2, D), u32),
            pltpu.VMEM((2, 3 * NG, KROWS, 128), f32),
            pltpu.VMEM((3, 3 * NG, KROWS, 128), f32),
            pltpu.VMEM((NG, S + 8, 128), f32),
            pltpu.VMEM((2, TB, D), bf16),
            pltpu.VMEM((8, 128), u32),
            pltpu.SemaphoreType.DMA((10 + 2 * NKC,)),
            pltpu.SemaphoreType.DMA((2,)),
        ],
        compiler_params=pltpu.CompilerParams(vmem_limit_bytes=110 * 2**20, disable_bounds_checks=True,
                                             disable_semaphore_checks=True),
        name="adaln_fused",
    )(A_x, A_wqkv, A_wo, B_w1, B_w3, B_w2, c, w_mod)
```

```python
import functools
import jax
import jax.numpy as jnp
from jax import lax
import jax.experimental.pallas as pl
import jax.experimental.pallas.tpu as pltpu

S, D, F = 2048, 1024, 3584
H, DH, W, DIL = 32, 32, 8, 2
NG = D // 128
HALO = 16
T = 128
NT = S // T
NP = T // 16
SKEW = 3
M0 = SKEW * T
NS = NT - SKEW
TB = 128
NTB = S // TB
PPI = TB // 64
WROWS = HALO + 16 * PPI
FC = 512
NFC = F // FC
KOFF = HALO
KROWS = KOFF + T + 8
LOG2E = 1.4426950408889634
QSCALE = (DH ** -0.5) * LOG2E
NEG = -1e9 * DH ** 0.5
KC = 128
NKC = D // KC
NMOD = 6 * NG
NL = 2 * NG
MPS = 2
MLAG = 3
EPS = 1e-5
G0, GN = 3, 5
MV = 16
GS = 22.0; GA = 0.0; STG = 1
CQ = 1; CP = 1
E0 = 3; EN = 5; PLAN = 0
PAD = "wp,wo,w2,h,w1"
padw = lambda k: 128 if k in PAD.split(",") else 0
WR = 3
MR = 2
UG = 4
f32, bf16, u32 = jnp.float32, jnp.bfloat16, jnp.uint32
scope = jax.named_scope


def _butterfly(vs):
    vs = list(vs)
    lane = lax.broadcasted_iota(jnp.int32, vs[0].shape, 1)
    for s in range(3):
        m = (lane & (4 << s)) != 0
        for g in range(NG):
            if g & (1 << s):
                continue
            a, b = vs[g], vs[g | (1 << s)]
            vs[g] = jnp.where(m, b, a)
            vs[g | (1 << s)] = jnp.where(m, a, b)
    return vs


def _to_head_lanes(vs):
    ys = _butterfly(vs)
    lane = lax.broadcasted_iota(jnp.int32, vs[0].shape, 1)
    head = lane & 31
    out = []
    for g in range(NG):
        src = ((head & 3) << 5) | (((head >> 2) ^ g) << 2) | (lane >> 5)
        out.append(jnp.take_along_axis(ys[g], src, axis=1))
    return out


def _from_head_lanes(zs):
    lane = lax.broadcasted_iota(jnp.int32, zs[0].shape, 1)
    ys = []
    for g in range(NG):
        src = ((lane & 3) << 5) | ((((lane >> 2) & 7) ^ g) << 2) | (lane >> 5)
        ys.append(jnp.take_along_axis(zs[g], src, axis=1))
    return _butterfly(ys)


def _add(a, b):
    return a + b


def _or(a, b):
    return a | b


def _bits(x):
    return pltpu.bitcast(x, u32)


def _dot(a, b):
    return jnp.dot(a, b, preferred_element_type=f32)


def _after(x, dep):
    if dep is None:
        return x
    return pltpu.bitcast(_bits(x) | dep, x.dtype)


def _norm8(xs, dep=None):
    xs = [_after(xs[0], dep)] + list(xs[1:])
    m = jnp.sum(functools.reduce(_add, xs), axis=-1, keepdims=True) * (1.0 / D)
    xc = [v - m for v in xs]
    var = jnp.sum(functools.reduce(_add, [v * v for v in xc]), axis=-1, keepdims=True) * (1.0 / D)
    r = lax.rsqrt(var + EPS)
    return [v * r for v in xc]


def _groups(x):
    return [x[:, g * 128:(g + 1) * 128] for g in range(x.shape[1] // 128)]


def _kernel(x_hbm, wqkv_hbm, wo_hbm, w1_hbm, w3_hbm, w2_hbm, c_hbm, wmod_hbm, out_hbm,
            x_v, c_v, sc_v, cb_v, wm_v, wl_v, wraw_v, wpe_v, wpo_v, wo_v, w1_v, w3_v, w2_v, mod_v, modr_v,
            xn_v, he_v, ho_v, h_v, h2_v, x1_v, win_v, st_v, o_v, p0_v, p1_v, a_v, ob_v,
            zv_v, sem, osem):
    names = ["c", "x0", "x1", "x2", "xr", "wo", "w1", "w3", "w2", "wm"]
    srcdst = dict(
        c=(c_hbm, c_v),
        x0=(x_hbm.at[0, 0:M0, :], x_v.at[0:M0, :]),
        x1=(x_hbm.at[0, M0:M0 + T, :], x_v.at[M0:M0 + T, :]),
        x2=(x_hbm.at[0, M0 + T:M0 + 2 * T, :], x_v.at[M0 + T:M0 + 2 * T, :]),
        xr=(x_hbm.at[0, M0 + 2 * T:S, :], x_v.at[M0 + 2 * T:S, :]),
        wo=(wo_hbm, wo_v.at[:, 0:D]),
        wm=(wl_v.at[0:NL], wl_v.at[0:NL]),
        w1=(w1_hbm, w1_v.at[:, 0:F]), w3=(w3_hbm, w3_v.at[:, 0:F]), w2=(w2_hbm, w2_v.at[:, 0:D]),
    )
    copies = {n: pltpu.make_async_copy(srcdst[n][0], srcdst[n][1], sem.at[i]) for i, n in enumerate(names)}
    SEM_C = len(names)
    SEM_W = SEM_C + NKC

    def slab_copy(j, s):
        return pltpu.make_async_copy(wmod_hbm.at[:, pl.ds(pl.multiple_of(j * 128, 128), 128)], wm_v.at[j], sem.at[s])

    def chunk_copies(c):
        rows = pl.ds(pl.multiple_of(c * KC, KC), KC)
        return [slab_copy(c, SEM_C + c), slab_copy(NG + c, SEM_C + c),
                pltpu.make_async_copy(wqkv_hbm.at[rows, :], wraw_v.at[rows, :], sem.at[SEM_W + c])]

    copies["c"].start()
    copies["x0"].start()
    for c in range(NKC):
        for cp in chunk_copies(c):
            cp.start()
    for n in ("x1", "x2", "wo", "xr"):
        copies[n].start()
    for j in range(NL):
        pltpu.make_async_copy(wmod_hbm.at[:, 2 * D + j * 256:2 * D + (j + 1) * 256], wl_v.at[j],
                              sem.at[names.index("wm")]).start()
    for n in ("w1", "w3", "w2"):
        copies[n].start()
    zv_v[...] = jnp.zeros(zv_v.shape, u32)
    wl_v[NL] = jnp.zeros((D, 256), bf16)

    proj = (p0_v, p1_v)
    mcol = lambda sec, g: mod_v[sec * NG + g] if sec < 2 else modr_v[(sec - 2) * NG + g]
    row8 = lax.broadcasted_iota(jnp.int32, (8, 128), 0)

    def mod_round(j, kh):
        ks = slice(kh * 512, (kh + 1) * 512)
        return _dot(sc_v[:, ks], wm_v[j, ks, :])[0:8]

    def ln1_rows(xt, drow, dep):
        xn = _norm8(_groups(xt[drow:drow + 8, :].astype(f32)), dep)
        ys = [xn[g] * mcol(1, g) + mcol(0, g) for g in range(NG)]
        h_v[drow:drow + 8, 0:D] = jnp.concatenate(ys, axis=1).astype(bf16)
        return _bits(ys[NG - 1])

    def ln2_rows(t, drow, dep):
        xt, at = x_v.at[pl.ds(t, TB), :], a_v.at[:, pl.ds(t, TB), :]
        x = _groups(xt[drow:drow + 8, :].astype(f32))
        x1 = [x[g] + mcol(2, g) * at[g, drow:drow + 8, :] for g in range(NG)]
        x1_v[drow:drow + 8, :] = jnp.concatenate(x1, axis=1)
        xn = _norm8(x1, dep)
        ys = [xn[g] * mcol(4, g) + mcol(3, g) for g in range(NG)]
        h2_v[drow:drow + 8, 0:D] = jnp.concatenate(ys, axis=1).astype(bf16)
        return _bits(ys[NG - 1])

    def attn8(src, t0, pb, par, dep):
        r0 = KOFF + 16 * pb + par
        rows = lambda j: pl.ds(r0 - DIL * j, 8, stride=DIL)
        zvec = zv_v[...]
        s = [None] * W
        for g in range(NG):
            q = src[g, rows(0), :]
            if g == 0:
                q = _after(q, dep)
            elif CQ and g % CQ == 0:
                q = _after(q, _bits(s[W - 1]) & zvec)
            for j in range(W):
                p = q * src[NG + g, rows(j), :]
                s[j] = p if s[j] is None else s[j] + p
        for j in range(W):
            s[j] = s[j] + pltpu.roll(s[j], 64, 1)
            s[j] = s[j] + pltpu.roll(s[j], 32, 1)
            if t0 is not None and pb == 0 and j > 0:
                s[j] = jnp.where(t0 + par + DIL * row8 >= DIL * j, s[j], NEG)
        m = functools.reduce(jnp.maximum, s)
        e = [jnp.exp2((s[j] - m) * QSCALE) for j in range(W)]
        den = functools.reduce(_add, e)
        r = pl.reciprocal(den, approx=True)
        inv = r * (2.0 - den * r)
        og = [None] * NG
        for j in range(W):
            p = e[j] * inv
            if CP and j and j % CP == 0:
                p = _after(p, _bits(og[NG - 1]) & zvec)
            for g in range(NG):
                t = p * src[2 * NG + g, rows(j), :]
                og[g] = t if og[g] is None else og[g] + t
        return og

    def attn16(src, t0, pb, srow, dep, dep2=None):
        a = attn8(src, t0, pb, 0, dep)
        b = attn8(src, t0, pb, 1, dep if dep2 is None else dep2)
        for g in range(NG):
            st_v[srow:srow + 8, g * 128:(g + 1) * 128] = _bits(jnp.concatenate([a[g], b[g]], axis=0).astype(bf16))
        return _bits(a[NG - 1]) | _bits(b[NG - 1])

    def unstage(r0, r1):
        return jnp.concatenate(_from_head_lanes(_groups(st_v[r0:r1, :])), axis=1)

    def out_proj(o, t0, side=None):
        a = _groups(_dot(o, wo_v[:, 0:D]))
        links = side(a) if side is not None else {}
        at = a_v.at[:, pl.ds(t0, o.shape[0] + 8), :]
        for g in range(NG):
            for rb in range(a[g].shape[0] // 8):
                v = a[g][rb * 8:(rb + 1) * 8]
                if rb == 0 and g in links:
                    v = _after(v, links[g])
                at[g, pl.ds((rb // 2) * 16 + rb % 2, 8, stride=2), :] = v

    def mod_vpu(j, part, nparts, dep):
        n = D // nparts
        acc = [None] * 2
        for i in range(n // 8):
            rows = slice(part * n + i * 8, part * n + (i + 1) * 8)
            cb = cb_v[rows, :]
            if i == 0:
                cb = _after(cb, dep)
            t = wl_v[j, rows, :].astype(f32) * jnp.concatenate([cb, cb], axis=1)
            acc[i % 2] = t if acc[i % 2] is None else acc[i % 2] + t
        return acc[0] + acc[1]

    def chunk_block(c, par, do_prep, do_mm, extra=None):
        zvec = zv_v[...]
        links = {}

        def link(ct, v):
            links[ct] = (links[ct] | v) if ct in links else v

        def rounds(hc, wp, rs, between=None):
            res = {}
            for k, r in enumerate(rs):
                out = _groups(_dot(hc, pltpu.bitcast(wp[:, r * 512:(r + 1) * 512], bf16)))
                for n in range(4):
                    res[4 * r + n] = out[n]
                if between is not None:
                    between(k)
            return res

        def accumulate(res):
            for ct in res:
                for t in range(SKEW):
                    blk = res[ct][t * T:(t + 1) * T]
                    if t == SKEW - 1 and ct in links:
                        blk = jnp.concatenate([blk[0:T - 8], _after(blk[T - 8:T], links.pop(ct) & zvec)], axis=0)
                    proj[t % 2][t // 2, ct, KOFF:KOFF + T, :] += blk
        mr = []

        def mods(k):
            todo = range(len(mr), 4) if k is None else range(len(mr), min(4, (4 * (k + 1)) // MR))
            for r in todo:
                mr.append(mod_round(c + NG * (r // 2), r % 2))
        if do_prep:
            for cp in chunk_copies(c):
                cp.wait()
        if do_mm:
            res = rounds((he_v, ho_v)[1 - par][...], (wpe_v, wpo_v)[1 - par].at[(c - 1) >> 1], range(WR, 6),
                         mods if do_prep else None)
        if do_prep:
            mods(None)
            sh = mr[0] + mr[1]
            s1 = mr[2] + mr[3] + 1.0
            mod_v[c] = sh
            mod_v[NG + c] = s1
            hc = (xn_v[c].reshape(M0 // 8, 8, 128) * s1 + sh).reshape(M0, 128).astype(bf16)
            (he_v, ho_v)[par][...] = hc
            wp = (wpe_v, wpo_v)[par].at[c >> 1]
            for b in range(6):
                sec, half = b // 2, b % 2
                r0 = pl.multiple_of(c * KC + half * 64, 64)
                vs = _groups(_bits(wraw_v[pl.ds(r0, 64), sec * D:(sec + 1) * D]))
                vs = _to_head_lanes(vs)
                wp[half * 32:(half + 1) * 32, sec * D:(sec + 1) * D] = jnp.concatenate(vs, axis=1)
                if 2 * sec + 2 > WR:
                    link(4 * WR - 2 + half - 2 * (2 - sec), vs[NG - 1][24:32])
        if extra is not None:
            extra(res, link, zvec)
        if do_mm:
            accumulate(res)
        if do_prep:
            accumulate(rounds(hc, wp, range(WR)))

    with scope("p_first"):
        def zero(ct, carry):
            for t in range(SKEW):
                proj[t % 2][t // 2, ct, KOFF:KOFF + T, :] = jnp.zeros((T, 128), f32)
            return carry
        lax.fori_loop(0, 3 * NG, zero, 0)
        copies["c"].wait()
        c32 = c_v[...].astype(f32)
        sc = (c32 * jax.nn.sigmoid(c32)).astype(bf16)
        sc_v[...] = jnp.broadcast_to(sc, (16, D))
        diag = lax.broadcasted_iota(jnp.int32, (128, 128), 0) == lax.broadcasted_iota(jnp.int32, (128, 128), 1)
        for g, row in enumerate(_groups(sc.astype(f32))):
            col = jnp.sum(jnp.where(diag, row, 0.0), axis=1, keepdims=True)
            cb_v[g * 128:(g + 1) * 128, :] = jnp.broadcast_to(col, (128, 128))
        copies["x0"].wait()

        def stats(i, carry):
            for rb in range(12):
                rows = pl.ds(pl.multiple_of(i * 96, 32) + rb * 8, 8)
                xn = _norm8(_groups(x_v[rows, :].astype(f32)))
                for g in range(NG):
                    xn_v[g, rows, :] = xn[g]
            return carry
        lax.fori_loop(0, M0 // 96, stats, 0)
        chunk_block(0, 0, True, False)

    def kloop(i, carry):
        chunk_block(2 * i + 1, 1, True, True)

        @pl.when(2 * i + 2 < NKC)
        def _():
            chunk_block(2 * i + 2, 0, True, True)
        return carry
    with scope("p_kloop"):
        lax.fori_loop(0, NKC // 2, kloop, 0)

    with scope("p_last"):
        copies["x1"].wait()

        def ln_next(res, link, zvec):
            for rb in range(T // 8):
                ct = 4 * WR + (rb * (20 - 4 * WR)) // (T // 8)
                link(ct + 3, ln1_rows(x_v.at[M0:M0 + T, :], rb * 8, _bits(res[ct][M0 - 8:M0]) & zvec))
        chunk_block(NKC, 0, False, True, ln_next)
        for t in range(SKEW):
            for sg in range(NG, 3 * NG):
                if t == 0:
                    halo = jnp.broadcast_to(p0_v[0, sg, KOFF:KOFF + 1, :], (HALO, 128))
                else:
                    halo = proj[(t - 1) % 2][(t - 1) // 2, sg, KOFF + T - HALO:KOFF + T, :]
                proj[t % 2][t // 2, sg, KOFF - HALO:KOFF, :] = halo
        copies["x2"].wait()
        copies["wo"].wait()

    def step(s, par):
        if par == 1:
            @pl.when(s == 1)
            def _():
                copies["xr"].wait()

            @pl.when(s == MLAG)
            def _():
                copies["wm"].wait()
        jn = MPS * (s - MLAG)
        late = (s >= MLAG) & (jn < NL)
        zvec = zv_v[...]
        t0 = pl.multiple_of(s * T, T)
        slot = (s >> 1) & 1
        dst = proj[1 - par].at[((s + SKEW) >> 1) & 1]
        prev = proj[par].at[1 - slot]
        w = jnp.concatenate([(wpe_v, wpo_v)[c % 2][c // 2, :, 0:3 * D] for c in range(NKC)], axis=0)
        tiles = _groups(_dot(h_v[:, 0:D], pltpu.bitcast(w, bf16)))
        for ct in range(3 * NG):
            dst[ct, KOFF:KOFF + T, :] = tiles[ct]
            if ct >= NG:
                dst[ct, KOFF - HALO:KOFF, :] = prev[ct, KOFF + T - HALO:KOFF + T, :]
        t1 = pl.multiple_of(jnp.minimum(s + SKEW + 1, NT - 1) * T, T)
        src = proj[par].at[slot]
        links, rows = [], []
        def gate(pos):
            ct = int(pos)
            rb = min(T // 8 - 1, int((pos - ct) * (T // 8)))
            return _bits(tiles[ct][rb * 8:(rb + 1) * 8, :]) & zvec
        for pb in range(NP):
            ds = []
            for p2 in range(2):
                k = 2 * pb + (p2 if STG else 0)
                d = gate(GA + GS * k / (2 * NP))
                if pb >= 2:
                    d = d | (links[2 * pb + p2 - 4] & zvec)
                ds.append(d)
            attn16(src, t0 if par == 0 else None, pb, pb * 8, ds[0], ds[1])
            for rb in (2 * pb, 2 * pb + 1):
                links.append(ln1_rows(x_v.at[pl.ds(t1, T), :], rb * 8, gate(GA + GS * (rb if STG else 2 * pb) / (2 * NP))))
            if (pb + 1) % UG == 0:
                rows.append(pltpu.bitcast(unstage((pb + 1 - UG) * 8, (pb + 1) * 8), bf16))

        def mods(a):
            links = {}
            ev = tiles[3 * NG - 2:] + a
            for k in range(MPS):
                j = jnp.where(late, jn + k, NL)
                part = [mod_vpu(j, h, 4, _bits(ev[(7 * (4 * k + h)) // (4 * MPS)][T - 8:T]) & zvec) for h in range(4)]
                m = jnp.sum((part[0] + part[1]) + (part[2] + part[3]), axis=0, keepdims=True)
                m = jnp.broadcast_to(m + jnp.where(j >> 2 == 2, 1.0, 0.0), (8, 256))
                modr_v[2 * j] = m[:, 0:128]
                modr_v[2 * j + 1] = m[:, 128:256]
                links[min(4 * k + 5, NG - 1)] = _bits(m[:, 0:128]) & zvec
            if par == 0:
                for k in range(6):
                    seen = []
                    for sg in range(4 * k, 4 * k + 4):
                        lo = KOFF if sg < NG else KOFF - HALO
                        for r in range(lo, KOFF + T, 8):
                            v = p0_v[1, sg, r:r + 8, :]
                            if not seen:
                                v = _after(v, _bits(ev[k + 1][T - 8:T]) & zvec)
                            p1_v[2, sg, r:r + 8, :] = v
                            seen.append(_bits(v))
                    lk = functools.reduce(_or, seen) & zvec
                    links[k + 2] = (links[k + 2] | lk) if k + 2 in links else lk
            return links
        out_proj(jnp.concatenate(rows, axis=0), t0, mods)

    def phase_a(i, carry):
        step(2 * i, 0)

        @pl.when(2 * i + 1 < NS)
        def _():
            step(2 * i + 1, 1)
        return carry
    with scope("phase_a"):
        lax.fori_loop(0, (NS + 1) // 2, phase_a, 0)

    IPT = NP // PPI

    def fill_window(i, sgs, dep):
        src = p1_v.at[(i // IPT) % 3, :, pl.ds(pl.multiple_of((i % IPT) * 16 * PPI, 16 * PPI), WROWS), :]
        for sg in sgs:
            lo = KOFF if sg < NG else KOFF - HALO
            v = src[sg, lo:WROWS, :]
            if dep is not None:
                v = jnp.concatenate([_after(v[0:8], dep), v[8:]], axis=0)
            win_v[sg, lo:WROWS, :] = v
        return _bits(v[0:8])

    with scope("mid"):
        fill_window(0, range(3 * NG), None)
        for rb in range(TB // 8):
            ln2_rows(0, rb * 8, None)
        copies["w1"].wait()
        copies["w3"].wait()
        copies["w2"].wait()

    def out_copy(i, slot):
        return pltpu.make_async_copy(ob_v.at[slot], out_hbm.at[0, pl.ds(pl.multiple_of(i * TB, TB), TB), :], osem.at[slot])

    def phase_b(i, carry):
        t1 = pl.multiple_of(jnp.minimum(i + 1, NTB - 1) * TB, TB)
        slot = i & 1

        def late_proj(t, carry):
            rows = pl.ds(pl.multiple_of(t * (T // 2), T // 2), T // 2)
            out_proj(pltpu.bitcast(o_v[rows, :], bf16), pl.multiple_of((NS + t) * T, T))
            return carry
        if TB == T:
            @pl.when(i == SKEW * IPT)
            def _():
                out_proj(pltpu.bitcast(o_v[...], bf16), NS * T)
        else:
            lax.fori_loop(jnp.where(i == NTB - 2, 1, 0), jnp.where(i == NTB - 3, 1, jnp.where(i == NTB - 2, SKEW, 0)),
                          late_proj, 0)

        @pl.when(i >= 2)
        def _():
            out_copy(i - 2, slot).wait()
        zvec = zv_v[...]
        sl = (i // IPT) % 3
        orow = jnp.where(sl == 0, 0, jnp.where(sl == 1, T, T // 2)) + (i % IPT) * 8 * PPI

        def fin(dep):
            o = unstage(0, 8 * PPI)
            o_v[pl.ds(pl.multiple_of(orow, 8 * PPI), 8 * PPI), :] = o
            return o[8 * PPI - 8:8 * PPI, D - 128:D]
        NRB = TB // 8
        halves = {}

        def att(k, par):
            def run(d):
                halves[(k, par)] = attn8(win_v, None, k, par, d)
                if par == 1:
                    a, b = halves[(k, 0)], halves[(k, 1)]
                    for g in range(NG):
                        st_v[8 * k:8 * k + 8, g * 128:(g + 1) * 128] = _bits(jnp.concatenate([a[g], b[g]], axis=0).astype(bf16))
                return _bits(halves[(k, par)][NG - 1])
            return run
        ln = lambda r: (lambda d: ln2_rows(t1, r * 8, d))
        fw = lambda k: (lambda d: fill_window(i + 1, range(6 * k, 6 * k + 6), d))
        if PLAN == 0:
            side = [[att(0, 0), att(0, 1)], [att(1, 0), att(1, 1)], [fin] + [ln(r) for r in range(0, 4)],
                    [ln(r) for r in range(4, 8)] + [fw(0), fw(1)], [ln(r) for r in range(8, 12)] + [fw(2), fw(3)],
                    [ln(r) for r in range(12, 16)]]
        elif PLAN == 1:
            side = [[att(0, 0), att(0, 1), att(1, 0)], [att(1, 1), ln(0), ln(1)], [fin, ln(2), ln(3), ln(4), fw(0)],
                    [ln(5), ln(6), ln(7), ln(8), fw(1)], [ln(9), ln(10), ln(11), ln(12), fw(2)],
                    [ln(13), ln(14), ln(15), fw(3)]]
        h = h2_v[:, 0:D]
        gb = jnp.concatenate([mcol(5, g) for g in range(NG)], axis=1)
        scaled = lambda y: (y.reshape(NRB, 8, D) * gb).reshape(TB, D)
        acc = act_prev = None
        links = []
        for fc in range(NFC + 1):
            ev = []
            if fc < NFC:
                g = _dot(h, w1_v[:, fc * FC:(fc + 1) * FC])
                u = _dot(h, w3_v[:, fc * FC:(fc + 1) * FC])
                ev = _groups(g) + _groups(u)
                if 1 <= fc <= len(side):
                    u0 = _after(u[TB - 8:TB, FC - 128:FC], functools.reduce(_or, links[fc - 1]) & zvec)
                    u = jnp.concatenate([u[0:TB - 8, :], jnp.concatenate([u[TB - 8:TB, 0:FC - 128], u0], axis=1)], axis=0)
                hg = 0.5 * g
                act = (hg * (1.0 + jnp.tanh(hg)) * u).astype(bf16)
            if fc >= 1:
                y = _dot(act_prev, w2_v[(fc - 1) * FC:fc * FC, 0:D])
                ev = ev + _groups(y)
                acc = (x1_v[...] if acc is None else acc) + scaled(y)
            if fc < len(side):
                n = len(side[fc])
                pos = [min(E0 + (k * EN) // n, len(ev) - 1) if fc else min(G0 + (k * GN) // n, 7) for k in range(n)]
                links.append([fn(_bits(ev[p][TB - 16:TB - 8]) & zvec) for p, fn in zip(pos, side[fc])])
            act_prev = act
        ob_v[slot] = acc.astype(bf16)
        out_copy(i, slot).start()
        return carry
    with scope("phase_b"):
        lax.fori_loop(0, NTB, phase_b, 0)
    out_copy(NTB - 2, 0).wait()
    out_copy(NTB - 1, 1).wait()


@jax.jit
def pallas_adaLN_cond__sliding_local_dilated__glu_gated_swiglu__prompt_kernel(
    A_x, A_wqkv, A_wo, B_x, B_w1, B_w3, B_w2, c, w_mod):
    del B_x
    any_spec = pl.BlockSpec(memory_space=pl.ANY)
    return pl.pallas_call(
        _kernel,
        out_shape=jax.ShapeDtypeStruct((1, S, D), bf16),
        in_specs=[any_spec] * 8,
        out_specs=any_spec,
        scratch_shapes=[
            pltpu.VMEM((S, D), bf16),
            pltpu.VMEM((1, D), bf16),
            pltpu.VMEM((16, D), bf16),
            pltpu.VMEM((D, 128), f32),
            pltpu.VMEM((2 * NG, D, 128), bf16),
            pltpu.VMEM((NL + 1, D, 256), bf16),
            pltpu.VMEM((D, 3 * D), bf16),
            pltpu.VMEM((NKC // 2, KC // 2, 3 * D + padw('wp')), u32),
            pltpu.VMEM((NKC // 2, KC // 2, 3 * D + padw('wp')), u32),
            pltpu.VMEM((D, D + padw('wo')), bf16),
            pltpu.VMEM((D, F + padw('w1')), bf16),
            pltpu.VMEM((D, F + padw('w1')), bf16),
            pltpu.VMEM((F, D + padw('w2')), bf16),
            pltpu.VMEM((2 * NG, 8, 128), f32),
            pltpu.VMEM((2 * NL + 2, 8, 128), f32),
            pltpu.VMEM((NG, M0, 128), f32),
            pltpu.VMEM((M0, KC), bf16),
            pltpu.VMEM((M0, KC), bf16),
            pltpu.VMEM((T, D + padw('h')), bf16),
            pltpu.VMEM((TB, D + padw('h')), bf16),
            pltpu.VMEM((TB, D), f32),
            pltpu.VMEM((3 * NG, WROWS + 8, 128), f32),
            pltpu.VMEM((T // 2, D), u32),
            pltpu.VMEM((M0 // 2, D), u32),
            pltpu.VMEM((2, 3 * NG, KROWS, 128), f32),
            pltpu.VMEM((3, 3 * NG, KROWS, 128), f32),
            pltpu.VMEM((NG, S + 8, 128), f32),
            pltpu.VMEM((2, TB, D), bf16),
            pltpu.VMEM((8, 128), u32),
            pltpu.SemaphoreType.DMA((10 + 2 * NKC,)),
            pltpu.SemaphoreType.DMA((2,)),
        ],
        compiler_params=pltpu.CompilerParams(vmem_limit_bytes=110 * 2**20, disable_bounds_checks=True,
                                             disable_semaphore_checks=True),
        name="adaln_fused",
    )(A_x, A_wqkv, A_wo, B_w1, B_w3, B_w2, c, w_mod)
```

```python
import functools

import jax
import jax.numpy as jnp
from jax import lax
import jax.experimental.pallas as pl
import jax.experimental.pallas.tpu as pltpu

S, D, F = 2048, 1024, 3584
DH, W, DIL = 32, 8, 2
NG = D // 128
HALO = 16
T = 128
NT = S // T
NP = T // 16
NRB = T // 8
SKEW = 3
M0 = SKEW * T
NS = NT - SKEW
PPI = 2
IPT = NP // PPI
WROWS = HALO + 16 * PPI
FC = 512
NFC = F // FC
KOFF = HALO
KROWS = KOFF + T + 8
LOG2E = 1.4426950408889634
QSCALE = (DH ** -0.5) * LOG2E
NEG = -1e9 * DH ** 0.5
KC = 128
NKC = D // KC
WR = 4
NL = 2 * NG
MPS = 2
MLAG = 3
PADW = 128
EPS = 1e-5
GATES = {"first": (20.5, 0.3, 0.3, 5, 8), 1: (20.0, 0.0, 0.9, 4, 4), 0: (19.0, 0.3, 0.9, 5, 8)}
FPLAN = "aaa/all/flll/lwlll/lwlwl/lllwl"
f32, bf16, u32 = jnp.float32, jnp.bfloat16, jnp.uint32


def _butterfly(vs):
    vs = list(vs)
    lane = lax.broadcasted_iota(jnp.int32, vs[0].shape, 1)
    for s in range(3):
        m = (lane & (4 << s)) != 0
        for g in range(NG):
            if g & (1 << s):
                continue
            a, b = vs[g], vs[g | (1 << s)]
            vs[g] = jnp.where(m, b, a)
            vs[g | (1 << s)] = jnp.where(m, a, b)
    return vs


def _to_head_lanes(vs):
    ys = _butterfly(vs)
    lane = lax.broadcasted_iota(jnp.int32, vs[0].shape, 1)
    head = lane & 31
    out = []
    for g in range(NG):
        src = ((head & 3) << 5) | (((head >> 2) ^ g) << 2) | (lane >> 5)
        out.append(jnp.take_along_axis(ys[g], src, axis=1))
    return out


def _from_head_lanes(zs):
    lane = lax.broadcasted_iota(jnp.int32, zs[0].shape, 1)
    ys = []
    for g in range(NG):
        src = ((lane & 3) << 5) | ((((lane >> 2) & 7) ^ g) << 2) | (lane >> 5)
        ys.append(jnp.take_along_axis(zs[g], src, axis=1))
    return _butterfly(ys)


def _add(a, b):
    return a + b


def _or(a, b):
    return a | b


def _bits(x):
    return pltpu.bitcast(x, u32)


def _dot(a, b):
    return jnp.dot(a, b, preferred_element_type=f32)


def _after(x, dep):
    if dep is None:
        return x
    return pltpu.bitcast(_bits(x) | dep, x.dtype)


def _norm8(xs, dep=None):
    xs = [_after(xs[0], dep)] + list(xs[1:])
    m = jnp.sum(functools.reduce(_add, xs), axis=-1, keepdims=True) * (1.0 / D)
    xc = [v - m for v in xs]
    var = jnp.sum(functools.reduce(_add, [v * v for v in xc]), axis=-1, keepdims=True) * (1.0 / D)
    r = lax.rsqrt(var + EPS)
    return [v * r for v in xc]


def _groups(x):
    return [x[:, g * 128:(g + 1) * 128] for g in range(x.shape[1] // 128)]


def _kernel(x_hbm, wqkv_hbm, wo_hbm, w1_hbm, w3_hbm, w2_hbm, c_hbm, wmod_hbm, out_hbm,
            x_v, c_v, sc_v, cb_v, wm_v, wl_v, wraw_v, wpe_v, wpo_v, wo_v, w1_v, w3_v, w2_v, mod_v, modr_v,
            xn_v, he_v, ho_v, h_v, h2_v, x1_v, win_v, st_v, o_v, p0_v, p1_v, a_v, ob_v,
            zv_v, sem, osem):
    names = ["c", "x0", "x1", "x2", "xr", "wo", "w1", "w3", "w2", "wm"]
    srcdst = dict(
        c=(c_hbm, c_v),
        x0=(x_hbm.at[0, 0:M0, :], x_v.at[0:M0, :]),
        x1=(x_hbm.at[0, M0:M0 + T, :], x_v.at[M0:M0 + T, :]),
        x2=(x_hbm.at[0, M0 + T:M0 + 2 * T, :], x_v.at[M0 + T:M0 + 2 * T, :]),
        xr=(x_hbm.at[0, M0 + 2 * T:S, :], x_v.at[M0 + 2 * T:S, :]),
        wo=(wo_hbm, wo_v.at[:, 0:D]),
        wm=(wl_v.at[0:NL], wl_v.at[0:NL]),
        w1=(w1_hbm, w1_v.at[:, 0:F]), w3=(w3_hbm, w3_v.at[:, 0:F]), w2=(w2_hbm, w2_v.at[:, 0:D]),
    )
    copies = {n: pltpu.make_async_copy(srcdst[n][0], srcdst[n][1], sem.at[i]) for i, n in enumerate(names)}
    SEM_C = len(names)
    SEM_W = SEM_C + NKC

    def slab_copy(j, s):
        return pltpu.make_async_copy(wmod_hbm.at[:, pl.ds(pl.multiple_of(j * 128, 128), 128)], wm_v.at[j], sem.at[s])

    def chunk_copies(c):
        rows = pl.ds(pl.multiple_of(c * KC, KC), KC)
        return [slab_copy(c, SEM_C + c), slab_copy(NG + c, SEM_C + c),
                pltpu.make_async_copy(wqkv_hbm.at[rows, :], wraw_v.at[rows, :], sem.at[SEM_W + c])]

    copies["c"].start()
    copies["x0"].start()
    for c in range(NKC):
        for cp in chunk_copies(c):
            cp.start()
    for n in ("x1", "x2", "wo", "xr"):
        copies[n].start()
    for j in range(NL):
        pltpu.make_async_copy(wmod_hbm.at[:, 2 * D + j * 256:2 * D + (j + 1) * 256], wl_v.at[j],
                              sem.at[names.index("wm")]).start()
    for n in ("w1", "w3", "w2"):
        copies[n].start()
    zv_v[...] = jnp.zeros(zv_v.shape, u32)
    wl_v[NL] = jnp.zeros((D, 256), bf16)

    proj = (p0_v, p1_v)
    mcol = lambda sec, g: mod_v[sec * NG + g] if sec < 2 else modr_v[(sec - 2) * NG + g]
    row8 = lax.broadcasted_iota(jnp.int32, (8, 128), 0)

    def mod_round(j, kh):
        ks = slice(kh * 512, (kh + 1) * 512)
        return _dot(sc_v[:, ks], wm_v[j, ks, :])[0:8]

    def ln1_rows(xt, drow, dep):
        xn = _norm8(_groups(xt[drow:drow + 8, :].astype(f32)), dep)
        ys = [xn[g] * mcol(1, g) + mcol(0, g) for g in range(NG)]
        h_v[drow:drow + 8, 0:D] = jnp.concatenate(ys, axis=1).astype(bf16)
        return _bits(ys[NG - 1])

    def ln2_rows(t, drow, dep):
        xt, at = x_v.at[pl.ds(t, T), :], a_v.at[:, pl.ds(t, T), :]
        x = _groups(xt[drow:drow + 8, :].astype(f32))
        x1 = [x[g] + mcol(2, g) * at[g, drow:drow + 8, :] for g in range(NG)]
        x1_v[drow:drow + 8, :] = jnp.concatenate(x1, axis=1)
        xn = _norm8(x1, dep)
        ys = [xn[g] * mcol(4, g) + mcol(3, g) for g in range(NG)]
        h2_v[drow:drow + 8, 0:D] = jnp.concatenate(ys, axis=1).astype(bf16)
        return _bits(ys[NG - 1])

    def attn8(src, masked, pb, par, dep):
        r0 = KOFF + 16 * pb + par
        rows = lambda j: pl.ds(r0 - DIL * j, 8, stride=DIL)
        zvec = zv_v[...]
        s = [None] * W
        for g in range(NG):
            q = src[g, rows(0), :]
            if g == 0:
                q = _after(q, dep)
            else:
                q = _after(q, _bits(s[W - 1]) & zvec)
            for j in range(W):
                p = q * src[NG + g, rows(j), :]
                s[j] = p if s[j] is None else s[j] + p
        for j in range(W):
            s[j] = s[j] + pltpu.roll(s[j], 64, 1)
            s[j] = s[j] + pltpu.roll(s[j], 32, 1)
            if masked and pb == 0 and j > 0:
                s[j] = jnp.where(par + DIL * row8 >= DIL * j, s[j], NEG)
        m = functools.reduce(jnp.maximum, s)
        e = [jnp.exp2((s[j] - m) * QSCALE) for j in range(W)]
        den = functools.reduce(_add, e)
        r = pl.reciprocal(den, approx=True)
        inv = r * (2.0 - den * r)
        og = [None] * NG
        for j in range(W):
            p = e[j] * inv
            if j:
                p = _after(p, _bits(og[NG - 1]) & zvec)
            for g in range(NG):
                t = p * src[2 * NG + g, rows(j), :]
                og[g] = t if og[g] is None else og[g] + t
        return og

    def stage(pb, even, odd):
        for g in range(NG):
            st_v[8 * pb:8 * pb + 8, g * 128:(g + 1) * 128] = _bits(
                jnp.concatenate([even[g], odd[g]], axis=0).astype(bf16))

    def unstage(r0, r1):
        return jnp.concatenate(_from_head_lanes(_groups(st_v[r0:r1, :])), axis=1)

    def out_proj(o, t0, side=None):
        a = _groups(_dot(o, wo_v[:, 0:D]))
        links = side(a) if side is not None else {}
        at = a_v.at[:, pl.ds(t0, o.shape[0] + 8), :]
        for g in range(NG):
            for rb in range(a[g].shape[0] // 8):
                v = a[g][rb * 8:(rb + 1) * 8]
                if rb == 0 and g in links:
                    v = _after(v, links[g])
                at[g, pl.ds((rb // 2) * 16 + rb % 2, 8, stride=2), :] = v

    def mod_vpu(j, part, nparts, dep):
        n = D // nparts
        acc = [None] * 2
        for i in range(n // 8):
            rows = slice(part * n + i * 8, part * n + (i + 1) * 8)
            cb = cb_v[rows, :]
            if i == 0:
                cb = _after(cb, dep)
            t = wl_v[j, rows, :].astype(f32) * jnp.concatenate([cb, cb], axis=1)
            acc[i % 2] = t if acc[i % 2] is None else acc[i % 2] + t
        return acc[0] + acc[1]

    def chunk_block(c, par, do_prep, do_mm, extra=None):
        zvec = zv_v[...]
        links = {}

        def link(ct, v):
            links[ct] = (links[ct] | v) if ct in links else v

        def rounds(hc, wp, rs, between=None):
            res = {}
            for k, r in enumerate(rs):
                out = _groups(_dot(hc, pltpu.bitcast(wp[:, r * 512:(r + 1) * 512], bf16)))
                for n in range(4):
                    res[4 * r + n] = out[n]
                if between is not None:
                    between(k)
            return res

        def accumulate(res):
            for ct in res:
                for t in range(SKEW):
                    blk = res[ct][t * T:(t + 1) * T]
                    if t == SKEW - 1 and ct in links:
                        blk = jnp.concatenate([blk[0:T - 8], _after(blk[T - 8:T], links.pop(ct) & zvec)], axis=0)
                    proj[t % 2][t // 2, ct, KOFF:KOFF + T, :] += blk
        mr = []

        def mods(k):
            for r in range(len(mr), 4):
                mr.append(mod_round(c + NG * (r // 2), r % 2))
        if do_prep:
            for cp in chunk_copies(c):
                cp.wait()
        if do_mm:
            res = rounds((he_v, ho_v)[1 - par][...], (wpe_v, wpo_v)[1 - par].at[(c - 1) >> 1], range(WR, 6),
                         mods if do_prep else None)
        if do_prep:
            mods(None)
            sh = mr[0] + mr[1]
            s1 = mr[2] + mr[3] + 1.0
            mod_v[c] = sh
            mod_v[NG + c] = s1
            hc = (xn_v[c].reshape(M0 // 8, 8, 128) * s1 + sh).reshape(M0, 128).astype(bf16)
            (he_v, ho_v)[par][...] = hc
            wp = (wpe_v, wpo_v)[par].at[c >> 1]
            for b in range(6):
                sec, half = b // 2, b % 2
                r0 = pl.multiple_of(c * KC + half * 64, 64)
                vs = _groups(_bits(wraw_v[pl.ds(r0, 64), sec * D:(sec + 1) * D]))
                vs = _to_head_lanes(vs)
                wp[half * 32:(half + 1) * 32, sec * D:(sec + 1) * D] = jnp.concatenate(vs, axis=1)
                if 2 * sec + 2 > WR:
                    link(8 + 3 * half, vs[NG - 1][24:32])
        if extra is not None:
            extra(res, link, zvec)
        if do_mm:
            accumulate(res)
        if do_prep:
            accumulate(rounds(hc, wp, range(WR)))

    def zero(ct, carry):
        for t in range(SKEW):
            proj[t % 2][t // 2, ct, KOFF:KOFF + T, :] = jnp.zeros((T, 128), f32)
        return carry
    lax.fori_loop(0, 3 * NG, zero, 0)
    copies["c"].wait()
    c32 = c_v[...].astype(f32)
    sc = (c32 * jax.nn.sigmoid(c32)).astype(bf16)
    sc_v[...] = jnp.broadcast_to(sc, (16, D))
    diag = lax.broadcasted_iota(jnp.int32, (128, 128), 0) == lax.broadcasted_iota(jnp.int32, (128, 128), 1)
    for g, row in enumerate(_groups(sc.astype(f32))):
        col = jnp.sum(jnp.where(diag, row, 0.0), axis=1, keepdims=True)
        cb_v[g * 128:(g + 1) * 128, :] = jnp.broadcast_to(col, (128, 128))
    copies["x0"].wait()

    def stats(i, carry):
        for rb in range(12):
            rows = pl.ds(pl.multiple_of(i * 96, 32) + rb * 8, 8)
            xn = _norm8(_groups(x_v[rows, :].astype(f32)))
            for g in range(NG):
                xn_v[g, rows, :] = xn[g]
        return carry
    lax.fori_loop(0, M0 // 96, stats, 0)
    chunk_block(0, 0, True, False)

    def kloop(i, carry):
        chunk_block(2 * i + 1, 1, True, True)

        @pl.when(2 * i + 2 < NKC)
        def _():
            chunk_block(2 * i + 2, 0, True, True)
        return carry
    lax.fori_loop(0, NKC // 2, kloop, 0)

    copies["x1"].wait()

    def ln_next(res, link, zvec):
        for rb in range(T // 8):
            ct = 4 * WR + (rb * (20 - 4 * WR)) // (T // 8)
            link(ct + 3, ln1_rows(x_v.at[M0:M0 + T, :], rb * 8, _bits(res[ct][M0 - 8:M0]) & zvec))
    chunk_block(NKC, 0, False, True, ln_next)
    for t in range(SKEW):
        for sg in range(NG, 3 * NG):
            if t == 0:
                halo = jnp.broadcast_to(p0_v[0, sg, KOFF:KOFF + 1, :], (HALO, 128))
            else:
                halo = proj[(t - 1) % 2][(t - 1) // 2, sg, KOFF + T - HALO:KOFF + T, :]
            proj[t % 2][t // 2, sg, KOFF - HALO:KOFF, :] = halo
    copies["x2"].wait()

    def step(s, par, first=False):
        GS, GA, GL, LL, UG = GATES["first" if first else par]
        jn = MPS * (s - MLAG)
        late = (s >= MLAG) & (jn < NL)
        zvec = zv_v[...]
        t0 = 0 if first else pl.multiple_of(s * T, T)
        slot = (s >> 1) & 1
        dst = proj[1 - par].at[((s + SKEW) >> 1) & 1]
        prev = proj[par].at[1 - slot]
        w = jnp.concatenate([(wpe_v, wpo_v)[c % 2][c // 2, :, 0:3 * D] for c in range(NKC)], axis=0)
        tiles = _groups(_dot(h_v[:, 0:D], pltpu.bitcast(w, bf16)))
        for ct in range(3 * NG):
            dst[ct, KOFF:KOFF + T, :] = tiles[ct]
            if ct >= NG:
                dst[ct, KOFF - HALO:KOFF, :] = prev[ct, KOFF + T - HALO:KOFF + T, :]
        t1 = (SKEW + 1) * T if first else pl.multiple_of(jnp.minimum(s + SKEW + 1, NT - 1) * T, T)
        src = proj[par].at[slot]
        links, rows = [], []

        def gate(pos):
            ct = int(pos)
            rb = min(T // 8 - 1, int((pos - ct) * (T // 8)))
            return _bits(tiles[ct][rb * 8:(rb + 1) * 8, :]) & zvec

        for pb in range(NP):
            halves = []
            for k in (2 * pb, 2 * pb + 1):
                d = gate(GA + GS * k / NRB)
                if k >= LL:
                    d = d | (links[k - LL] & zvec)
                halves.append(attn8(src, first, pb, k % 2, d))
            stage(pb, *halves)
            for rb in (2 * pb, 2 * pb + 1):
                links.append(ln1_rows(x_v.at[pl.ds(t1, T), :], rb * 8, gate(GA + GL + GS * rb / NRB)))
            if (pb + 1) % UG == 0:
                rows.append(pltpu.bitcast(unstage((pb + 1 - UG) * 8, (pb + 1) * 8), bf16))

        def mods(a):
            links = {}
            ev = tiles[3 * NG - 2:] + a
            for k in range(MPS):
                j = jnp.where(late, jn + k, NL)
                part = [mod_vpu(j, h, 4, _bits(ev[(7 * (4 * k + h)) // (4 * MPS)][T - 8:T]) & zvec) for h in range(4)]
                m = jnp.sum((part[0] + part[1]) + (part[2] + part[3]), axis=0, keepdims=True)
                m = jnp.broadcast_to(m + jnp.where(j >> 2 == 2, 1.0, 0.0), (8, 256))
                modr_v[2 * j] = m[:, 0:128]
                modr_v[2 * j + 1] = m[:, 128:256]
                links[min(4 * k + 5, NG - 1)] = _bits(m[:, 0:128]) & zvec
            if par == 0:
                for k in range(6):
                    seen = []
                    for sg in range(4 * k, 4 * k + 4):
                        lo = KOFF if sg < NG else KOFF - HALO
                        for r in range(lo, KOFF + T, 8):
                            v = p0_v[1, sg, r:r + 8, :]
                            if not seen:
                                v = _after(v, _bits(ev[k + 1][T - 8:T]) & zvec)
                            p1_v[2, sg, r:r + 8, :] = v
                            seen.append(_bits(v))
                    lk = functools.reduce(_or, seen) & zvec
                    links[k + 2] = (links[k + 2] | lk) if k + 2 in links else lk
            return links
        if first:
            copies["wo"].wait()
            out_proj(jnp.concatenate(rows, axis=0), t0)
        else:
            out_proj(jnp.concatenate(rows, axis=0), t0, mods)

    def phase_a(i, carry):
        @pl.when(i == 0)
        def _():
            copies["xr"].wait()

        @pl.when(2 * i + 1 == MLAG)
        def _():
            copies["wm"].wait()
        step(2 * i + 1, 1)

        @pl.when(i == NS // 2 - 1)
        def _():
            for n in ("w1", "w3", "w2"):
                copies[n].wait()
        step(2 * i + 2, 0)
        return carry
    step(0, 0, True)
    lax.fori_loop(0, NS // 2, phase_a, 0)

    def fill_window(i, sgs, dep):
        src = p1_v.at[(i // IPT) % 3, :, pl.ds(pl.multiple_of((i % IPT) * 16 * PPI, 16 * PPI), WROWS), :]
        seen = []
        for sg in sgs:
            lo = KOFF if sg < NG else KOFF - HALO
            v = src[sg, lo:WROWS, :]
            if not seen:
                v = jnp.concatenate([_after(v[0:8], dep), v[8:]], axis=0)
            win_v[sg, lo:WROWS, :] = v
            seen += [_bits(v[r:r + 8]) for r in range(0, WROWS - lo, 8)]
        return functools.reduce(_or, seen)

    fill_window(0, range(3 * NG), None)
    for rb in range(T // 8):
        ln2_rows(0, rb * 8, None)

    def out_copy(i, slot, half):
        cols = pl.ds(half * (D // 2), D // 2)
        return pltpu.make_async_copy(ob_v.at[slot, :, cols], out_hbm.at[0, pl.ds(pl.multiple_of(i * T, T), T), cols],
                                     osem.at[slot])

    def phase_b(i, carry):
        t1 = pl.multiple_of(jnp.minimum(i + 1, NT - 1) * T, T)
        slot = i & 1

        @pl.when(i >= 2)
        def _():
            for half in range(2):
                out_copy(i - 2, slot, half).wait()
        zvec = zv_v[...]
        sl = (i // IPT) % 3
        orow = jnp.where(sl == 0, 0, jnp.where(sl == 1, T, T // 2)) + (i % IPT) * 8 * PPI

        def fin(dep):
            o = unstage(0, 8 * PPI)
            o_v[pl.ds(pl.multiple_of(orow, 8 * PPI), 8 * PPI), :] = o
            return o[8 * PPI - 8:8 * PPI, D - 128:D]
        halves = []

        def att(n):
            def run(d):
                halves.append(attn8(win_v, False, n // 2, n % 2, d))
                if n % 2:
                    stage(n // 2, *halves[-2:])
                return _bits(halves[-1][NG - 1])
            return run
        ln = lambda r: (lambda d: ln2_rows(t1, r * 8, d))
        fw = lambda k: (lambda d: fill_window(i + 1, range(6 * k, 6 * k + 6), d))
        code = {"a": att, "f": lambda n: fin, "l": ln, "w": fw}
        cnt = dict.fromkeys(code, 0)
        side = []
        for chunk in FPLAN.split("/"):
            side.append([])
            for c in chunk:
                side[-1].append(code[c](cnt[c]))
                cnt[c] += 1
        assert cnt == {"a": 2 * PPI, "f": 1, "l": NRB, "w": 4}, cnt
        h = h2_v[:, 0:D]
        gb = jnp.concatenate([mcol(5, g) for g in range(NG)], axis=1)
        scaled = lambda y: (y.reshape(NRB, 8, D) * gb).reshape(T, D)
        acc = act_prev = None
        links = []
        for fc in range(NFC + 1):
            ev = []
            if fc < NFC:
                g = _dot(h, w1_v[:, fc * FC:(fc + 1) * FC])
                u = _dot(h, w3_v[:, fc * FC:(fc + 1) * FC])
                ev = _groups(g) + _groups(u)
                if 1 <= fc <= len(side):
                    u0 = _after(u[T - 8:T, FC - 128:FC], functools.reduce(_or, links[fc - 1]) & zvec)
                    u = jnp.concatenate([u[0:T - 8, :], jnp.concatenate([u[T - 8:T, 0:FC - 128], u0], axis=1)], axis=0)
                hg = 0.5 * g
                act = (hg * (1.0 + jnp.tanh(hg)) * u).astype(bf16)
            if fc >= 1:
                y = _dot(act_prev, w2_v[(fc - 1) * FC:fc * FC, 0:D])
                ev = ev + _groups(y)
                acc = (x1_v[...] if acc is None else acc) + scaled(y)
            if fc < len(side):
                n = len(side[fc])
                pos = [4 + (k * 12) // n if fc else 3 + (k * 5) // n for k in range(n)]
                links.append([fn(_bits(ev[p][T - 16:T - 8]) & zvec) for p, fn in zip(pos, side[fc])])
            act_prev = act
        for half in range(2):
            cols = slice(half * (D // 2), (half + 1) * (D // 2))
            ob_v[slot, :, cols] = acc[:, cols].astype(bf16)
            out_copy(i, slot, half).start()

        @pl.when(i == SKEW * IPT - 1)
        def _():
            out_proj(pltpu.bitcast(o_v[...], bf16), NS * T)
        return carry
    lax.fori_loop(0, NT, phase_b, 0)
    for half in range(2):
        out_copy(NT - 2, 0, half).wait()
    for half in range(2):
        out_copy(NT - 1, 1, half).wait()


@jax.jit
def pallas_adaLN_cond__sliding_local_dilated__glu_gated_swiglu__prompt_kernel(
    A_x, A_wqkv, A_wo, B_x, B_w1, B_w3, B_w2, c, w_mod):
    del B_x
    any_spec = pl.BlockSpec(memory_space=pl.ANY)
    return pl.pallas_call(
        _kernel,
        out_shape=jax.ShapeDtypeStruct((1, S, D), bf16),
        in_specs=[any_spec] * 8,
        out_specs=any_spec,
        scratch_shapes=[
            pltpu.VMEM((S, D), bf16),
            pltpu.VMEM((1, D), bf16),
            pltpu.VMEM((16, D), bf16),
            pltpu.VMEM((D, 128), f32),
            pltpu.VMEM((2 * NG, D, 128), bf16),
            pltpu.VMEM((NL + 1, D, 256), bf16),
            pltpu.VMEM((D, 3 * D), bf16),
            pltpu.VMEM((NKC // 2, KC // 2, 3 * D + PADW), u32),
            pltpu.VMEM((NKC // 2, KC // 2, 3 * D + PADW), u32),
            pltpu.VMEM((D, D + PADW), bf16),
            pltpu.VMEM((D, F + PADW), bf16),
            pltpu.VMEM((D, F + PADW), bf16),
            pltpu.VMEM((F, D + PADW), bf16),
            pltpu.VMEM((2 * NG, 8, 128), f32),
            pltpu.VMEM((2 * NL + 2, 8, 128), f32),
            pltpu.VMEM((NG, M0, 128), f32),
            pltpu.VMEM((M0, KC), bf16),
            pltpu.VMEM((M0, KC), bf16),
            pltpu.VMEM((T, D + PADW), bf16),
            pltpu.VMEM((T, D + PADW), bf16),
            pltpu.VMEM((T, D), f32),
            pltpu.VMEM((3 * NG, WROWS + 8, 128), f32),
            pltpu.VMEM((T // 2, D), u32),
            pltpu.VMEM((M0 // 2, D), u32),
            pltpu.VMEM((2, 3 * NG, KROWS, 128), f32),
            pltpu.VMEM((3, 3 * NG, KROWS, 128), f32),
            pltpu.VMEM((NG, S + 8, 128), f32),
            pltpu.VMEM((2, T, D), bf16),
            pltpu.VMEM((8, 128), u32),
            pltpu.SemaphoreType.DMA((10 + 2 * NKC,)),
            pltpu.SemaphoreType.DMA((2,)),
        ],
        compiler_params=pltpu.CompilerParams(vmem_limit_bytes=110 * 2**20, disable_bounds_checks=True,
                                             disable_semaphore_checks=True),
        name="adaln_fused",
    )(A_x, A_wqkv, A_wo, B_w1, B_w3, B_w2, c, w_mod)
```

```python
import functools

import jax
import jax.numpy as jnp
from jax import lax
import jax.experimental.pallas as pl
import jax.experimental.pallas.tpu as pltpu

S, D, F = 2048, 1024, 3584
DH, W, DIL = 32, 8, 2
NG = D // 128
HALO = 16
T = 128
NT = S // T
NP = T // 16
NRB = T // 8
SKEW = 3
M0 = SKEW * T
NS = NT - SKEW
NA = NS // 2
PPI = 2
IPT = NP // PPI
WROWS = HALO + 16 * PPI
FC = 512
NFC = F // FC
KOFF = HALO
KROWS = KOFF + T + 8
LOG2E = 1.4426950408889634
QSCALE = (DH ** -0.5) * LOG2E
NEG = -1e9 * DH ** 0.5
KC = 128
NKC = D // KC
WR = 4
LW = 512
NLP = 4 * D // LW
PADW = 128
EPS = 1e-5
GATES = {"first": (19.0, 0.5, 0.6, 6, 8), 1: (20.0, 0.0, 0.6, 4, 2), 0: (20.0, 0.7, 0.6, 4, 8)}
FPLAN = "aaa/all/flll/lwlll/lwlwl/lllwl"
f32, bf16, u32 = jnp.float32, jnp.bfloat16, jnp.uint32


def _butterfly(vs):
    vs = list(vs)
    lane = lax.broadcasted_iota(jnp.int32, vs[0].shape, 1)
    for s in range(3):
        m = (lane & (4 << s)) != 0
        for g in range(NG):
            if g & (1 << s):
                continue
            a, b = vs[g], vs[g | (1 << s)]
            vs[g] = jnp.where(m, b, a)
            vs[g | (1 << s)] = jnp.where(m, a, b)
    return vs


def _to_head_lanes(vs):
    ys = _butterfly(vs)
    lane = lax.broadcasted_iota(jnp.int32, vs[0].shape, 1)
    head = lane & 31
    out = []
    for g in range(NG):
        src = ((head & 3) << 5) | (((head >> 2) ^ g) << 2) | (lane >> 5)
        out.append(jnp.take_along_axis(ys[g], src, axis=1))
    return out


def _from_head_lanes(zs):
    lane = lax.broadcasted_iota(jnp.int32, zs[0].shape, 1)
    ys = []
    for g in range(NG):
        src = ((lane & 3) << 5) | ((((lane >> 2) & 7) ^ g) << 2) | (lane >> 5)
        ys.append(jnp.take_along_axis(zs[g], src, axis=1))
    return _butterfly(ys)


def _add(a, b):
    return a + b


def _or(a, b):
    return a | b


def _bits(x):
    return pltpu.bitcast(x, u32)


def _dot(a, b):
    return jnp.dot(a, b, preferred_element_type=f32)


def _after(x, dep):
    if dep is None:
        return x
    return pltpu.bitcast(_bits(x) | dep, x.dtype)


def _norm8(xs, dep=None):
    xs = [_after(xs[0], dep)] + list(xs[1:])
    m = jnp.sum(functools.reduce(_add, xs), axis=-1, keepdims=True) * (1.0 / D)
    xc = [v - m for v in xs]
    var = jnp.sum(functools.reduce(_add, [v * v for v in xc]), axis=-1, keepdims=True) * (1.0 / D)
    r = lax.rsqrt(var + EPS)
    return [v * r for v in xc]


def _groups(x):
    return [x[:, g * 128:(g + 1) * 128] for g in range(x.shape[1] // 128)]


def _kernel(x_hbm, wqkv_hbm, wo_hbm, w1_hbm, w3_hbm, w2_hbm, c_hbm, wmod_hbm, out_hbm,
            x_v, c_v, sc_v, cb_v, wm_v, wl0_v, wl1_v, wraw_v, wpe_v, wpo_v, wo_v, w1_v, w3_v, w2_v, mod_v, modr_v,
            xn_v, he_v, ho_v, h_v, h2_v, x1_v, win_v, st_v, o_v, p0_v, p1_v, a_v, ob_v,
            zv_v, sem, osem):
    names = ["c", "x0", "x1", "x2", "x3", "xr", "wo", "w1", "w3", "w2", "wl0", "wl1"]
    srcdst = dict(
        c=(c_hbm, c_v),
        x0=(x_hbm.at[0, 0:M0, :], x_v.at[0:M0, :]),
        x1=(x_hbm.at[0, M0:M0 + T, :], x_v.at[M0:M0 + T, :]),
        x2=(x_hbm.at[0, M0 + T:M0 + 2 * T, :], x_v.at[M0 + T:M0 + 2 * T, :]),
        x3=(x_hbm.at[0, M0 + 2 * T:M0 + 3 * T, :], x_v.at[M0 + 2 * T:M0 + 3 * T, :]),
        xr=(x_hbm.at[0, M0 + 3 * T:S, :], x_v.at[M0 + 3 * T:S, :]),
        wo=(wo_hbm, wo_v.at[:, 0:D]),
        w1=(w1_hbm, w1_v.at[:, 0:F]), w3=(w3_hbm, w3_v.at[:, 0:F]), w2=(w2_hbm, w2_v.at[:, 0:D]),
    )
    copies = {n: pltpu.make_async_copy(*srcdst[n], sem.at[names.index(n)]) for n in srcdst}
    SEM_C = len(names)
    SEM_W = SEM_C + NKC

    def slab_copy(j, s):
        return pltpu.make_async_copy(wmod_hbm.at[:, pl.ds(pl.multiple_of(j * 128, 128), 128)], wm_v.at[j], sem.at[s])

    def chunk_copies(c):
        rows = pl.ds(pl.multiple_of(c * KC, KC), KC)
        return [slab_copy(c, SEM_C + c), slab_copy(NG + c, SEM_C + c),
                pltpu.make_async_copy(wqkv_hbm.at[rows, :], wraw_v.at[rows, :], sem.at[SEM_W + c])]

    def late_copy(p, par):
        cols = pl.ds(pl.multiple_of(2 * D + p * LW, LW), LW)
        return pltpu.make_async_copy(wmod_hbm.at[:, cols], (wl0_v, wl1_v)[par], sem.at[names.index("wl0") + par])

    copies["c"].start()
    copies["x0"].start()
    for c in range(NKC):
        for cp in chunk_copies(c):
            cp.start()
    for n in ("x1", "x2", "wo", "x3"):
        copies[n].start()
    late_copy(0, 1).start()
    late_copy(1, 0).start()
    copies["xr"].start()
    for n in ("w1", "w3", "w2"):
        copies[n].start(priority=1)
    zv_v[...] = jnp.zeros(zv_v.shape, u32)

    proj = (p0_v, p1_v)
    mcol = lambda sec, g: mod_v[sec * NG + g] if sec < 2 else modr_v[(sec - 2) * NG + g]
    row8 = lax.broadcasted_iota(jnp.int32, (8, 128), 0)

    def mod_round(j, kh):
        ks = slice(kh * 512, (kh + 1) * 512)
        return _dot(sc_v[:, ks], wm_v[j, ks, :])[0:8]

    def ln1_rows(xt, drow, dep):
        xn = _norm8(_groups(xt[drow:drow + 8, :].astype(f32)), dep)
        ys = [xn[g] * mcol(1, g) + mcol(0, g) for g in range(NG)]
        h_v[drow:drow + 8, 0:D] = jnp.concatenate(ys, axis=1).astype(bf16)
        return _bits(ys[NG - 1])

    def ln2_rows(t, drow, dep):
        xt, at = x_v.at[pl.ds(t, T), :], a_v.at[:, pl.ds(t, T), :]
        x = _groups(xt[drow:drow + 8, :].astype(f32))
        x1 = [x[g] + mcol(2, g) * at[g, drow:drow + 8, :] for g in range(NG)]
        x1_v[drow:drow + 8, :] = jnp.concatenate(x1, axis=1)
        xn = _norm8(x1, dep)
        ys = [xn[g] * mcol(4, g) + mcol(3, g) for g in range(NG)]
        h2_v[drow:drow + 8, 0:D] = jnp.concatenate(ys, axis=1).astype(bf16)
        return _bits(ys[NG - 1])

    def attn8(src, masked, pb, par, dep):
        r0 = KOFF + 16 * pb + par
        rows = lambda j: pl.ds(r0 - DIL * j, 8, stride=DIL)
        zvec = zv_v[...]
        s = [None] * W
        for g in range(NG):
            q = src[g, rows(0), :]
            if g == 0:
                q = _after(q, dep)
            else:
                q = _after(q, _bits(s[W - 1]) & zvec)
            for j in range(W):
                p = q * src[NG + g, rows(j), :]
                s[j] = p if s[j] is None else s[j] + p
        for j in range(W):
            s[j] = s[j] + pltpu.roll(s[j], 64, 1)
            s[j] = s[j] + pltpu.roll(s[j], 32, 1)
            if masked and pb == 0 and j > 0:
                s[j] = jnp.where(par + DIL * row8 >= DIL * j, s[j], NEG)
        m = functools.reduce(jnp.maximum, s)
        e = [jnp.exp2((s[j] - m) * QSCALE) for j in range(W)]
        den = functools.reduce(_add, e)
        r = pl.reciprocal(den, approx=True)
        inv = r * (2.0 - den * r)
        og = [None] * NG
        for j in range(W):
            p = e[j] * inv
            if j:
                p = _after(p, _bits(og[NG - 1]) & zvec)
            for g in range(NG):
                t = p * src[2 * NG + g, rows(j), :]
                og[g] = t if og[g] is None else og[g] + t
        return og

    def stage(pb, even, odd):
        for g in range(NG):
            st_v[8 * pb:8 * pb + 8, g * 128:(g + 1) * 128] = _bits(
                jnp.concatenate([even[g], odd[g]], axis=0).astype(bf16))

    def unstage(r0, r1):
        return jnp.concatenate(_from_head_lanes(_groups(st_v[r0:r1, :])), axis=1)

    def out_proj(o, t0, side=None):
        a = _groups(_dot(o, wo_v[:, 0:D]))
        links = side(a) if side is not None else {}
        at = a_v.at[:, pl.ds(t0, o.shape[0] + 8), :]
        for g in range(NG):
            for rb in range(a[g].shape[0] // 8):
                v = a[g][rb * 8:(rb + 1) * 8]
                if rb == 0 and g in links:
                    v = _after(v, links[g])
                at[g, pl.ds((rb // 2) * 16 + rb % 2, 8, stride=2), :] = v

    def mod_vpu(wl, k, half, dep):
        zvec = zv_v[...]
        acc = None
        for i in range(D // 16):
            rows = slice(half * (D // 2) + i * 8, half * (D // 2) + (i + 1) * 8)
            cb = cb_v[rows, :]
            if i % 4 == 0:
                cb = _after(cb, dep if i == 0 else _bits(acc[:, 0:128]) & zvec)
            t = wl[rows, k * 256:(k + 1) * 256].astype(f32) * jnp.concatenate([cb, cb], axis=1)
            acc = t if acc is None else acc + t
        return acc

    def chunk_block(c, par, do_prep, do_mm, extra=None):
        zvec = zv_v[...]
        links = {}

        def link(ct, v):
            links[ct] = (links[ct] | v) if ct in links else v

        def rounds(hc, wp, rs, between=None):
            res = {}
            for k, r in enumerate(rs):
                out = _groups(_dot(hc, pltpu.bitcast(wp[:, r * 512:(r + 1) * 512], bf16)))
                for n in range(4):
                    res[4 * r + n] = out[n]
                if between is not None:
                    between(k)
            return res

        def accumulate(res):
            for ct in res:
                for t in range(SKEW):
                    blk = res[ct][t * T:(t + 1) * T]
                    if t == SKEW - 1 and ct in links:
                        blk = jnp.concatenate([blk[0:T - 8], _after(blk[T - 8:T], links.pop(ct) & zvec)], axis=0)
                    proj[t % 2][t // 2, ct, KOFF:KOFF + T, :] += blk
        mr = []

        def mods(k):
            for r in range(len(mr), 4):
                mr.append(mod_round(c + NG * (r // 2), r % 2))
        if do_prep:
            for cp in chunk_copies(c):
                cp.wait()
        if do_mm:
            res = rounds((he_v, ho_v)[1 - par][...], (wpe_v, wpo_v)[1 - par].at[(c - 1) >> 1], range(WR, 6),
                         mods if do_prep else None)
        if do_prep:
            mods(None)
            sh = mr[0] + mr[1]
            s1 = mr[2] + mr[3] + 1.0
            mod_v[c] = sh
            mod_v[NG + c] = s1
            hc = (xn_v[c].reshape(M0 // 8, 8, 128) * s1 + sh).reshape(M0, 128).astype(bf16)
            (he_v, ho_v)[par][...] = hc
            wp = (wpe_v, wpo_v)[par].at[c >> 1]
            for b in range(6):
                sec, half = b // 2, b % 2
                r0 = pl.multiple_of(c * KC + half * 64, 64)
                vs = _groups(_bits(wraw_v[pl.ds(r0, 64), sec * D:(sec + 1) * D]))
                vs = _to_head_lanes(vs)
                wp[half * 32:(half + 1) * 32, sec * D:(sec + 1) * D] = jnp.concatenate(vs, axis=1)
                if 2 * sec + 2 > WR:
                    link(8 + 3 * half, vs[NG - 1][24:32])
        if extra is not None:
            extra(res, link, zvec)
        if do_mm:
            accumulate(res)
        if do_prep:
            accumulate(rounds(hc, wp, range(WR)))

    def zero(ct, carry):
        for t in range(SKEW):
            proj[t % 2][t // 2, ct, KOFF:KOFF + T, :] = jnp.zeros((T, 128), f32)
        return carry
    lax.fori_loop(0, 3 * NG, zero, 0)
    copies["c"].wait()
    c32 = c_v[...].astype(f32)
    sc = (c32 * jax.nn.sigmoid(c32)).astype(bf16)
    sc_v[...] = jnp.broadcast_to(sc, (16, D))
    diag = lax.broadcasted_iota(jnp.int32, (128, 128), 0) == lax.broadcasted_iota(jnp.int32, (128, 128), 1)
    for g, row in enumerate(_groups(sc.astype(f32))):
        col = jnp.sum(jnp.where(diag, row, 0.0), axis=1, keepdims=True)
        cb_v[g * 128:(g + 1) * 128, :] = jnp.broadcast_to(col, (128, 128))
    copies["x0"].wait()

    def stats(i, carry):
        for rb in range(12):
            rows = pl.ds(pl.multiple_of(i * 96, 32) + rb * 8, 8)
            xn = _norm8(_groups(x_v[rows, :].astype(f32)))
            for g in range(NG):
                xn_v[g, rows, :] = xn[g]
        return carry
    lax.fori_loop(0, M0 // 96, stats, 0)
    chunk_block(0, 0, True, False)

    def kloop(i, carry):
        chunk_block(2 * i + 1, 1, True, True)

        @pl.when(2 * i + 2 < NKC)
        def _():
            chunk_block(2 * i + 2, 0, True, True)
        return carry
    lax.fori_loop(0, NKC // 2, kloop, 0)

    copies["x1"].wait()

    def ln_next(res, link, zvec):
        for rb in range(T // 8):
            ct = 4 * WR + (rb * (20 - 4 * WR)) // (T // 8)
            link(ct + 3, ln1_rows(x_v.at[M0:M0 + T, :], rb * 8, _bits(res[ct][M0 - 8:M0]) & zvec))
    chunk_block(NKC, 0, False, True, ln_next)
    for t in range(SKEW):
        for sg in range(NG, 3 * NG):
            if t == 0:
                halo = jnp.broadcast_to(p0_v[0, sg, KOFF:KOFF + 1, :], (HALO, 128))
            else:
                halo = proj[(t - 1) % 2][(t - 1) // 2, sg, KOFF + T - HALO:KOFF + T, :]
            proj[t % 2][t // 2, sg, KOFF - HALO:KOFF, :] = halo
    copies["x2"].wait()

    def step(s, par, first=False):
        GS, GA, GL, LL, UG = GATES["first" if first else par]
        piece = jnp.minimum(s - 1, NLP - 1 - par)
        zvec = zv_v[...]
        t0 = 0 if first else pl.multiple_of(s * T, T)
        slot = (s >> 1) & 1
        dst = proj[1 - par].at[((s + SKEW) >> 1) & 1]
        prev = proj[par].at[1 - slot]
        w = jnp.concatenate([(wpe_v, wpo_v)[c % 2][c // 2, :, 0:3 * D] for c in range(NKC)], axis=0)
        tiles = _groups(_dot(h_v[:, 0:D], pltpu.bitcast(w, bf16)))
        for ct in range(3 * NG):
            dst[ct, KOFF:KOFF + T, :] = tiles[ct]
            if ct >= NG:
                dst[ct, KOFF - HALO:KOFF, :] = prev[ct, KOFF + T - HALO:KOFF + T, :]
        t1 = (SKEW + 1) * T if first else pl.multiple_of(jnp.minimum(s + SKEW + 1, NT - 1) * T, T)
        src = proj[par].at[slot]
        links, rows = [], []

        def gate(pos):
            ct = int(pos)
            rb = min(T // 8 - 1, int((pos - ct) * (T // 8)))
            return _bits(tiles[ct][rb * 8:(rb + 1) * 8, :]) & zvec

        for pb in range(NP):
            halves = []
            for k in (2 * pb, 2 * pb + 1):
                d = gate(GA + GS * k / NRB)
                if k >= LL:
                    d = d | (links[k - LL] & zvec)
                halves.append(attn8(src, first, pb, k % 2, d))
            stage(pb, *halves)
            for rb in (2 * pb, 2 * pb + 1):
                links.append(ln1_rows(x_v.at[pl.ds(t1, T), :], rb * 8, gate(GA + GL + GS * rb / NRB)))
            if (pb + 1) % UG == 0:
                rows.append(pltpu.bitcast(unstage((pb + 1 - UG) * 8, (pb + 1) * 8), bf16))

        def side(a):
            links = {}
            ev = tiles[3 * NG - 2:] + a
            for k in range(LW // 256):
                part = [mod_vpu((wl0_v, wl1_v)[par], k, h, _bits(ev[(7 * (2 * k + h)) // 4][T - 8:T]) & zvec)
                        for h in range(2)]
                m = jnp.sum(part[0] + part[1], axis=0, keepdims=True)
                m = jnp.broadcast_to(m + jnp.where(piece >> 1 == 2, 1.0, 0.0), (8, 256))
                modr_v[4 * piece + 2 * k] = m[:, 0:128]
                modr_v[4 * piece + 2 * k + 1] = m[:, 128:256]
                links[5 + 2 * k] = _bits(m[:, 0:128]) & zvec
            if par == 0:
                for k in range(6):
                    seen = []
                    for sg in range(4 * k, 4 * k + 4):
                        lo = KOFF if sg < NG else KOFF - HALO
                        for r in range(lo, KOFF + T, 8):
                            v = p0_v[1, sg, r:r + 8, :]
                            if not seen:
                                v = _after(v, _bits(ev[k + 1][T - 8:T]) & zvec)
                            p1_v[2, sg, r:r + 8, :] = v
                            seen.append(_bits(v))
                    lk = functools.reduce(_or, seen) & zvec
                    links[k + 2] = (links[k + 2] | lk) if k + 2 in links else lk
            return links
        if first:
            copies["wo"].wait()
            out_proj(jnp.concatenate(rows, axis=0), t0)
        else:
            out_proj(jnp.concatenate(rows, axis=0), t0, side)

            @pl.when(s + 1 < NLP)
            def _():
                late_copy(s + 1, par).start()

    def phase_a(i):
        @pl.when(i == 0)
        def _():
            copies["x3"].wait()

        @pl.when(2 * i < NLP)
        def _():
            late_copy(2 * i, 1).wait()
        step(2 * i + 1, 1)

        @pl.when(i == 0)
        def _():
            copies["xr"].wait()

        @pl.when(2 * i + 1 < NLP)
        def _():
            late_copy(2 * i + 1, 0).wait()
        step(2 * i + 2, 0)

        @pl.when(i == NA - 1)
        def _():
            for n in ("w1", "w3", "w2"):
                copies[n].wait()
            fill_window(0, range(3 * NG), None)
            for rb in range(NRB):
                ln2_rows(0, rb * 8, None)

    def fill_window(i, sgs, dep):
        src = p1_v.at[(i // IPT) % 3, :, pl.ds(pl.multiple_of((i % IPT) * 16 * PPI, 16 * PPI), WROWS), :]
        seen = []
        for sg in sgs:
            lo = KOFF if sg < NG else KOFF - HALO
            v = src[sg, lo:WROWS, :]
            if not seen:
                v = jnp.concatenate([_after(v[0:8], dep), v[8:]], axis=0)
            win_v[sg, lo:WROWS, :] = v
            seen += [_bits(v[r:r + 8]) for r in range(0, WROWS - lo, 8)]
        return functools.reduce(_or, seen)

    def phase_b(i):
        i = i - NA
        t1 = pl.multiple_of(jnp.minimum(i + 1, NT - 1) * T, T)
        zvec = zv_v[...]
        sl = (i // IPT) % 3
        orow = jnp.where(sl == 0, 0, jnp.where(sl == 1, T, T // 2)) + (i % IPT) * 8 * PPI

        def fin(dep):
            o = unstage(0, 8 * PPI)
            o_v[pl.ds(pl.multiple_of(orow, 8 * PPI), 8 * PPI), :] = o
            return o[8 * PPI - 8:8 * PPI, D - 128:D]
        halves = []

        def att(n):
            def run(d):
                halves.append(attn8(win_v, False, n // 2, n % 2, d))
                if n % 2:
                    stage(n // 2, *halves[-2:])
                return _bits(halves[-1][NG - 1])
            return run
        ln = lambda r: (lambda d: ln2_rows(t1, r * 8, d))
        fw = lambda k: (lambda d: fill_window(i + 1, range(6 * k, 6 * k + 6), d))
        code = {"a": att, "f": lambda n: fin, "l": ln, "w": fw}
        cnt = dict.fromkeys(code, 0)
        side = []
        for chunk in FPLAN.split("/"):
            side.append([])
            for c in chunk:
                side[-1].append(code[c](cnt[c]))
                cnt[c] += 1
        assert cnt == {"a": 2 * PPI, "f": 1, "l": NRB, "w": 4}, cnt
        h = h2_v[:, 0:D]
        gb = jnp.concatenate([mcol(5, g) for g in range(NG)], axis=1)
        scaled = lambda y: (y.reshape(NRB, 8, D) * gb).reshape(T, D)
        acc = act_prev = None
        links = []
        for fc in range(NFC + 1):
            ev = []
            if fc < NFC:
                g = _dot(h, w1_v[:, fc * FC:(fc + 1) * FC])
                u = _dot(h, w3_v[:, fc * FC:(fc + 1) * FC])
                ev = _groups(g) + _groups(u)
                if 1 <= fc <= len(side):
                    u0 = _after(u[T - 8:T, FC - 128:FC], functools.reduce(_or, links[fc - 1]) & zvec)
                    u = jnp.concatenate([u[0:T - 8, :], jnp.concatenate([u[T - 8:T, 0:FC - 128], u0], axis=1)], axis=0)
                hg = 0.5 * g
                act = (hg * (1.0 + jnp.tanh(hg)) * u).astype(bf16)
            if fc >= 1:
                y = _dot(act_prev, w2_v[(fc - 1) * FC:fc * FC, 0:D])
                ev = ev + _groups(y)
                acc = (x1_v[...] if acc is None else acc) + scaled(y)
            if fc < len(side):
                n = len(side[fc])
                pos = [4 + (k * 12) // n if fc else 3 + (k * 5) // n for k in range(n)]
                links.append([fn(_bits(ev[p][T - 16:T - 8]) & zvec) for p, fn in zip(pos, side[fc])])
            act_prev = act
        rows = pl.ds(pl.multiple_of(i * T, T), T)
        for half in range(2):
            cols = slice(half * (D // 2), (half + 1) * (D // 2))
            ob_v[rows, cols] = acc[:, cols].astype(bf16)
            pltpu.make_async_copy(ob_v.at[rows, cols], out_hbm.at[0, rows, cols], osem.at[0]).start()

        @pl.when(i == SKEW * IPT - 1)
        def _():
            out_proj(pltpu.bitcast(o_v[...], bf16), NS * T)

    def main(i, carry):
        lax.cond(i < NA, phase_a, phase_b, i)
        return carry
    step(0, 0, True)
    lax.fori_loop(0, NA + NT, main, 0)
    pltpu.make_async_copy(ob_v, out_hbm.at[0], osem.at[0]).wait()


@jax.jit
def pallas_adaLN_cond__sliding_local_dilated__glu_gated_swiglu__prompt_kernel(
    A_x, A_wqkv, A_wo, B_x, B_w1, B_w3, B_w2, c, w_mod):
    del B_x
    any_spec = pl.BlockSpec(memory_space=pl.ANY)
    return pl.pallas_call(
        _kernel,
        out_shape=jax.ShapeDtypeStruct((1, S, D), bf16),
        in_specs=[any_spec] * 8,
        out_specs=any_spec,
        scratch_shapes=[
            pltpu.VMEM((S, D), bf16),
            pltpu.VMEM((1, D), bf16),
            pltpu.VMEM((16, D), bf16),
            pltpu.VMEM((D, 128), f32),
            pltpu.VMEM((2 * NG, D, 128), bf16),
            pltpu.VMEM((D, LW), bf16),
            pltpu.VMEM((D, LW), bf16),
            pltpu.VMEM((D, 3 * D), bf16),
            pltpu.VMEM((NKC // 2, KC // 2, 3 * D + PADW), u32),
            pltpu.VMEM((NKC // 2, KC // 2, 3 * D + PADW), u32),
            pltpu.VMEM((D, D + PADW), bf16),
            pltpu.VMEM((D, F + PADW), bf16),
            pltpu.VMEM((D, F + PADW), bf16),
            pltpu.VMEM((F, D + PADW), bf16),
            pltpu.VMEM((2 * NG, 8, 128), f32),
            pltpu.VMEM((4 * NG, 8, 128), f32),
            pltpu.VMEM((NG, M0, 128), f32),
            pltpu.VMEM((M0, KC), bf16),
            pltpu.VMEM((M0, KC), bf16),
            pltpu.VMEM((T, D + PADW), bf16),
            pltpu.VMEM((T, D + PADW), bf16),
            pltpu.VMEM((T, D), f32),
            pltpu.VMEM((3 * NG, WROWS + 8, 128), f32),
            pltpu.VMEM((T // 2, D), u32),
            pltpu.VMEM((M0 // 2, D), u32),
            pltpu.VMEM((2, 3 * NG, KROWS, 128), f32),
            pltpu.VMEM((3, 3 * NG, KROWS, 128), f32),
            pltpu.VMEM((NG, S + 8, 128), f32),
            pltpu.VMEM((S, D), bf16),
            pltpu.VMEM((8, 128), u32),
            pltpu.SemaphoreType.DMA((12 + 2 * NKC,)),
            pltpu.SemaphoreType.DMA((1,)),
        ],
        compiler_params=pltpu.CompilerParams(vmem_limit_bytes=110 * 2**20, disable_bounds_checks=True,
                                             disable_semaphore_checks=True),
        name="adaln_fused",
    )(A_x, A_wqkv, A_wo, B_w1, B_w3, B_w2, c, w_mod)
```

```python
import functools

import jax
import jax.numpy as jnp
from jax import lax
import jax.experimental.pallas as pl
import jax.experimental.pallas.tpu as pltpu

S, D, F = 2048, 1024, 3584
DH, W, DIL = 32, 8, 2
NG = D // 128
HALO = 16
T = 128
NT = S // T
NP = T // 16
NRB = T // 8
SKEW = 3
M0 = SKEW * T
NS = NT - SKEW
NA = NS // 2
PPI = 2
IPT = NP // PPI
WROWS = HALO + 16 * PPI
FC = 512
NFC = F // FC
KOFF = HALO
KROWS = KOFF + T + 8
LOG2E = 1.4426950408889634
QSCALE = (DH ** -0.5) * LOG2E
NEG = -1e9 * DH ** 0.5
KC = 128
NKC = D // KC
WR = 4
LW = 512
NLP = 4 * D // LW
PADW = 128
EPS = 1e-5
GATES = {"first": (19.0, 0.5, 0.6, 6, 8), 1: (20.0, 0.0, 0.6, 4, 2), 0: (20.0, 0.7, 0.6, 4, 8)}
FPLAN = "aaa/all/flll/lwlll/lwlwl/lllwl"
f32, bf16, u32 = jnp.float32, jnp.bfloat16, jnp.uint32


def _lane_tables():
    lane = lax.broadcasted_iota(jnp.int32, (8, 128), 1)
    head = lane & 31
    masks = [(lane & (4 << s)) != 0 for s in range(3)]
    fwd = [((head & 3) << 5) | (((head >> 2) ^ g) << 2) | (lane >> 5) for g in range(NG)]
    inv = [((lane & 3) << 5) | ((((lane >> 2) & 7) ^ g) << 2) | (lane >> 5) for g in range(NG)]
    return masks, fwd, inv


def _butterfly(vs, masks):
    n = vs[0].shape[0] // 8
    vs = [v.reshape(n, 8, 128) for v in vs]
    for s in range(3):
        for g in range(NG):
            if g & (1 << s):
                continue
            a, b = vs[g], vs[g | (1 << s)]
            vs[g] = jnp.where(masks[s], b, a)
            vs[g | (1 << s)] = jnp.where(masks[s], a, b)
    return [v.reshape(n * 8, 128) for v in vs]


def _gather_lanes(v, idx):
    idx = jnp.concatenate([idx] * (v.shape[0] // 8), axis=0)
    return jnp.take_along_axis(v, idx, axis=1, mode="promise_in_bounds")


def _to_head_lanes(vs, tabs):
    return [_gather_lanes(y, i) for y, i in zip(_butterfly(vs, tabs[0]), tabs[1])]


def _from_head_lanes(zs, tabs):
    return _butterfly([_gather_lanes(z, i) for z, i in zip(zs, tabs[2])], tabs[0])


def _add(a, b):
    return a + b


def _or(a, b):
    return a | b


def _bits(x):
    return pltpu.bitcast(x, u32)


def _dot(a, b):
    return jnp.dot(a, b, preferred_element_type=f32)


def _after(x, dep):
    if dep is None:
        return x
    return pltpu.bitcast(_bits(x) | dep, x.dtype)


def _norm8(xs, dep=None):
    xs = [_after(xs[0], dep)] + list(xs[1:])
    m = jnp.sum(functools.reduce(_add, xs), axis=-1, keepdims=True) * (1.0 / D)
    xc = [v - m for v in xs]
    var = jnp.sum(functools.reduce(_add, [v * v for v in xc]), axis=-1, keepdims=True) * (1.0 / D)
    r = lax.rsqrt(var + EPS)
    return [v * r for v in xc]


def _groups(x):
    return [x[:, g * 128:(g + 1) * 128] for g in range(x.shape[1] // 128)]


def _kernel(x_hbm, wqkv_hbm, wo_hbm, w1_hbm, w3_hbm, w2_hbm, c_hbm, wmod_hbm, out_hbm,
            x_v, c_v, sc_v, cb_v, wm_v, wl0_v, wl1_v, wraw_v, wpe_v, wpo_v, wo_v, w1_v, w3_v, w2_v, mod_v, modr_v,
            xn_v, he_v, ho_v, h_v, h2_v, x1_v, win_v, st_v, o_v, p0_v, p1_v, a_v, ob_v,
            zv_v, sem, osem):
    names = ["c", "x0", "x1", "x2", "x3", "xr", "wo", "w1", "w3", "w2", "wl0", "wl1"]
    srcdst = dict(
        c=(c_hbm, c_v),
        x0=(x_hbm.at[0, 0:M0, :], x_v.at[0:M0, :]),
        x1=(x_hbm.at[0, M0:M0 + T, :], x_v.at[M0:M0 + T, :]),
        x2=(x_hbm.at[0, M0 + T:M0 + 2 * T, :], x_v.at[M0 + T:M0 + 2 * T, :]),
        x3=(x_hbm.at[0, M0 + 2 * T:M0 + 3 * T, :], x_v.at[M0 + 2 * T:M0 + 3 * T, :]),
        xr=(x_hbm.at[0, M0 + 3 * T:S, :], x_v.at[M0 + 3 * T:S, :]),
        wo=(wo_hbm, wo_v.at[:, 0:D]),
        w1=(w1_hbm, w1_v.at[:, 0:F]), w3=(w3_hbm, w3_v.at[:, 0:F]), w2=(w2_hbm, w2_v.at[:, 0:D]),
    )
    copies = {n: pltpu.make_async_copy(*srcdst[n], sem.at[names.index(n)]) for n in srcdst}
    SEM_C = len(names)
    SEM_W = SEM_C + NKC

    def slab_copy(j, s):
        return pltpu.make_async_copy(wmod_hbm.at[:, pl.ds(pl.multiple_of(j * 128, 128), 128)], wm_v.at[j], sem.at[s])

    def chunk_copies(c):
        rows = pl.ds(pl.multiple_of(c * KC, KC), KC)
        return [slab_copy(c, SEM_C + c), slab_copy(NG + c, SEM_C + c),
                pltpu.make_async_copy(wqkv_hbm.at[rows, :], wraw_v.at[rows, :], sem.at[SEM_W + c])]

    def late_copy(p, par):
        cols = pl.ds(pl.multiple_of(2 * D + p * LW, LW), LW)
        return pltpu.make_async_copy(wmod_hbm.at[:, cols], (wl0_v, wl1_v)[par], sem.at[names.index("wl0") + par])

    copies["c"].start()
    copies["x0"].start()
    for c in range(NKC):
        for cp in chunk_copies(c):
            cp.start()
    for n in ("x1", "x2", "wo", "x3"):
        copies[n].start()
    late_copy(0, 1).start()
    late_copy(1, 0).start()
    copies["xr"].start()
    for n in ("w1", "w3", "w2"):
        copies[n].start(priority=1)
    zv_v[...] = jnp.zeros(zv_v.shape, u32)

    tabs = _lane_tables()
    proj = (p0_v, p1_v)
    mcol = lambda sec, g: mod_v[sec * NG + g] if sec < 2 else modr_v[(sec - 2) * NG + g]
    row8 = lax.broadcasted_iota(jnp.int32, (8, 128), 0)

    def mod_round(j, kh):
        ks = slice(kh * 512, (kh + 1) * 512)
        return _dot(sc_v[:, ks], wm_v[j, ks, :])[0:8]

    def ln1_rows(xt, drow, dep):
        xn = _norm8(_groups(xt[drow:drow + 8, :].astype(f32)), dep)
        ys = [xn[g] * mcol(1, g) + mcol(0, g) for g in range(NG)]
        h_v[drow:drow + 8, 0:D] = jnp.concatenate(ys, axis=1).astype(bf16)
        return _bits(ys[NG - 1])

    def ln2_rows(t, drow, dep):
        xt, at = x_v.at[pl.ds(t, T), :], a_v.at[:, pl.ds(t, T), :]
        x = _groups(xt[drow:drow + 8, :].astype(f32))
        x1 = [x[g] + mcol(2, g) * at[g, drow:drow + 8, :] for g in range(NG)]
        x1_v[drow:drow + 8, :] = jnp.concatenate(x1, axis=1)
        xn = _norm8(x1, dep)
        ys = [xn[g] * mcol(4, g) + mcol(3, g) for g in range(NG)]
        h2_v[drow:drow + 8, 0:D] = jnp.concatenate(ys, axis=1).astype(bf16)
        return _bits(ys[NG - 1])

    def attn8(src, masked, pb, par, dep):
        r0 = KOFF + 16 * pb + par
        rows = lambda j: pl.ds(r0 - DIL * j, 8, stride=DIL)
        zvec = zv_v[...]
        s = [None] * W
        for g in range(NG):
            q = src[g, rows(0), :]
            if g == 0:
                q = _after(q, dep)
            else:
                q = _after(q, _bits(s[W - 1]) & zvec)
            for j in range(W):
                p = q * src[NG + g, rows(j), :]
                s[j] = p if s[j] is None else s[j] + p
        for j in range(W):
            s[j] = s[j] + pltpu.roll(s[j], 64, 1)
            s[j] = s[j] + pltpu.roll(s[j], 32, 1)
            if masked and pb == 0 and j > 0:
                s[j] = jnp.where(par + DIL * row8 >= DIL * j, s[j], NEG)
        m = functools.reduce(jnp.maximum, s)
        e = [jnp.exp2((s[j] - m) * QSCALE) for j in range(W)]
        den = functools.reduce(_add, e)
        r = pl.reciprocal(den, approx=True)
        inv = r * (2.0 - den * r)
        og = [None] * NG
        for j in range(W):
            p = e[j] * inv
            if j:
                p = _after(p, _bits(og[NG - 1]) & zvec)
            for g in range(NG):
                t = p * src[2 * NG + g, rows(j), :]
                og[g] = t if og[g] is None else og[g] + t
        return og

    def stage(pb, even, odd):
        for g in range(NG):
            st_v[8 * pb:8 * pb + 8, g * 128:(g + 1) * 128] = _bits(
                jnp.concatenate([even[g], odd[g]], axis=0).astype(bf16))

    def unstage(r0, r1):
        return jnp.concatenate(_from_head_lanes(_groups(st_v[r0:r1, :]), tabs), axis=1)

    def out_proj(o, t0, side=None):
        a = _groups(_dot(o, wo_v[:, 0:D]))
        links = side(a) if side is not None else {}
        at = a_v.at[:, pl.ds(t0, o.shape[0] + 8), :]
        for g in range(NG):
            for rb in range(a[g].shape[0] // 8):
                v = a[g][rb * 8:(rb + 1) * 8]
                if rb == 0 and g in links:
                    v = _after(v, links[g])
                at[g, pl.ds((rb // 2) * 16 + rb % 2, 8, stride=2), :] = v

    def mod_vpu(wl, k, half, dep):
        zvec = zv_v[...]
        acc = None
        for i in range(D // 16):
            rows = slice(half * (D // 2) + i * 8, half * (D // 2) + (i + 1) * 8)
            cb = cb_v[rows, :]
            if i % 4 == 0:
                cb = _after(cb, dep if i == 0 else _bits(acc[:, 0:128]) & zvec)
            t = wl[rows, k * 256:(k + 1) * 256].astype(f32) * jnp.concatenate([cb, cb], axis=1)
            acc = t if acc is None else acc + t
        return acc

    def chunk_block(c, par, do_prep, do_mm, extra=None):
        zvec = zv_v[...]
        links = {}

        def link(ct, v):
            links[ct] = (links[ct] | v) if ct in links else v

        def rounds(hc, wp, rs, between=None):
            res = {}
            for k, r in enumerate(rs):
                out = _groups(_dot(hc, pltpu.bitcast(wp[:, r * 512:(r + 1) * 512], bf16)))
                for n in range(4):
                    res[4 * r + n] = out[n]
                if between is not None:
                    between(k)
            return res

        def accumulate(res):
            for ct in res:
                for t in range(SKEW):
                    blk = res[ct][t * T:(t + 1) * T]
                    if t == SKEW - 1 and ct in links:
                        blk = jnp.concatenate([blk[0:T - 8], _after(blk[T - 8:T], links.pop(ct) & zvec)], axis=0)
                    proj[t % 2][t // 2, ct, KOFF:KOFF + T, :] += blk
        mr = []

        def mods(k):
            for r in range(len(mr), 4):
                mr.append(mod_round(c + NG * (r // 2), r % 2))
        if do_prep:
            for cp in chunk_copies(c):
                cp.wait()
        if do_mm:
            res = rounds((he_v, ho_v)[1 - par][...], (wpe_v, wpo_v)[1 - par].at[(c - 1) >> 1], range(WR, 6),
                         mods if do_prep else None)
        if do_prep:
            mods(None)
            sh = mr[0] + mr[1]
            s1 = mr[2] + mr[3] + 1.0
            mod_v[c] = sh
            mod_v[NG + c] = s1
            hc = (xn_v[c].reshape(M0 // 8, 8, 128) * s1 + sh).reshape(M0, 128).astype(bf16)
            (he_v, ho_v)[par][...] = hc
            wp = (wpe_v, wpo_v)[par].at[c >> 1]
            for b in range(6):
                sec, half = b // 2, b % 2
                r0 = pl.multiple_of(c * KC + half * 64, 64)
                vs = _groups(_bits(wraw_v[pl.ds(r0, 64), sec * D:(sec + 1) * D]))
                vs = _to_head_lanes(vs, tabs)
                wp[half * 32:(half + 1) * 32, sec * D:(sec + 1) * D] = jnp.concatenate(vs, axis=1)
                if 2 * sec + 2 > WR:
                    link(8 + 3 * half, vs[NG - 1][24:32])
        if extra is not None:
            extra(res, link, zvec)
        if do_mm:
            accumulate(res)
        if do_prep:
            accumulate(rounds(hc, wp, range(WR)))

    def prologue():
        def zero(ct, carry):
            for t in range(SKEW):
                proj[t % 2][t // 2, ct, KOFF:KOFF + T, :] = jnp.zeros((T, 128), f32)
            return carry
        lax.fori_loop(0, 3 * NG, zero, 0)
        copies["c"].wait()
        c32 = c_v[...].astype(f32)
        sc = (c32 * jax.nn.sigmoid(c32)).astype(bf16)
        sc_v[...] = jnp.broadcast_to(sc, (16, D))
        diag = lax.broadcasted_iota(jnp.int32, (128, 128), 0) == lax.broadcasted_iota(jnp.int32, (128, 128), 1)
        for g, row in enumerate(_groups(sc.astype(f32))):
            col = jnp.sum(jnp.where(diag, row, 0.0), axis=1, keepdims=True)
            cb_v[g * 128:(g + 1) * 128, :] = jnp.broadcast_to(col, (128, 128))
        copies["x0"].wait()

        def stats(i, carry):
            for rb in range(12):
                rows = pl.ds(pl.multiple_of(i * 96, 32) + rb * 8, 8)
                xn = _norm8(_groups(x_v[rows, :].astype(f32)))
                for g in range(NG):
                    xn_v[g, rows, :] = xn[g]
            return carry
        lax.fori_loop(0, M0 // 96, stats, 0)
        chunk_block(0, 0, True, False)

        def kloop(i, carry):
            chunk_block(2 * i + 1, 1, True, True)

            @pl.when(2 * i + 2 < NKC)
            def _():
                chunk_block(2 * i + 2, 0, True, True)
            return carry
        lax.fori_loop(0, NKC // 2, kloop, 0)

        copies["x1"].wait()

        def ln_next(res, link, zvec):
            for rb in range(T // 8):
                ct = 4 * WR + (rb * (20 - 4 * WR)) // (T // 8)
                link(ct + 3, ln1_rows(x_v.at[M0:M0 + T, :], rb * 8, _bits(res[ct][M0 - 8:M0]) & zvec))
        chunk_block(NKC, 0, False, True, ln_next)
        for t in range(SKEW):
            for sg in range(NG, 3 * NG):
                if t == 0:
                    halo = jnp.broadcast_to(p0_v[0, sg, KOFF:KOFF + 1, :], (HALO, 128))
                else:
                    halo = proj[(t - 1) % 2][(t - 1) // 2, sg, KOFF + T - HALO:KOFF + T, :]
                proj[t % 2][t // 2, sg, KOFF - HALO:KOFF, :] = halo
        copies["x2"].wait()

    def step(s, par, first=False):
        GS, GA, GL, LL, UG = GATES["first" if first else par]
        piece = jnp.minimum(s - 1, NLP - 1 - par)
        zvec = zv_v[...]
        t0 = 0 if first else pl.multiple_of(s * T, T)
        slot = (s >> 1) & 1
        dst = proj[1 - par].at[((s + SKEW) >> 1) & 1]
        prev = proj[par].at[1 - slot]
        w = jnp.concatenate([(wpe_v, wpo_v)[c % 2][c // 2, :, 0:3 * D] for c in range(NKC)], axis=0)
        tiles = _groups(_dot(h_v[:, 0:D], pltpu.bitcast(w, bf16)))
        for ct in range(3 * NG):
            dst[ct, KOFF:KOFF + T, :] = tiles[ct]
            if ct >= NG:
                dst[ct, KOFF - HALO:KOFF, :] = prev[ct, KOFF + T - HALO:KOFF + T, :]
        t1 = (SKEW + 1) * T if first else pl.multiple_of(jnp.minimum(s + SKEW + 1, NT - 1) * T, T)
        src = proj[par].at[slot]
        links, rows = [], []

        def gate(pos):
            ct = int(pos)
            rb = min(T // 8 - 1, int((pos - ct) * (T // 8)))
            return _bits(tiles[ct][rb * 8:(rb + 1) * 8, :]) & zvec

        for pb in range(NP):
            halves = []
            for k in (2 * pb, 2 * pb + 1):
                d = gate(GA + GS * k / NRB)
                if k >= LL:
                    d = d | (links[k - LL] & zvec)
                halves.append(attn8(src, first, pb, k % 2, d))
            stage(pb, *halves)
            for rb in (2 * pb, 2 * pb + 1):
                links.append(ln1_rows(x_v.at[pl.ds(t1, T), :], rb * 8, gate(GA + GL + GS * rb / NRB)))
            if (pb + 1) % UG == 0:
                rows.append(pltpu.bitcast(unstage((pb + 1 - UG) * 8, (pb + 1) * 8), bf16))

        def side(a):
            links = {}
            ev = tiles[3 * NG - 2:] + a
            for k in range(LW // 256):
                part = [mod_vpu((wl0_v, wl1_v)[par], k, h, _bits(ev[(7 * (2 * k + h)) // 4][T - 8:T]) & zvec)
                        for h in range(2)]
                m = jnp.sum(part[0] + part[1], axis=0, keepdims=True)
                m = jnp.broadcast_to(m + jnp.where(piece >> 1 == 2, 1.0, 0.0), (8, 256))
                modr_v[4 * piece + 2 * k] = m[:, 0:128]
                modr_v[4 * piece + 2 * k + 1] = m[:, 128:256]
                links[5 + 2 * k] = _bits(m[:, 0:128]) & zvec
            if par == 0:
                for k in range(6):
                    seen = []
                    for sg in range(4 * k, 4 * k + 4):
                        lo = KOFF if sg < NG else KOFF - HALO
                        for r in range(lo, KOFF + T, 8):
                            v = p0_v[1, sg, r:r + 8, :]
                            if not seen:
                                v = _after(v, _bits(ev[k + 1][T - 8:T]) & zvec)
                            p1_v[2, sg, r:r + 8, :] = v
                            seen.append(_bits(v))
                    lk = functools.reduce(_or, seen) & zvec
                    links[k + 2] = (links[k + 2] | lk) if k + 2 in links else lk
            return links
        if first:
            copies["wo"].wait()
            out_proj(jnp.concatenate(rows, axis=0), t0)
        else:
            out_proj(jnp.concatenate(rows, axis=0), t0, side)

            @pl.when(s + 1 < NLP)
            def _():
                late_copy(s + 1, par).start()

    def phase_a(i):
        @pl.when(i == 0)
        def _():
            prologue()
            step(0, 0, True)

        @pl.when(i == 0)
        def _():
            copies["x3"].wait()

        @pl.when(2 * i < NLP)
        def _():
            late_copy(2 * i, 1).wait()
        step(2 * i + 1, 1)

        @pl.when(i == 0)
        def _():
            copies["xr"].wait()

        @pl.when(2 * i + 1 < NLP)
        def _():
            late_copy(2 * i + 1, 0).wait()
        step(2 * i + 2, 0)

        @pl.when(i == NA - 1)
        def _():
            for n in ("w1", "w3", "w2"):
                copies[n].wait()
            fill_window(0, range(3 * NG), None)
            for rb in range(NRB):
                ln2_rows(0, rb * 8, None)

    def fill_window(i, sgs, dep):
        src = p1_v.at[(i // IPT) % 3, :, pl.ds(pl.multiple_of((i % IPT) * 16 * PPI, 16 * PPI), WROWS), :]
        seen = []
        for sg in sgs:
            lo = KOFF if sg < NG else KOFF - HALO
            v = src[sg, lo:WROWS, :]
            if not seen:
                v = jnp.concatenate([_after(v[0:8], dep), v[8:]], axis=0)
            win_v[sg, lo:WROWS, :] = v
            seen += [_bits(v[r:r + 8]) for r in range(0, WROWS - lo, 8)]
        return functools.reduce(_or, seen)

    def phase_b(i):
        i = i - NA
        t1 = pl.multiple_of(jnp.minimum(i + 1, NT - 1) * T, T)
        zvec = zv_v[...]
        sl = (i // IPT) % 3
        orow = jnp.where(sl == 0, 0, jnp.where(sl == 1, T, T // 2)) + (i % IPT) * 8 * PPI

        def fin(dep):
            o = unstage(0, 8 * PPI)
            o_v[pl.ds(pl.multiple_of(orow, 8 * PPI), 8 * PPI), :] = o
            return o[8 * PPI - 8:8 * PPI, D - 128:D]
        halves = []

        def att(n):
            def run(d):
                halves.append(attn8(win_v, False, n // 2, n % 2, d))
                if n % 2:
                    stage(n // 2, *halves[-2:])
                return _bits(halves[-1][NG - 1])
            return run
        ln = lambda r: (lambda d: ln2_rows(t1, r * 8, d))
        fw = lambda k: (lambda d: fill_window(i + 1, range(6 * k, 6 * k + 6), d))
        code = {"a": att, "f": lambda n: fin, "l": ln, "w": fw}
        cnt = dict.fromkeys(code, 0)
        side = []
        for chunk in FPLAN.split("/"):
            side.append([])
            for c in chunk:
                side[-1].append(code[c](cnt[c]))
                cnt[c] += 1
        assert cnt == {"a": 2 * PPI, "f": 1, "l": NRB, "w": 4}, cnt
        h = h2_v[:, 0:D]
        gb = jnp.concatenate([mcol(5, g) for g in range(NG)], axis=1)
        scaled = lambda y: (y.reshape(NRB, 8, D) * gb).reshape(T, D)
        acc = act_prev = None
        links = []
        for fc in range(NFC + 1):
            ev = []
            if fc < NFC:
                g = _dot(h, w1_v[:, fc * FC:(fc + 1) * FC])
                u = _dot(h, w3_v[:, fc * FC:(fc + 1) * FC])
                ev = _groups(g) + _groups(u)
                if 1 <= fc <= len(side):
                    u0 = _after(u[T - 8:T, FC - 128:FC], functools.reduce(_or, links[fc - 1]) & zvec)
                    u = jnp.concatenate([u[0:T - 8, :], jnp.concatenate([u[T - 8:T, 0:FC - 128], u0], axis=1)], axis=0)
                hg = 0.5 * g
                act = (hg * (1.0 + jnp.tanh(hg)) * u).astype(bf16)
            if fc >= 1:
                y = _dot(act_prev, w2_v[(fc - 1) * FC:fc * FC, 0:D])
                ev = ev + _groups(y)
                acc = (x1_v[...] if acc is None else acc) + scaled(y)
            if fc < len(side):
                n = len(side[fc])
                pos = [4 + (k * 12) // n if fc else 3 + (k * 5) // n for k in range(n)]
                links.append([fn(_bits(ev[p][T - 16:T - 8]) & zvec) for p, fn in zip(pos, side[fc])])
            act_prev = act
        rows = pl.ds(pl.multiple_of(i * T, T), T)
        for half in range(2):
            cols = slice(half * (D // 2), (half + 1) * (D // 2))
            ob_v[rows, cols] = acc[:, cols].astype(bf16)
            pltpu.make_async_copy(ob_v.at[rows, cols], out_hbm.at[0, rows, cols], osem.at[0]).start()

        @pl.when(i == SKEW * IPT - 1)
        def _():
            out_proj(pltpu.bitcast(o_v[...], bf16), NS * T)

    def main(i, carry):
        lax.cond(i < NA, phase_a, phase_b, i)
        return carry
    lax.fori_loop(0, NA + NT, main, 0)
    pltpu.make_async_copy(ob_v, out_hbm.at[0], osem.at[0]).wait()


@jax.jit
def pallas_adaLN_cond__sliding_local_dilated__glu_gated_swiglu__prompt_kernel(
    A_x, A_wqkv, A_wo, B_x, B_w1, B_w3, B_w2, c, w_mod):
    del B_x
    any_spec = pl.BlockSpec(memory_space=pl.ANY)
    return pl.pallas_call(
        _kernel,
        out_shape=jax.ShapeDtypeStruct((1, S, D), bf16),
        in_specs=[any_spec] * 8,
        out_specs=any_spec,
        scratch_shapes=[
            pltpu.VMEM((S, D), bf16),
            pltpu.VMEM((1, D), bf16),
            pltpu.VMEM((16, D), bf16),
            pltpu.VMEM((D, 128), f32),
            pltpu.VMEM((2 * NG, D, 128), bf16),
            pltpu.VMEM((D, LW), bf16),
            pltpu.VMEM((D, LW), bf16),
            pltpu.VMEM((D, 3 * D), bf16),
            pltpu.VMEM((NKC // 2, KC // 2, 3 * D + PADW), u32),
            pltpu.VMEM((NKC // 2, KC // 2, 3 * D + PADW), u32),
            pltpu.VMEM((D, D + PADW), bf16),
            pltpu.VMEM((D, F + PADW), bf16),
            pltpu.VMEM((D, F + PADW), bf16),
            pltpu.VMEM((F, D + PADW), bf16),
            pltpu.VMEM((2 * NG, 8, 128), f32),
            pltpu.VMEM((4 * NG, 8, 128), f32),
            pltpu.VMEM((NG, M0, 128), f32),
            pltpu.VMEM((M0, KC), bf16),
            pltpu.VMEM((M0, KC), bf16),
            pltpu.VMEM((T, D + PADW), bf16),
            pltpu.VMEM((T, D + PADW), bf16),
            pltpu.VMEM((T, D), f32),
            pltpu.VMEM((3 * NG, WROWS + 8, 128), f32),
            pltpu.VMEM((T // 2, D), u32),
            pltpu.VMEM((M0 // 2, D), u32),
            pltpu.VMEM((2, 3 * NG, KROWS, 128), f32),
            pltpu.VMEM((3, 3 * NG, KROWS, 128), f32),
            pltpu.VMEM((NG, S + 8, 128), f32),
            pltpu.VMEM((S, D), bf16),
            pltpu.VMEM((8, 128), u32),
            pltpu.SemaphoreType.DMA((12 + 2 * NKC,)),
            pltpu.SemaphoreType.DMA((1,)),
        ],
        compiler_params=pltpu.CompilerParams(vmem_limit_bytes=110 * 2**20, disable_bounds_checks=True,
                                             disable_semaphore_checks=True),
        name="adaln_fused",
    )(A_x, A_wqkv, A_wo, B_w1, B_w3, B_w2, c, w_mod)
```

```python
import functools

import jax
import jax.numpy as jnp
from jax import lax
import jax.experimental.pallas as pl
import jax.experimental.pallas.tpu as pltpu

S, D, F = 2048, 1024, 3584
DH, W, DIL = 32, 8, 2
NG = D // 128
HALO = 16
T = 128
NT = S // T
NP = T // 16
NRB = T // 8
SKEW = 3
M0 = SKEW * T
NS = NT - SKEW
NA = NS // 2
PPI = 2
IPT = NP // PPI
WROWS = HALO + 16 * PPI
FC = 512
NFC = F // FC
KOFF = HALO
KROWS = KOFF + T + 8
LOG2E = 1.4426950408889634
QSCALE = (DH ** -0.5) * LOG2E
NEG = -1e9 * DH ** 0.5
KC = 128
NKC = D // KC
WR = 4
LW = 512
NLP = 4 * D // LW
PADW = 128
EPS = 1e-5
GATES = {"first": (19.0, 0.5, 0.6, 6, 8), 1: (20.0, 0.0, 0.6, 4, 2), 0: (20.0, 0.7, 0.6, 4, 8)}
FPLAN = "aaa/all/flll/lwlll/lwlwl/lllwl"
f32, bf16, u32 = jnp.float32, jnp.bfloat16, jnp.uint32


def _lane_tables():
    lane = lax.broadcasted_iota(jnp.int32, (8, 128), 1)
    head = lane & 31
    masks = [(lane & (4 << s)) != 0 for s in range(3)]
    fwd = [((head & 3) << 5) | (((head >> 2) ^ g) << 2) | (lane >> 5) for g in range(NG)]
    inv = [((lane & 3) << 5) | ((((lane >> 2) & 7) ^ g) << 2) | (lane >> 5) for g in range(NG)]
    return masks, fwd, inv


def _butterfly(vs, masks):
    n = vs[0].shape[0] // 8
    vs = [v.reshape(n, 8, 128) for v in vs]
    for s in range(3):
        for g in range(NG):
            if g & (1 << s):
                continue
            a, b = vs[g], vs[g | (1 << s)]
            vs[g] = jnp.where(masks[s], b, a)
            vs[g | (1 << s)] = jnp.where(masks[s], a, b)
    return [v.reshape(n * 8, 128) for v in vs]


def _gather_lanes(v, idx):
    idx = jnp.concatenate([idx] * (v.shape[0] // 8), axis=0)
    return jnp.take_along_axis(v, idx, axis=1, mode="promise_in_bounds")


def _to_head_lanes(vs, tabs):
    return [_gather_lanes(y, i) for y, i in zip(_butterfly(vs, tabs[0]), tabs[1])]


def _from_head_lanes(zs, tabs):
    return _butterfly([_gather_lanes(z, i) for z, i in zip(zs, tabs[2])], tabs[0])


def _add(a, b):
    return a + b


def _or(a, b):
    return a | b


def _bits(x):
    return pltpu.bitcast(x, u32)


def _dot(a, b):
    return jnp.dot(a, b, preferred_element_type=f32)


def _after(x, dep):
    if dep is None:
        return x
    return pltpu.bitcast(_bits(x) | dep, x.dtype)


def _norm8(xs, dep=None):
    xs = [_after(xs[0], dep)] + list(xs[1:])
    m = jnp.sum(functools.reduce(_add, xs), axis=-1, keepdims=True) * (1.0 / D)
    xc = [v - m for v in xs]
    var = jnp.sum(functools.reduce(_add, [v * v for v in xc]), axis=-1, keepdims=True) * (1.0 / D)
    r = lax.rsqrt(var + EPS)
    return [v * r for v in xc]


def _groups(x):
    return [x[:, g * 128:(g + 1) * 128] for g in range(x.shape[1] // 128)]


def _kernel(x_hbm, wqkv_hbm, wo_hbm, w1_hbm, w3_hbm, w2_hbm, c_hbm, wmod_hbm, out_hbm,
            x_v, c_v, cb_v, wm_v, wl0_v, wl1_v, wraw_v, wpe_v, wpo_v, wo_v, w1_v, w3_v, w2_v, mod_v, modr_v,
            xn_v, he_v, ho_v, h_v, h2_v, x1_v, win_v, st_v, o_v, p0_v, p1_v, a_v, ob_v,
            zv_v, sem, osem):
    names = ["c", "x0", "x1", "x2", "x3", "xr", "wo", "w1", "w3", "w2", "wl0", "wl1"]
    srcdst = dict(
        c=(c_hbm, c_v),
        x0=(x_hbm.at[0, 0:M0, :], x_v.at[0:M0, :]),
        x1=(x_hbm.at[0, M0:M0 + T, :], x_v.at[M0:M0 + T, :]),
        x2=(x_hbm.at[0, M0 + T:M0 + 2 * T, :], x_v.at[M0 + T:M0 + 2 * T, :]),
        x3=(x_hbm.at[0, M0 + 2 * T:M0 + 3 * T, :], x_v.at[M0 + 2 * T:M0 + 3 * T, :]),
        xr=(x_hbm.at[0, M0 + 3 * T:S, :], x_v.at[M0 + 3 * T:S, :]),
        wo=(wo_hbm, wo_v.at[:, 0:D]),
        w1=(w1_hbm, w1_v.at[:, 0:F]), w3=(w3_hbm, w3_v.at[:, 0:F]), w2=(w2_hbm, w2_v.at[:, 0:D]),
    )
    copies = {n: pltpu.make_async_copy(*srcdst[n], sem.at[names.index(n)]) for n in srcdst}
    SEM_C = len(names)
    SEM_W = SEM_C + NKC

    def slab_copy(c, sec):
        cols = pl.ds(pl.multiple_of(sec * D + c * KC, KC), KC)
        return pltpu.make_async_copy(wmod_hbm.at[:, cols], wm_v.at[c, :, sec * KC:(sec + 1) * KC], sem.at[SEM_C + c])

    def chunk_copies(c):
        rows = pl.ds(pl.multiple_of(c * KC, KC), KC)
        return [slab_copy(c, 0), slab_copy(c, 1),
                pltpu.make_async_copy(wqkv_hbm.at[rows, :], wraw_v.at[rows, :], sem.at[SEM_W + c])]

    def late_copy(p, par):
        cols = pl.ds(pl.multiple_of(2 * D + p * LW, LW), LW)
        return pltpu.make_async_copy(wmod_hbm.at[:, cols], (wl0_v, wl1_v)[par], sem.at[names.index("wl0") + par])

    copies["c"].start()
    copies["x0"].start()
    for c in range(NKC):
        for cp in chunk_copies(c):
            cp.start()
    for n in ("x1", "x2", "wo", "x3"):
        copies[n].start()
    late_copy(0, 1).start()
    late_copy(1, 0).start()
    copies["xr"].start()
    for n in ("w1", "w3", "w2"):
        copies[n].start(priority=1)
    zv_v[...] = jnp.zeros(zv_v.shape, u32)

    tabs = _lane_tables()
    proj = (p0_v, p1_v)
    mcol = lambda sec, g: mod_v[sec * NG + g] if sec < 2 else modr_v[(sec - 2) * NG + g]
    row8 = lax.broadcasted_iota(jnp.int32, (8, 128), 0)

    def ln1_rows(xt, drow, dep):
        xn = _norm8(_groups(xt[drow:drow + 8, :].astype(f32)), dep)
        ys = [xn[g] * mcol(1, g) + mcol(0, g) for g in range(NG)]
        h_v[drow:drow + 8, 0:D] = jnp.concatenate(ys, axis=1).astype(bf16)
        return _bits(ys[NG - 1])

    def ln2_rows(t, drow, dep):
        xt, at = x_v.at[pl.ds(t, T), :], a_v.at[:, pl.ds(t, T), :]
        x = _groups(xt[drow:drow + 8, :].astype(f32))
        x1 = [x[g] + mcol(2, g) * at[g, drow:drow + 8, :] for g in range(NG)]
        x1_v[drow:drow + 8, :] = jnp.concatenate(x1, axis=1)
        xn = _norm8(x1, dep)
        ys = [xn[g] * mcol(4, g) + mcol(3, g) for g in range(NG)]
        h2_v[drow:drow + 8, 0:D] = jnp.concatenate(ys, axis=1).astype(bf16)
        return _bits(ys[NG - 1])

    def attn8(src, masked, pb, par, dep):
        r0 = KOFF + 16 * pb + par
        rows = lambda j: pl.ds(r0 - DIL * j, 8, stride=DIL)
        zvec = zv_v[...]
        s = [None] * W
        for g in range(NG):
            q = src[g, rows(0), :]
            if g == 0:
                q = _after(q, dep)
            else:
                q = _after(q, _bits(s[W - 1]) & zvec)
            for j in range(W):
                p = q * src[NG + g, rows(j), :]
                s[j] = p if s[j] is None else s[j] + p
        for j in range(W):
            s[j] = s[j] + pltpu.roll(s[j], 64, 1)
            s[j] = s[j] + pltpu.roll(s[j], 32, 1)
            if masked and pb == 0 and j > 0:
                s[j] = jnp.where(par + DIL * row8 >= DIL * j, s[j], NEG)
        m = functools.reduce(jnp.maximum, s)
        e = [jnp.exp2((s[j] - m) * QSCALE) for j in range(W)]
        den = functools.reduce(_add, e)
        r = pl.reciprocal(den, approx=True)
        inv = r * (2.0 - den * r)
        og = [None] * NG
        for j in range(W):
            p = e[j] * inv
            if j:
                p = _after(p, _bits(og[NG - 1]) & zvec)
            for g in range(NG):
                t = p * src[2 * NG + g, rows(j), :]
                og[g] = t if og[g] is None else og[g] + t
        return og

    def stage(pb, even, odd):
        for g in range(NG):
            st_v[8 * pb:8 * pb + 8, g * 128:(g + 1) * 128] = _bits(
                jnp.concatenate([even[g], odd[g]], axis=0).astype(bf16))

    def unstage(r0, r1):
        return jnp.concatenate(_from_head_lanes(_groups(st_v[r0:r1, :]), tabs), axis=1)

    def out_proj(o, t0, side=None):
        a = _groups(_dot(o, wo_v[:, 0:D]))
        links = side(a) if side is not None else {}
        at = a_v.at[:, pl.ds(t0, o.shape[0] + 8), :]
        for g in range(NG):
            for rb in range(a[g].shape[0] // 8):
                v = a[g][rb * 8:(rb + 1) * 8]
                if rb == 0 and g in links:
                    v = _after(v, links[g])
                at[g, pl.ds((rb // 2) * 16 + rb % 2, 8, stride=2), :] = v

    def mod_vpu(wl, k, part, nparts, dep):
        n = D // nparts
        zvec = zv_v[...]
        acc = None
        for i in range(n // 8):
            rows = slice(part * n + i * 8, part * n + (i + 1) * 8)
            cb = cb_v[rows, :]
            if i % 4 == 0:
                cb = _after(cb, dep if i == 0 else _bits(acc[:, 0:128]) & zvec)
            t = wl[rows, k * 256:(k + 1) * 256].astype(f32) * jnp.concatenate([cb, cb], axis=1)
            acc = t if acc is None else acc + t
        return acc

    def chunk_block(c, par, do_prep, do_mm, extra=None):
        zvec = zv_v[...]
        links = {}

        def link(ct, v):
            links[ct] = (links[ct] | v) if ct in links else v

        def rounds(hc, wp, rs):
            res = {}
            for r in rs:
                out = _groups(_dot(hc, pltpu.bitcast(wp[:, r * 512:(r + 1) * 512], bf16)))
                for n in range(4):
                    res[4 * r + n] = out[n]
            return res

        def accumulate(res):
            for ct in res:
                for t in range(SKEW):
                    blk = res[ct][t * T:(t + 1) * T]
                    if t == SKEW - 1 and ct in links:
                        blk = jnp.concatenate([blk[0:T - 8], _after(blk[T - 8:T], links.pop(ct) & zvec)], axis=0)
                    proj[t % 2][t // 2, ct, KOFF:KOFF + T, :] += blk
        if do_prep:
            for cp in chunk_copies(c):
                cp.wait()
        if do_mm:
            res = rounds((he_v, ho_v)[1 - par][...], (wpe_v, wpo_v)[1 - par].at[(c - 1) >> 1], range(WR, 6))
        if do_prep:
            part = [mod_vpu(wm_v.at[c], 0, h, 4, None) for h in range(4)]
            m = jnp.broadcast_to(jnp.sum(functools.reduce(_add, part), axis=0, keepdims=True), (8, 256))
            sh = m[:, 0:128]
            s1 = m[:, 128:256] + 1.0
            mod_v[c] = sh
            mod_v[NG + c] = s1
            hc = (xn_v[c].reshape(M0 // 8, 8, 128) * s1 + sh).reshape(M0, 128).astype(bf16)
            (he_v, ho_v)[par][...] = hc
            wp = (wpe_v, wpo_v)[par].at[c >> 1]
            for b in range(6):
                sec, half = b // 2, b % 2
                r0 = pl.multiple_of(c * KC + half * 64, 64)
                vs = _groups(_bits(wraw_v[pl.ds(r0, 64), sec * D:(sec + 1) * D]))
                vs = _to_head_lanes(vs, tabs)
                wp[half * 32:(half + 1) * 32, sec * D:(sec + 1) * D] = jnp.concatenate(vs, axis=1)
                if 2 * sec + 2 > WR:
                    link(8 + 3 * half, vs[NG - 1][24:32])
        if extra is not None:
            extra(res, link, zvec)
        if do_mm:
            accumulate(res)
        if do_prep:
            accumulate(rounds(hc, wp, range(WR)))

    def prologue():
        def zero(ct, carry):
            for t in range(SKEW):
                proj[t % 2][t // 2, ct, KOFF:KOFF + T, :] = jnp.zeros((T, 128), f32)
            return carry
        lax.fori_loop(0, 3 * NG, zero, 0)
        copies["c"].wait()
        c32 = c_v[...].astype(f32)
        sc = (c32 * jax.nn.sigmoid(c32)).astype(bf16)
        diag = lax.broadcasted_iota(jnp.int32, (128, 128), 0) == lax.broadcasted_iota(jnp.int32, (128, 128), 1)
        for g, row in enumerate(_groups(sc.astype(f32))):
            col = jnp.sum(jnp.where(diag, row, 0.0), axis=1, keepdims=True)
            cb_v[g * 128:(g + 1) * 128, :] = jnp.broadcast_to(col, (128, 128))
        copies["x0"].wait()

        def stats(i, carry):
            for rb in range(12):
                rows = pl.ds(pl.multiple_of(i * 96, 32) + rb * 8, 8)
                xn = _norm8(_groups(x_v[rows, :].astype(f32)))
                for g in range(NG):
                    xn_v[g, rows, :] = xn[g]
            return carry
        lax.fori_loop(0, M0 // 96, stats, 0)
        chunk_block(0, 0, True, False)

        def kloop(i, carry):
            chunk_block(2 * i + 1, 1, True, True)

            @pl.when(2 * i + 2 < NKC)
            def _():
                chunk_block(2 * i + 2, 0, True, True)
            return carry
        lax.fori_loop(0, NKC // 2, kloop, 0)

        copies["x1"].wait()

        def ln_next(res, link, zvec):
            for rb in range(T // 8):
                ct = 4 * WR + (rb * (20 - 4 * WR)) // (T // 8)
                link(ct + 3, ln1_rows(x_v.at[M0:M0 + T, :], rb * 8, _bits(res[ct][M0 - 8:M0]) & zvec))
        chunk_block(NKC, 0, False, True, ln_next)
        for t in range(SKEW):
            for sg in range(NG, 3 * NG):
                if t == 0:
                    halo = jnp.broadcast_to(p0_v[0, sg, KOFF:KOFF + 1, :], (HALO, 128))
                else:
                    halo = proj[(t - 1) % 2][(t - 1) // 2, sg, KOFF + T - HALO:KOFF + T, :]
                proj[t % 2][t // 2, sg, KOFF - HALO:KOFF, :] = halo
        copies["x2"].wait()

    def step(s, par, first=False):
        GS, GA, GL, LL, UG = GATES["first" if first else par]
        piece = jnp.minimum(s - 1, NLP - 1 - par)
        zvec = zv_v[...]
        t0 = 0 if first else pl.multiple_of(s * T, T)
        slot = (s >> 1) & 1
        dst = proj[1 - par].at[((s + SKEW) >> 1) & 1]
        prev = proj[par].at[1 - slot]
        w = jnp.concatenate([(wpe_v, wpo_v)[c % 2][c // 2, :, 0:3 * D] for c in range(NKC)], axis=0)
        tiles = _groups(_dot(h_v[:, 0:D], pltpu.bitcast(w, bf16)))
        for ct in range(3 * NG):
            dst[ct, KOFF:KOFF + T, :] = tiles[ct]
            if ct >= NG:
                dst[ct, KOFF - HALO:KOFF, :] = prev[ct, KOFF + T - HALO:KOFF + T, :]
        t1 = (SKEW + 1) * T if first else pl.multiple_of(jnp.minimum(s + SKEW + 1, NT - 1) * T, T)
        src = proj[par].at[slot]
        links, rows = [], []

        def gate(pos):
            ct = int(pos)
            rb = min(T // 8 - 1, int((pos - ct) * (T // 8)))
            return _bits(tiles[ct][rb * 8:(rb + 1) * 8, :]) & zvec

        for pb in range(NP):
            halves = []
            for k in (2 * pb, 2 * pb + 1):
                d = gate(GA + GS * k / NRB)
                if k >= LL:
                    d = d | (links[k - LL] & zvec)
                halves.append(attn8(src, first, pb, k % 2, d))
            stage(pb, *halves)
            for rb in (2 * pb, 2 * pb + 1):
                links.append(ln1_rows(x_v.at[pl.ds(t1, T), :], rb * 8, gate(GA + GL + GS * rb / NRB)))
            if (pb + 1) % UG == 0:
                rows.append(pltpu.bitcast(unstage((pb + 1 - UG) * 8, (pb + 1) * 8), bf16))

        def side(a):
            links = {}
            ev = tiles[3 * NG - 2:] + a
            for k in range(LW // 256):
                part = [mod_vpu((wl0_v, wl1_v)[par], k, h, 2, _bits(ev[(7 * (2 * k + h)) // 4][T - 8:T]) & zvec)
                        for h in range(2)]
                m = jnp.sum(part[0] + part[1], axis=0, keepdims=True)
                m = jnp.broadcast_to(m + jnp.where(piece >> 1 == 2, 1.0, 0.0), (8, 256))
                modr_v[4 * piece + 2 * k] = m[:, 0:128]
                modr_v[4 * piece + 2 * k + 1] = m[:, 128:256]
                links[5 + 2 * k] = _bits(m[:, 0:128]) & zvec
            if par == 0:
                for k in range(6):
                    seen = []
                    for sg in range(4 * k, 4 * k + 4):
                        lo = KOFF if sg < NG else KOFF - HALO
                        for r in range(lo, KOFF + T, 8):
                            v = p0_v[1, sg, r:r + 8, :]
                            if not seen:
                                v = _after(v, _bits(ev[k + 1][T - 8:T]) & zvec)
                            p1_v[2, sg, r:r + 8, :] = v
                            seen.append(_bits(v))
                    lk = functools.reduce(_or, seen) & zvec
                    links[k + 2] = (links[k + 2] | lk) if k + 2 in links else lk
            return links
        if first:
            copies["wo"].wait()
            out_proj(jnp.concatenate(rows, axis=0), t0)
        else:
            out_proj(jnp.concatenate(rows, axis=0), t0, side)

            @pl.when(s + 1 < NLP)
            def _():
                late_copy(s + 1, par).start()

    def phase_a(i):
        @pl.when(i == 0)
        def _():
            prologue()
            step(0, 0, True)

        @pl.when(i == 0)
        def _():
            copies["x3"].wait()

        @pl.when(2 * i < NLP)
        def _():
            late_copy(2 * i, 1).wait()
        step(2 * i + 1, 1)

        @pl.when(i == 0)
        def _():
            copies["xr"].wait()

        @pl.when(2 * i + 1 < NLP)
        def _():
            late_copy(2 * i + 1, 0).wait()
        step(2 * i + 2, 0)

        @pl.when(i == NA - 1)
        def _():
            for n in ("w1", "w3", "w2"):
                copies[n].wait()
            fill_window(0, range(3 * NG), None)
            for rb in range(NRB):
                ln2_rows(0, rb * 8, None)

    def fill_window(i, sgs, dep):
        src = p1_v.at[(i // IPT) % 3, :, pl.ds(pl.multiple_of((i % IPT) * 16 * PPI, 16 * PPI), WROWS), :]
        seen = []
        for sg in sgs:
            lo = KOFF if sg < NG else KOFF - HALO
            v = src[sg, lo:WROWS, :]
            if not seen:
                v = jnp.concatenate([_after(v[0:8], dep), v[8:]], axis=0)
            win_v[sg, lo:WROWS, :] = v
            seen += [_bits(v[r:r + 8]) for r in range(0, WROWS - lo, 8)]
        return functools.reduce(_or, seen)

    def phase_b(i):
        i = i - NA
        t1 = pl.multiple_of(jnp.minimum(i + 1, NT - 1) * T, T)
        zvec = zv_v[...]
        sl = (i // IPT) % 3
        orow = jnp.where(sl == 0, 0, jnp.where(sl == 1, T, T // 2)) + (i % IPT) * 8 * PPI

        def fin(dep):
            o = unstage(0, 8 * PPI)
            o_v[pl.ds(pl.multiple_of(orow, 8 * PPI), 8 * PPI), :] = o
            return o[8 * PPI - 8:8 * PPI, D - 128:D]
        halves = []

        def att(n):
            def run(d):
                halves.append(attn8(win_v, False, n // 2, n % 2, d))
                if n % 2:
                    stage(n // 2, *halves[-2:])
                return _bits(halves[-1][NG - 1])
            return run
        ln = lambda r: (lambda d: ln2_rows(t1, r * 8, d))
        fw = lambda k: (lambda d: fill_window(i + 1, range(6 * k, 6 * k + 6), d))
        code = {"a": att, "f": lambda n: fin, "l": ln, "w": fw}
        cnt = dict.fromkeys(code, 0)
        side = []
        for chunk in FPLAN.split("/"):
            side.append([])
            for c in chunk:
                side[-1].append(code[c](cnt[c]))
                cnt[c] += 1
        assert cnt == {"a": 2 * PPI, "f": 1, "l": NRB, "w": 4}, cnt
        h = h2_v[:, 0:D]
        gb = jnp.concatenate([mcol(5, g) for g in range(NG)], axis=1)
        scaled = lambda y: (y.reshape(NRB, 8, D) * gb).reshape(T, D)
        acc = act_prev = None
        links = []
        for fc in range(NFC + 1):
            ev = []
            if fc < NFC:
                g = _dot(h, w1_v[:, fc * FC:(fc + 1) * FC])
                u = _dot(h, w3_v[:, fc * FC:(fc + 1) * FC])
                ev = _groups(g) + _groups(u)
                if 1 <= fc <= len(side):
                    u0 = _after(u[T - 8:T, FC - 128:FC], functools.reduce(_or, links[fc - 1]) & zvec)
                    u = jnp.concatenate([u[0:T - 8, :], jnp.concatenate([u[T - 8:T, 0:FC - 128], u0], axis=1)], axis=0)
                hg = 0.5 * g
                act = (hg * (1.0 + jnp.tanh(hg)) * u).astype(bf16)
            if fc >= 1:
                y = _dot(act_prev, w2_v[(fc - 1) * FC:fc * FC, 0:D])
                ev = ev + _groups(y)
                acc = (x1_v[...] if acc is None else acc) + scaled(y)
            if fc < len(side):
                n = len(side[fc])
                pos = [4 + (k * 12) // n if fc else 3 + (k * 5) // n for k in range(n)]
                links.append([fn(_bits(ev[p][T - 16:T - 8]) & zvec) for p, fn in zip(pos, side[fc])])
            act_prev = act
        rows = pl.ds(pl.multiple_of(i * T, T), T)
        for half in range(2):
            cols = slice(half * (D // 2), (half + 1) * (D // 2))
            ob_v[rows, cols] = acc[:, cols].astype(bf16)
            pltpu.make_async_copy(ob_v.at[rows, cols], out_hbm.at[0, rows, cols], osem.at[0]).start()

        @pl.when(i == SKEW * IPT - 1)
        def _():
            out_proj(pltpu.bitcast(o_v[...], bf16), NS * T)

    def main(i, carry):
        lax.cond(i < NA, phase_a, phase_b, i)
        return carry
    lax.fori_loop(0, NA + NT, main, 0)
    pltpu.make_async_copy(ob_v, out_hbm.at[0], osem.at[0]).wait()


@jax.jit
def pallas_adaLN_cond__sliding_local_dilated__glu_gated_swiglu__prompt_kernel(
    A_x, A_wqkv, A_wo, B_x, B_w1, B_w3, B_w2, c, w_mod):
    del B_x
    any_spec = pl.BlockSpec(memory_space=pl.ANY)
    return pl.pallas_call(
        _kernel,
        out_shape=jax.ShapeDtypeStruct((1, S, D), bf16),
        in_specs=[any_spec] * 8,
        out_specs=any_spec,
        scratch_shapes=[
            pltpu.VMEM((S, D), bf16),
            pltpu.VMEM((1, D), bf16),
            pltpu.VMEM((D, 128), f32),
            pltpu.VMEM((NKC, D, 2 * KC), bf16),
            pltpu.VMEM((D, LW), bf16),
            pltpu.VMEM((D, LW), bf16),
            pltpu.VMEM((D, 3 * D), bf16),
            pltpu.VMEM((NKC // 2, KC // 2, 3 * D + PADW), u32),
            pltpu.VMEM((NKC // 2, KC // 2, 3 * D + PADW), u32),
            pltpu.VMEM((D, D + PADW), bf16),
            pltpu.VMEM((D, F + PADW), bf16),
            pltpu.VMEM((D, F + PADW), bf16),
            pltpu.VMEM((F, D + PADW), bf16),
            pltpu.VMEM((2 * NG, 8, 128), f32),
            pltpu.VMEM((4 * NG, 8, 128), f32),
            pltpu.VMEM((NG, M0, 128), f32),
            pltpu.VMEM((M0, KC), bf16),
            pltpu.VMEM((M0, KC), bf16),
            pltpu.VMEM((T, D + PADW), bf16),
            pltpu.VMEM((T, D + PADW), bf16),
            pltpu.VMEM((T, D), f32),
            pltpu.VMEM((3 * NG, WROWS + 8, 128), f32),
            pltpu.VMEM((T // 2, D), u32),
            pltpu.VMEM((M0 // 2, D), u32),
            pltpu.VMEM((2, 3 * NG, KROWS, 128), f32),
            pltpu.VMEM((3, 3 * NG, KROWS, 128), f32),
            pltpu.VMEM((NG, S + 8, 128), f32),
            pltpu.VMEM((S, D), bf16),
            pltpu.VMEM((8, 128), u32),
            pltpu.SemaphoreType.DMA((12 + 2 * NKC,)),
            pltpu.SemaphoreType.DMA((1,)),
        ],
        compiler_params=pltpu.CompilerParams(vmem_limit_bytes=110 * 2**20, disable_bounds_checks=True,
                                             disable_semaphore_checks=True),
        name="adaln_fused",
    )(A_x, A_wqkv, A_wo, B_w1, B_w3, B_w2, c, w_mod)
```

```python
import functools

import jax
import jax.numpy as jnp
from jax import lax
import jax.experimental.pallas as pl
import jax.experimental.pallas.tpu as pltpu

S, D, F = 2048, 1024, 3584
DH, W, DIL = 32, 8, 2
NG = D // 128
HALO = 16
T = 128
NT = S // T
NP = T // 16
NRB = T // 8
SKEW = 3
M0 = SKEW * T
NS = NT - SKEW
NA = NS // 2
PPI = 2
IPT = NP // PPI
WROWS = HALO + 16 * PPI
FC = 512
NFC = F // FC
KOFF = HALO
KROWS = KOFF + T + 8
LOG2E = 1.4426950408889634
QSCALE = (DH ** -0.5) * LOG2E
NEG = -1e9 * DH ** 0.5
KC = 128
NKC = D // KC
WR = 4
LW = 512
NLP = 4 * D // LW
PADW = 128
EPS = 1e-5
GATES = {"first": (19.0, 0.5, 0.6, 6, 8), 1: (20.0, 0.0, 0.6, 4, 2), 0: (20.0, 0.7, 0.6, 4, 8)}
FPLAN = "aaa/all/flll/lwlll/lwlwl/lllwl"
f32, bf16, u32 = jnp.float32, jnp.bfloat16, jnp.uint32


def _lane_tables():
    lane = lax.broadcasted_iota(jnp.int32, (8, 128), 1)
    head = lane & 31
    masks = [(lane & (4 << s)) != 0 for s in range(3)]
    fwd = [((head & 3) << 5) | (((head >> 2) ^ g) << 2) | (lane >> 5) for g in range(NG)]
    inv = [((lane & 3) << 5) | ((((lane >> 2) & 7) ^ g) << 2) | (lane >> 5) for g in range(NG)]
    return masks, fwd, inv


def _butterfly(vs, masks):
    n = vs[0].shape[0] // 8
    vs = [v.reshape(n, 8, 128) for v in vs]
    for s in range(3):
        for g in range(NG):
            if g & (1 << s):
                continue
            a, b = vs[g], vs[g | (1 << s)]
            vs[g] = jnp.where(masks[s], b, a)
            vs[g | (1 << s)] = jnp.where(masks[s], a, b)
    return [v.reshape(n * 8, 128) for v in vs]


def _gather_lanes(v, idx):
    idx = jnp.concatenate([idx] * (v.shape[0] // 8), axis=0)
    return jnp.take_along_axis(v, idx, axis=1, mode="promise_in_bounds")


def _to_head_lanes(vs, tabs):
    return [_gather_lanes(y, i) for y, i in zip(_butterfly(vs, tabs[0]), tabs[1])]


def _from_head_lanes(zs, tabs):
    return _butterfly([_gather_lanes(z, i) for z, i in zip(zs, tabs[2])], tabs[0])


def _add(a, b):
    return a + b


def _or(a, b):
    return a | b


def _bits(x):
    return pltpu.bitcast(x, u32)


def _dot(a, b):
    return jnp.dot(a, b, preferred_element_type=f32)


def _after(x, dep):
    if dep is None:
        return x
    return pltpu.bitcast(_bits(x) | dep, x.dtype)


def _norm8(xs, dep=None):
    xs = [_after(xs[0], dep)] + list(xs[1:])
    m = jnp.sum(functools.reduce(_add, xs), axis=-1, keepdims=True) * (1.0 / D)
    xc = [v - m for v in xs]
    var = jnp.sum(functools.reduce(_add, [v * v for v in xc]), axis=-1, keepdims=True) * (1.0 / D)
    r = lax.rsqrt(var + EPS)
    return [v * r for v in xc]


def _groups(x):
    return [x[:, g * 128:(g + 1) * 128] for g in range(x.shape[1] // 128)]


def _kernel(x_hbm, wqkv_hbm, wo_hbm, w1_hbm, w3_hbm, w2_hbm, c_hbm, wmod_hbm, out_hbm,
            x_v, c_v, cb_v, wm_v, wl0_v, wl1_v, wraw_v, wpe_v, wpo_v, wo_v, w1_v, w3_v, w2_v, mod_v, modr_v,
            xn_v, he_v, ho_v, h_v, h2_v, x1_v, win_v, st_v, o_v, p0_v, p1_v, a_v, ob_v,
            zv_v, sem, osem):
    names = ["c", "x0", "x1", "x2", "x3", "xr", "wo", "w1", "w3", "w2", "wl0", "wl1"]
    srcdst = dict(
        c=(c_hbm, c_v),
        x0=(x_hbm.at[0, 0:M0, :], x_v.at[0:M0, :]),
        x1=(x_hbm.at[0, M0:M0 + T, :], x_v.at[M0:M0 + T, :]),
        x2=(x_hbm.at[0, M0 + T:M0 + 2 * T, :], x_v.at[M0 + T:M0 + 2 * T, :]),
        x3=(x_hbm.at[0, M0 + 2 * T:M0 + 3 * T, :], x_v.at[M0 + 2 * T:M0 + 3 * T, :]),
        xr=(x_hbm.at[0, M0 + 3 * T:S, :], x_v.at[M0 + 3 * T:S, :]),
        wo=(wo_hbm, wo_v.at[:, 0:D]),
        w1=(w1_hbm, w1_v.at[:, 0:F]), w3=(w3_hbm, w3_v.at[:, 0:F]), w2=(w2_hbm, w2_v.at[:, 0:D]),
    )
    copies = {n: pltpu.make_async_copy(*srcdst[n], sem.at[names.index(n)]) for n in srcdst}
    SEM_C = len(names)
    SEM_W = SEM_C + NKC

    def slab_copy(c, sec):
        cols = pl.ds(pl.multiple_of(sec * D + c * KC, KC), KC)
        return pltpu.make_async_copy(wmod_hbm.at[:, cols], wm_v.at[c, :, sec * KC:(sec + 1) * KC], sem.at[SEM_C + c])

    def chunk_copies(c):
        rows = pl.ds(pl.multiple_of(c * KC, KC), KC)
        return [slab_copy(c, 0), slab_copy(c, 1),
                pltpu.make_async_copy(wqkv_hbm.at[rows, :], wraw_v.at[rows, :], sem.at[SEM_W + c])]

    def late_copy(p, par):
        cols = pl.ds(pl.multiple_of(2 * D + p * LW, LW), LW)
        return pltpu.make_async_copy(wmod_hbm.at[:, cols], (wl0_v, wl1_v)[par], sem.at[names.index("wl0") + par])

    copies["c"].start()
    copies["x0"].start()
    for c in range(NKC):
        for cp in chunk_copies(c):
            cp.start()
    for n in ("x1", "x2", "wo", "x3"):
        copies[n].start()
    late_copy(0, 1).start()
    late_copy(1, 0).start()
    copies["xr"].start()
    for n in ("w1", "w3", "w2"):
        copies[n].start(priority=1)
    zv_v[...] = jnp.zeros(zv_v.shape, u32)

    tabs = _lane_tables()
    proj = (p0_v, p1_v)
    mcol = lambda sec, g: mod_v[sec * NG + g] if sec < 2 else modr_v[(sec - 2) * NG + g]
    row8 = lax.broadcasted_iota(jnp.int32, (8, 128), 0)

    def ln1_rows(xt, drow, dep):
        xn = _norm8(_groups(xt[drow:drow + 8, :].astype(f32)), dep)
        ys = [xn[g] * mcol(1, g) + mcol(0, g) for g in range(NG)]
        h_v[drow:drow + 8, 0:D] = jnp.concatenate(ys, axis=1).astype(bf16)
        return _bits(ys[NG - 1])

    def ln2_rows(t, drow, dep):
        xt, at = x_v.at[pl.ds(t, T), :], a_v.at[:, pl.ds(t, T), :]
        x = _groups(xt[drow:drow + 8, :].astype(f32))
        x1 = [x[g] + mcol(2, g) * at[g, drow:drow + 8, :] for g in range(NG)]
        x1_v[drow:drow + 8, :] = jnp.concatenate(x1, axis=1)
        xn = _norm8(x1, dep)
        ys = [xn[g] * mcol(4, g) + mcol(3, g) for g in range(NG)]
        h2_v[drow:drow + 8, 0:D] = jnp.concatenate(ys, axis=1).astype(bf16)
        return _bits(ys[NG - 1])

    def attn8(src, masked, pb, par, dep):
        r0 = KOFF + 16 * pb + par
        rows = lambda j: pl.ds(r0 - DIL * j, 8, stride=DIL)
        zvec = zv_v[...]
        s = [None] * W
        for g in range(NG):
            q = src[g, rows(0), :]
            if g == 0:
                q = _after(q, dep)
            else:
                q = _after(q, _bits(s[W - 1]) & zvec)
            for j in range(W):
                p = q * src[NG + g, rows(j), :]
                s[j] = p if s[j] is None else s[j] + p
        for j in range(W):
            s[j] = s[j] + pltpu.roll(s[j], 64, 1)
            s[j] = s[j] + pltpu.roll(s[j], 32, 1)
            if masked and pb == 0 and j > 0:
                s[j] = jnp.where(par + DIL * row8 >= DIL * j, s[j], NEG)
        m = functools.reduce(jnp.maximum, s)
        e = [jnp.exp2((s[j] - m) * QSCALE) for j in range(W)]
        den = functools.reduce(_add, e)
        r = pl.reciprocal(den, approx=True)
        inv = r * (2.0 - den * r)
        og = [None] * NG
        for j in range(W):
            p = e[j] * inv
            if j:
                p = _after(p, _bits(og[NG - 1]) & zvec)
            for g in range(NG):
                t = p * src[2 * NG + g, rows(j), :]
                og[g] = t if og[g] is None else og[g] + t
        return og

    def stage(pb, even, odd):
        for g in range(NG):
            st_v[8 * pb:8 * pb + 8, g * 128:(g + 1) * 128] = _bits(
                jnp.concatenate([even[g], odd[g]], axis=0).astype(bf16))

    def unstage(r0, r1):
        return jnp.concatenate(_from_head_lanes(_groups(st_v[r0:r1, :]), tabs), axis=1)

    def out_proj(o, t0, side=None):
        a = _groups(_dot(o, wo_v[:, 0:D]))
        links = side(a) if side is not None else {}
        at = a_v.at[:, pl.ds(t0, o.shape[0] + 8), :]
        for g in range(NG):
            for rb in range(a[g].shape[0] // 8):
                v = a[g][rb * 8:(rb + 1) * 8]
                if rb == 0 and g in links:
                    v = _after(v, links[g])
                at[g, pl.ds((rb // 2) * 16 + rb % 2, 8, stride=2), :] = v

    def mod_vpu(wl, k, part, nparts, dep):
        n = D // nparts
        zvec = zv_v[...]
        acc = None
        for i in range(n // 8):
            rows = slice(part * n + i * 8, part * n + (i + 1) * 8)
            cb = cb_v[rows, :]
            if i % 4 == 0:
                cb = _after(cb, dep if i == 0 else _bits(acc[:, 0:128]) & zvec)
            t = wl[rows, k * 256:(k + 1) * 256].astype(f32) * jnp.concatenate([cb, cb], axis=1)
            acc = t if acc is None else acc + t
        return acc

    def chunk_block(c, par, do_prep, do_mm, extra=None):
        zvec = zv_v[...]
        links = {}

        def link(ct, v):
            links[ct] = (links[ct] | v) if ct in links else v

        def rounds(hc, wp, rs):
            res = {}
            for r in rs:
                out = _groups(_dot(hc, pltpu.bitcast(wp[:, r * 512:(r + 1) * 512], bf16)))
                for n in range(4):
                    res[4 * r + n] = out[n]
            return res

        def accumulate(res):
            for ct in res:
                for t in range(SKEW):
                    blk = res[ct][t * T:(t + 1) * T]
                    if t == SKEW - 1 and ct in links:
                        blk = jnp.concatenate([blk[0:T - 8], _after(blk[T - 8:T], links.pop(ct) & zvec)], axis=0)
                    proj[t % 2][t // 2, ct, KOFF:KOFF + T, :] += blk
        if do_prep:
            for cp in chunk_copies(c):
                cp.wait()
        if do_mm:
            res = rounds((he_v, ho_v)[1 - par][...], (wpe_v, wpo_v)[1 - par].at[(c - 1) >> 1], range(WR, 6))
        if do_prep:
            part = [mod_vpu(wm_v.at[c], 0, h, 4, None) for h in range(4)]
            m = jnp.broadcast_to(jnp.sum(functools.reduce(_add, part), axis=0, keepdims=True), (8, 256))
            sh = m[:, 0:128]
            s1 = m[:, 128:256] + 1.0
            mod_v[c] = sh
            mod_v[NG + c] = s1
            hc = (xn_v[c].reshape(M0 // 8, 8, 128) * s1 + sh).reshape(M0, 128).astype(bf16)
            (he_v, ho_v)[par][...] = hc
            wp = (wpe_v, wpo_v)[par].at[c >> 1]
            for b in range(6):
                sec, half = b // 2, b % 2
                r0 = pl.multiple_of(c * KC + half * 64, 64)
                vs = _groups(_bits(wraw_v[pl.ds(r0, 64), sec * D:(sec + 1) * D]))
                vs = _to_head_lanes(vs, tabs)
                wp[half * 32:(half + 1) * 32, sec * D:(sec + 1) * D] = jnp.concatenate(vs, axis=1)
                if 2 * sec + 2 > WR:
                    link(8 + 3 * half, vs[NG - 1][24:32])
        if extra is not None:
            extra(res, link, zvec)
        if do_mm:
            accumulate(res)
        if do_prep:
            accumulate(rounds(hc, wp, range(WR)))

    def prologue():
        def zero(ct, carry):
            for t in range(SKEW):
                proj[t % 2][t // 2, ct, KOFF:KOFF + T, :] = jnp.zeros((T, 128), f32)
            return carry
        lax.fori_loop(0, 3 * NG, zero, 0)
        copies["c"].wait()
        c32 = c_v[...].astype(f32)
        sc = (c32 * jax.nn.sigmoid(c32)).astype(bf16)
        diag = lax.broadcasted_iota(jnp.int32, (128, 128), 0) == lax.broadcasted_iota(jnp.int32, (128, 128), 1)
        for g, row in enumerate(_groups(sc.astype(f32))):
            col = jnp.sum(jnp.where(diag, row, 0.0), axis=1, keepdims=True)
            cb_v[g * 128:(g + 1) * 128, :] = jnp.broadcast_to(col, (128, 128))
        copies["x0"].wait()

        def stats(i, carry):
            for rb in range(12):
                rows = pl.ds(pl.multiple_of(i * 96, 32) + rb * 8, 8)
                xn = _norm8(_groups(x_v[rows, :].astype(f32)))
                for g in range(NG):
                    xn_v[g, rows, :] = xn[g]
            return carry
        lax.fori_loop(0, M0 // 96, stats, 0)
        chunk_block(0, 0, True, False)

        def kloop(i, carry):
            chunk_block(2 * i + 1, 1, True, True)

            @pl.when(2 * i + 2 < NKC)
            def _():
                chunk_block(2 * i + 2, 0, True, True)
            return carry
        lax.fori_loop(0, NKC // 2, kloop, 0)

        copies["x1"].wait()

        def ln_next(res, link, zvec):
            for rb in range(T // 8):
                ct = 4 * WR + (rb * (20 - 4 * WR)) // (T // 8)
                link(ct + 3, ln1_rows(x_v.at[M0:M0 + T, :], rb * 8, _bits(res[ct][M0 - 8:M0]) & zvec))
        chunk_block(NKC, 0, False, True, ln_next)
        for t in range(SKEW):
            for sg in range(NG, 3 * NG):
                if t == 0:
                    halo = jnp.broadcast_to(p0_v[0, sg, KOFF:KOFF + 1, :], (HALO, 128))
                else:
                    halo = proj[(t - 1) % 2][(t - 1) // 2, sg, KOFF + T - HALO:KOFF + T, :]
                proj[t % 2][t // 2, sg, KOFF - HALO:KOFF, :] = halo
        copies["x2"].wait()

    def step(s, par, first=False, last=False):
        GS, GA, GL, LL, UG = GATES["first" if first else par]
        zvec = zv_v[...]
        t0 = s * T if first or last else pl.multiple_of(s * T, T)
        slot = (s >> 1) & 1
        dst = proj[1 - par].at[((s + SKEW) >> 1) & 1]
        prev = proj[par].at[1 - slot]
        w = jnp.concatenate([(wpe_v, wpo_v)[c % 2][c // 2, :, 0:3 * D] for c in range(NKC)], axis=0)
        tiles = _groups(_dot(h_v[:, 0:D], pltpu.bitcast(w, bf16)))
        for ct in range(3 * NG):
            dst[ct, KOFF:KOFF + T, :] = tiles[ct]
            if ct >= NG:
                dst[ct, KOFF - HALO:KOFF, :] = prev[ct, KOFF + T - HALO:KOFF + T, :]
        t1 = t0 + (SKEW + 1) * T
        src = proj[par].at[slot]
        links, rows = [], []

        def gate(pos):
            ct = int(pos)
            rb = min(T // 8 - 1, int((pos - ct) * (T // 8)))
            return _bits(tiles[ct][rb * 8:(rb + 1) * 8, :]) & zvec

        for pb in range(NP):
            halves = []
            for k in (2 * pb, 2 * pb + 1):
                d = gate(GA + GS * k / NRB)
                if k >= LL:
                    d = d | (links[k - LL] & zvec)
                halves.append(attn8(src, first, pb, k % 2, d))
            stage(pb, *halves)
            for rb in (2 * pb, 2 * pb + 1):
                d = gate(GA + GL + GS * rb / NRB)
                links.append(ln2_rows(0, rb * 8, d) if last else ln1_rows(x_v.at[pl.ds(t1, T), :], rb * 8, d))
            if (pb + 1) % UG == 0:
                rows.append(pltpu.bitcast(unstage((pb + 1 - UG) * 8, (pb + 1) * 8), bf16))

        def mods(a):
            links = {}
            ev = tiles[3 * NG - 2:] + a
            piece = jnp.minimum(s - 1, NLP - 1 - par)
            for k in range(LW // 256):
                part = [mod_vpu((wl0_v, wl1_v)[par], k, h, 2, _bits(ev[(7 * (2 * k + h)) // 4][T - 8:T]) & zvec)
                        for h in range(2)]
                m = jnp.sum(part[0] + part[1], axis=0, keepdims=True)
                m = jnp.broadcast_to(m + jnp.where(piece >> 1 == 2, 1.0, 0.0), (8, 256))
                modr_v[4 * piece + 2 * k] = m[:, 0:128]
                modr_v[4 * piece + 2 * k + 1] = m[:, 128:256]
                links[5 + 2 * k] = _bits(m[:, 0:128]) & zvec
            return links

        def handover(a):
            links = {}
            ev = tiles[3 * NG - 2:] + a
            for k in range(4):
                links[k + 3] = fill_window(0, range(6 * k, 6 * k + 6), _bits(ev[k + 2][T - 8:T]) & zvec) & zvec
            for k in range(6):
                seen = []
                for sg in range(4 * k, 4 * k + 4):
                    lo = KOFF if sg < NG else KOFF - HALO
                    for r in range(lo, KOFF + T, 8):
                        v = p0_v[1, sg, r:r + 8, :]
                        if not seen:
                            v = _after(v, _bits(ev[k + 1][T - 8:T]) & zvec)
                        p1_v[2, sg, r:r + 8, :] = v
                        seen.append(_bits(v))
                lk = functools.reduce(_or, seen) & zvec
                links[k + 2] = (links[k + 2] | lk) if k + 2 in links else lk
            return links
        if first:
            copies["wo"].wait()
            out_proj(jnp.concatenate(rows, axis=0), t0)
        elif last:
            out_proj(jnp.concatenate(rows, axis=0), t0, handover)
        else:
            out_proj(jnp.concatenate(rows, axis=0), t0, mods)

            @pl.when(s + 1 < NLP)
            def _():
                late_copy(s + 1, par).start()

    def phase_a(i):
        @pl.when(i == 0)
        def _():
            prologue()
            step(0, 0, first=True)

        @pl.when(i == 0)
        def _():
            copies["x3"].wait()

        @pl.when(2 * i < NLP)
        def _():
            late_copy(2 * i, 1).wait()
        step(2 * i + 1, 1)

        @pl.when(i < NA - 1)
        def _():
            @pl.when(i == 0)
            def _():
                copies["xr"].wait()

            @pl.when(2 * i + 1 < NLP)
            def _():
                late_copy(2 * i + 1, 0).wait()
            step(2 * i + 2, 0)

        @pl.when(i == NA - 1)
        def _():
            for n in ("w1", "w3", "w2"):
                copies[n].wait()
            step(NS - 1, 0, last=True)

    def fill_window(i, sgs, dep):
        row = (i % IPT) * 16 * PPI
        src = p1_v.at[(i // IPT) % 3, :, pl.ds(row if isinstance(i, int) else pl.multiple_of(row, 16 * PPI), WROWS), :]
        seen = []
        for sg in sgs:
            lo = KOFF if sg < NG else KOFF - HALO
            v = src[sg, lo:WROWS, :]
            if not seen:
                v = jnp.concatenate([_after(v[0:8], dep), v[8:]], axis=0)
            win_v[sg, lo:WROWS, :] = v
            seen += [_bits(v[r:r + 8]) for r in range(0, WROWS - lo, 8)]
        return functools.reduce(_or, seen)

    def phase_b(i):
        i = i - NA
        t1 = pl.multiple_of(jnp.minimum(i + 1, NT - 1) * T, T)
        zvec = zv_v[...]
        sl = (i // IPT) % 3
        orow = jnp.where(sl == 0, 0, jnp.where(sl == 1, T, T // 2)) + (i % IPT) * 8 * PPI

        def fin(dep):
            o = unstage(0, 8 * PPI)
            o_v[pl.ds(pl.multiple_of(orow, 8 * PPI), 8 * PPI), :] = o
            return o[8 * PPI - 8:8 * PPI, D - 128:D]
        halves = []

        def att(n):
            def run(d):
                halves.append(attn8(win_v, False, n // 2, n % 2, d))
                if n % 2:
                    stage(n // 2, *halves[-2:])
                return _bits(halves[-1][NG - 1])
            return run
        ln = lambda r: (lambda d: ln2_rows(t1, r * 8, d))
        fw = lambda k: (lambda d: fill_window(i + 1, range(6 * k, 6 * k + 6), d))
        code = {"a": att, "f": lambda n: fin, "l": ln, "w": fw}
        cnt = dict.fromkeys(code, 0)
        side = []
        for chunk in FPLAN.split("/"):
            side.append([])
            for c in chunk:
                side[-1].append(code[c](cnt[c]))
                cnt[c] += 1
        assert cnt == {"a": 2 * PPI, "f": 1, "l": NRB, "w": 4}, cnt
        h = h2_v[:, 0:D]
        gb = jnp.concatenate([mcol(5, g) for g in range(NG)], axis=1)
        scaled = lambda y: (y.reshape(NRB, 8, D) * gb).reshape(T, D)
        acc = act_prev = None
        links = []
        for fc in range(NFC + 1):
            ev = []
            if fc < NFC:
                g = _dot(h, w1_v[:, fc * FC:(fc + 1) * FC])
                u = _dot(h, w3_v[:, fc * FC:(fc + 1) * FC])
                ev = _groups(g) + _groups(u)
                if 1 <= fc <= len(side):
                    u0 = _after(u[T - 8:T, FC - 128:FC], functools.reduce(_or, links[fc - 1]) & zvec)
                    u = jnp.concatenate([u[0:T - 8, :], jnp.concatenate([u[T - 8:T, 0:FC - 128], u0], axis=1)], axis=0)
                hg = 0.5 * g
                act = (hg * (1.0 + jnp.tanh(hg)) * u).astype(bf16)
            if fc >= 1:
                y = _dot(act_prev, w2_v[(fc - 1) * FC:fc * FC, 0:D])
                ev = ev + _groups(y)
                acc = (x1_v[...] if acc is None else acc) + scaled(y)
            if fc < len(side):
                n = len(side[fc])
                pos = [4 + (k * 12) // n if fc else 3 + (k * 5) // n for k in range(n)]
                links.append([fn(_bits(ev[p][T - 16:T - 8]) & zvec) for p, fn in zip(pos, side[fc])])
            act_prev = act
        rows = pl.ds(pl.multiple_of(i * T, T), T)
        for half in range(2):
            cols = slice(half * (D // 2), (half + 1) * (D // 2))
            ob_v[rows, cols] = acc[:, cols].astype(bf16)
            pltpu.make_async_copy(ob_v.at[rows, cols], out_hbm.at[0, rows, cols], osem.at[0]).start()

        def late_proj(t, carry):
            rows = pl.ds(pl.multiple_of(t * (M0 // 4), M0 // 4), M0 // 4)
            out_proj(pltpu.bitcast(o_v[rows, :], bf16), pl.multiple_of(NS * T + t * (M0 // 2), 64))
            return carry
        lax.fori_loop(0, jnp.where(i == SKEW * IPT - 1, 2, 0), late_proj, 0)

    def main(i, carry):
        lax.cond(i < NA, phase_a, phase_b, i)
        return carry
    lax.fori_loop(0, NA + NT, main, 0)
    pltpu.make_async_copy(ob_v, out_hbm.at[0], osem.at[0]).wait()


@jax.jit
def pallas_adaLN_cond__sliding_local_dilated__glu_gated_swiglu__prompt_kernel(
    A_x, A_wqkv, A_wo, B_x, B_w1, B_w3, B_w2, c, w_mod):
    del B_x
    any_spec = pl.BlockSpec(memory_space=pl.ANY)
    return pl.pallas_call(
        _kernel,
        out_shape=jax.ShapeDtypeStruct((1, S, D), bf16),
        in_specs=[any_spec] * 8,
        out_specs=any_spec,
        scratch_shapes=[
            pltpu.VMEM((S, D), bf16),
            pltpu.VMEM((1, D), bf16),
            pltpu.VMEM((D, 128), f32),
            pltpu.VMEM((NKC, D, 2 * KC), bf16),
            pltpu.VMEM((D, LW), bf16),
            pltpu.VMEM((D, LW), bf16),
            pltpu.VMEM((D, 3 * D), bf16),
            pltpu.VMEM((NKC // 2, KC // 2, 3 * D + PADW), u32),
            pltpu.VMEM((NKC // 2, KC // 2, 3 * D + PADW), u32),
            pltpu.VMEM((D, D + PADW), bf16),
            pltpu.VMEM((D, F + PADW), bf16),
            pltpu.VMEM((D, F + PADW), bf16),
            pltpu.VMEM((F, D + PADW), bf16),
            pltpu.VMEM((2 * NG, 8, 128), f32),
            pltpu.VMEM((4 * NG, 8, 128), f32),
            pltpu.VMEM((NG, M0, 128), f32),
            pltpu.VMEM((M0, KC), bf16),
            pltpu.VMEM((M0, KC), bf16),
            pltpu.VMEM((T, D + PADW), bf16),
            pltpu.VMEM((T, D + PADW), bf16),
            pltpu.VMEM((T, D), f32),
            pltpu.VMEM((3 * NG, WROWS + 8, 128), f32),
            pltpu.VMEM((T // 2, D), u32),
            pltpu.VMEM((M0 // 2, D), u32),
            pltpu.VMEM((2, 3 * NG, KROWS, 128), f32),
            pltpu.VMEM((3, 3 * NG, KROWS, 128), f32),
            pltpu.VMEM((NG, S + 8, 128), f32),
            pltpu.VMEM((S, D), bf16),
            pltpu.VMEM((8, 128), u32),
            pltpu.SemaphoreType.DMA((12 + 2 * NKC,)),
            pltpu.SemaphoreType.DMA((1,)),
        ],
        compiler_params=pltpu.CompilerParams(vmem_limit_bytes=110 * 2**20, disable_bounds_checks=True,
                                             disable_semaphore_checks=True),
        name="adaln_fused",
    )(A_x, A_wqkv, A_wo, B_w1, B_w3, B_w2, c, w_mod)
```

```python
import functools

import jax
import jax.numpy as jnp
from jax import lax
import jax.experimental.pallas as pl
import jax.experimental.pallas.tpu as pltpu

S, D, F = 2048, 1024, 3584
DH, W, DIL = 32, 8, 2
NG = D // 128
HALO = 16
T = 128
NT = S // T
NP = T // 16
NRB = T // 8
SKEW = 3
M0 = SKEW * T
NS = NT - SKEW
NA = NS // 2
PPI = 2
IPT = NP // PPI
WROWS = HALO + 16 * PPI
FC = 512
NFC = F // FC
KOFF = HALO
KROWS = KOFF + T + 8
LOG2E = 1.4426950408889634
QSCALE = (DH ** -0.5) * LOG2E
NEG = -1e9 * DH ** 0.5
KC = 128
NKC = D // KC
WR = 4
LW = 512
NLP = 4 * D // LW
PADW = 128
EPS = 1e-5
GATES = {"first": (19.0, 0.5, 0.6, 6, 8), 1: (20.0, 0.0, 0.6, 4, 2), 0: (20.0, 0.7, 0.6, 4, 8)}
FPLAN = "aaa/all/flll/lwlll/lwlwl/lllwl"
f32, bf16, u32 = jnp.float32, jnp.bfloat16, jnp.uint32


def _lane_tables():
    lane = lax.broadcasted_iota(jnp.int32, (8, 128), 1)
    head = lane & 31
    masks = [(lane & (4 << s)) != 0 for s in range(3)]
    fwd = [((head & 3) << 5) | (((head >> 2) ^ g) << 2) | (lane >> 5) for g in range(NG)]
    inv = [((lane & 3) << 5) | ((((lane >> 2) & 7) ^ g) << 2) | (lane >> 5) for g in range(NG)]
    return masks, fwd, inv


def _butterfly(vs, masks):
    n = vs[0].shape[0] // 8
    vs = [v.reshape(n, 8, 128) for v in vs]
    for s in range(3):
        for g in range(NG):
            if g & (1 << s):
                continue
            a, b = vs[g], vs[g | (1 << s)]
            vs[g] = jnp.where(masks[s], b, a)
            vs[g | (1 << s)] = jnp.where(masks[s], a, b)
    return [v.reshape(n * 8, 128) for v in vs]


def _gather_lanes(v, idx):
    idx = jnp.concatenate([idx] * (v.shape[0] // 8), axis=0)
    return jnp.take_along_axis(v, idx, axis=1, mode="promise_in_bounds")


def _to_head_lanes(vs, tabs):
    return [_gather_lanes(y, i) for y, i in zip(_butterfly(vs, tabs[0]), tabs[1])]


def _from_head_lanes(zs, tabs):
    return _butterfly([_gather_lanes(z, i) for z, i in zip(zs, tabs[2])], tabs[0])


def _add(a, b):
    return a + b


def _or(a, b):
    return a | b


def _bits(x):
    return pltpu.bitcast(x, u32)


def _dot(a, b):
    return jnp.dot(a, b, preferred_element_type=f32)


def _after(x, dep):
    if dep is None:
        return x
    return pltpu.bitcast(_bits(x) | dep, x.dtype)


def _norm8(xs, dep=None):
    xs = [_after(xs[0], dep)] + list(xs[1:])
    m = jnp.sum(functools.reduce(_add, xs), axis=-1, keepdims=True) * (1.0 / D)
    xc = [v - m for v in xs]
    var = jnp.sum(functools.reduce(_add, [v * v for v in xc]), axis=-1, keepdims=True) * (1.0 / D)
    r = lax.rsqrt(var + EPS)
    return [v * r for v in xc]


def _groups(x):
    return [x[:, g * 128:(g + 1) * 128] for g in range(x.shape[1] // 128)]


def _kernel(x_hbm, wqkv_hbm, wo_hbm, w1_hbm, w3_hbm, w2_hbm, c_hbm, wmod_hbm, out_hbm,
            x_v, c_v, cb_v, wm_v, wl0_v, wl1_v, wraw_v, wpe_v, wpo_v, wo_v, w1_v, w3_v, w2_v, mod_v, modr_v,
            xn_v, he_v, ho_v, h_v, h2_v, x1_v, win_v, st_v, o_v, p0_v, p1_v, a_v, ob_v,
            zv_v, sem, osem):
    names = ["c", "x0", "x1", "x2", "x3", "xr", "wo", "w1", "w3", "w2", "wl0", "wl1"]
    srcdst = dict(
        c=(c_hbm, c_v),
        x0=(x_hbm.at[0, 0:M0, :], x_v.at[0:M0, :]),
        x1=(x_hbm.at[0, M0:M0 + T, :], x_v.at[M0:M0 + T, :]),
        x2=(x_hbm.at[0, M0 + T:M0 + 2 * T, :], x_v.at[M0 + T:M0 + 2 * T, :]),
        x3=(x_hbm.at[0, M0 + 2 * T:M0 + 3 * T, :], x_v.at[M0 + 2 * T:M0 + 3 * T, :]),
        xr=(x_hbm.at[0, M0 + 3 * T:S, :], x_v.at[M0 + 3 * T:S, :]),
        wo=(wo_hbm, wo_v.at[:, 0:D]),
        w1=(w1_hbm, w1_v.at[:, 0:F]), w3=(w3_hbm, w3_v.at[:, 0:F]), w2=(w2_hbm, w2_v.at[:, 0:D]),
    )
    copies = {n: pltpu.make_async_copy(*srcdst[n], sem.at[names.index(n)]) for n in srcdst}
    SEM_C = len(names)
    SEM_W = SEM_C + NKC

    def slab_copy(c, sec):
        cols = pl.ds(pl.multiple_of(sec * D + c * KC, KC), KC)
        return pltpu.make_async_copy(wmod_hbm.at[:, cols], wm_v.at[c, :, sec * KC:(sec + 1) * KC], sem.at[SEM_C + c])

    def chunk_copies(c):
        rows = pl.ds(pl.multiple_of(c * KC, KC), KC)
        return [slab_copy(c, 0), slab_copy(c, 1),
                pltpu.make_async_copy(wqkv_hbm.at[rows, :], wraw_v.at[rows, :], sem.at[SEM_W + c])]

    def late_copy(p, par):
        cols = pl.ds(pl.multiple_of(2 * D + p * LW, LW), LW)
        return pltpu.make_async_copy(wmod_hbm.at[:, cols], (wl0_v, wl1_v)[par], sem.at[names.index("wl0") + par])

    copies["c"].start()
    copies["x0"].start()
    for c in range(NKC):
        for cp in chunk_copies(c):
            cp.start()
    for n in ("x1", "x2", "wo", "x3"):
        copies[n].start()
    late_copy(0, 1).start()
    late_copy(1, 0).start()
    copies["xr"].start()
    for n in ("w1", "w3", "w2"):
        copies[n].start(priority=1)
    zv_v[...] = jnp.zeros(zv_v.shape, u32)

    tabs = _lane_tables()
    proj = (p0_v, p1_v)
    mcol = lambda sec, g: mod_v[sec * NG + g] if sec < 2 else modr_v[(sec - 2) * NG + g]
    row8 = lax.broadcasted_iota(jnp.int32, (8, 128), 0)

    def ln1_rows(xt, drow, dep):
        xn = _norm8(_groups(xt[drow:drow + 8, :].astype(f32)), dep)
        ys = [xn[g] * mcol(1, g) + mcol(0, g) for g in range(NG)]
        h_v[drow:drow + 8, 0:D] = jnp.concatenate(ys, axis=1).astype(bf16)
        return _bits(ys[NG - 1])

    def ln2_rows(t, drow, dep):
        xt, at = x_v.at[pl.ds(t, T), :], a_v.at[:, pl.ds(t, T), :]
        x = _groups(xt[drow:drow + 8, :].astype(f32))
        x1 = [x[g] + mcol(2, g) * at[g, drow:drow + 8, :] for g in range(NG)]
        x1_v[drow:drow + 8, :] = jnp.concatenate(x1, axis=1)
        xn = _norm8(x1, dep)
        ys = [xn[g] * mcol(4, g) + mcol(3, g) for g in range(NG)]
        h2_v[drow:drow + 8, 0:D] = jnp.concatenate(ys, axis=1).astype(bf16)
        return _bits(ys[NG - 1])

    def attn8(src, masked, pb, par, dep):
        r0 = KOFF + 16 * pb + par
        rows = lambda j: pl.ds(r0 - DIL * j, 8, stride=DIL)
        zvec = zv_v[...]
        s = [None] * W
        for g in range(NG):
            q = src[g, rows(0), :]
            if g == 0:
                q = _after(q, dep)
            else:
                q = _after(q, _bits(s[W - 1]) & zvec)
            for j in range(W):
                p = q * src[NG + g, rows(j), :]
                s[j] = p if s[j] is None else s[j] + p
        for j in range(W):
            s[j] = s[j] + pltpu.roll(s[j], 64, 1)
            s[j] = s[j] + pltpu.roll(s[j], 32, 1)
            if masked and pb == 0 and j > 0:
                s[j] = jnp.where(par + DIL * row8 >= DIL * j, s[j], NEG)
        m = functools.reduce(jnp.maximum, s)
        e = [jnp.exp2((s[j] - m) * QSCALE) for j in range(W)]
        den = functools.reduce(_add, e)
        r = pl.reciprocal(den, approx=True)
        inv = r * (2.0 - den * r)
        og = [None] * NG
        for j in range(W):
            p = e[j] * inv
            if j:
                p = _after(p, _bits(og[NG - 1]) & zvec)
            for g in range(NG):
                t = p * src[2 * NG + g, rows(j), :]
                og[g] = t if og[g] is None else og[g] + t
        return og

    def stage(pb, even, odd):
        for g in range(NG):
            st_v[8 * pb:8 * pb + 8, g * 128:(g + 1) * 128] = _bits(
                jnp.concatenate([even[g], odd[g]], axis=0).astype(bf16))

    def unstage(r0, r1):
        return jnp.concatenate(_from_head_lanes(_groups(st_v[r0:r1, :]), tabs), axis=1)

    def out_proj(o, t0, side=None):
        a = _groups(_dot(o, wo_v[:, 0:D]))
        links = side(a) if side is not None else {}
        at = a_v.at[:, pl.ds(t0, o.shape[0] + 8), :]
        for g in range(NG):
            for rb in range(a[g].shape[0] // 8):
                v = a[g][rb * 8:(rb + 1) * 8]
                if rb == 0 and g in links:
                    v = _after(v, links[g])
                at[g, pl.ds((rb // 2) * 16 + rb % 2, 8, stride=2), :] = v

    def mod_vpu(wl, k, part, nparts, dep):
        n = D // nparts
        zvec = zv_v[...]
        acc = None
        for i in range(n // 8):
            rows = slice(part * n + i * 8, part * n + (i + 1) * 8)
            cb = cb_v[rows, :]
            if i % 4 == 0:
                cb = _after(cb, dep if i == 0 else _bits(acc[:, 0:128]) & zvec)
            t = wl[rows, k * 256:(k + 1) * 256].astype(f32) * jnp.concatenate([cb, cb], axis=1)
            acc = t if acc is None else acc + t
        return acc

    def chunk_block(c, par, do_prep, do_mm, extra=None):
        zvec = zv_v[...]
        links = {}

        def link(ct, v):
            links[ct] = (links[ct] | v) if ct in links else v

        def rounds(hc, wp, rs):
            res = {}
            for r in rs:
                out = _groups(_dot(hc, pltpu.bitcast(wp[:, r * 512:(r + 1) * 512], bf16)))
                for n in range(4):
                    res[4 * r + n] = out[n]
            return res

        def accumulate(res):
            for ct in res:
                for t in range(SKEW):
                    blk = res[ct][t * T:(t + 1) * T]
                    if t == SKEW - 1 and ct in links:
                        blk = jnp.concatenate([blk[0:T - 8], _after(blk[T - 8:T], links.pop(ct) & zvec)], axis=0)
                    proj[t % 2][t // 2, ct, KOFF:KOFF + T, :] += blk
        if do_prep:
            for cp in chunk_copies(c):
                cp.wait()
        if do_mm:
            res = rounds((he_v, ho_v)[1 - par][...], (wpe_v, wpo_v)[1 - par].at[(c - 1) >> 1], range(WR, 6))
        if do_prep:
            part = [mod_vpu(wm_v.at[c], 0, h, 4, None) for h in range(4)]
            m = jnp.broadcast_to(jnp.sum(functools.reduce(_add, part), axis=0, keepdims=True), (8, 256))
            sh = m[:, 0:128]
            s1 = m[:, 128:256] + 1.0
            mod_v[c] = sh
            mod_v[NG + c] = s1
            hc = (xn_v[c].reshape(M0 // 8, 8, 128) * s1 + sh).reshape(M0, 128).astype(bf16)
            (he_v, ho_v)[par][...] = hc
            wp = (wpe_v, wpo_v)[par].at[c >> 1]
            for b in range(6):
                sec, half = b // 2, b % 2
                r0 = pl.multiple_of(c * KC + half * 64, 64)
                vs = _groups(_bits(wraw_v[pl.ds(r0, 64), sec * D:(sec + 1) * D]))
                vs = _to_head_lanes(vs, tabs)
                wp[half * 32:(half + 1) * 32, sec * D:(sec + 1) * D] = jnp.concatenate(vs, axis=1)
                if 2 * sec + 2 > WR:
                    link(8 + 3 * half, vs[NG - 1][24:32])
        if extra is not None:
            extra(res, link, zvec)
        if do_mm:
            accumulate(res)
        if do_prep:
            accumulate(rounds(hc, wp, range(WR)))

    def prologue():
        def zero(ct, carry):
            for t in range(SKEW):
                proj[t % 2][t // 2, ct, KOFF:KOFF + T, :] = jnp.zeros((T, 128), f32)
            return carry
        lax.fori_loop(0, 3 * NG, zero, 0)
        copies["c"].wait()
        c32 = c_v[...].astype(f32)
        sc = (c32 * jax.nn.sigmoid(c32)).astype(bf16)
        diag = lax.broadcasted_iota(jnp.int32, (128, 128), 0) == lax.broadcasted_iota(jnp.int32, (128, 128), 1)
        for g, row in enumerate(_groups(sc.astype(f32))):
            col = jnp.sum(jnp.where(diag, row, 0.0), axis=1, keepdims=True)
            cb_v[g * 128:(g + 1) * 128, :] = jnp.broadcast_to(col, (128, 128))
        copies["x0"].wait()

        def stats(i, carry):
            for rb in range(12):
                rows = pl.ds(pl.multiple_of(i * 96, 32) + rb * 8, 8)
                xn = _norm8(_groups(x_v[rows, :].astype(f32)))
                for g in range(NG):
                    xn_v[g, rows, :] = xn[g]
            return carry
        lax.fori_loop(0, M0 // 96, stats, 0)
        chunk_block(0, 0, True, False)

        def kloop(i, carry):
            chunk_block(2 * i + 1, 1, True, True)

            @pl.when(2 * i + 2 < NKC)
            def _():
                chunk_block(2 * i + 2, 0, True, True)
            return carry
        lax.fori_loop(0, NKC // 2, kloop, 0)

        copies["x1"].wait()

        def ln_next(res, link, zvec):
            for rb in range(T // 8):
                ct = 4 * WR + (rb * (20 - 4 * WR)) // (T // 8)
                link(ct + 3, ln1_rows(x_v.at[M0:M0 + T, :], rb * 8, _bits(res[ct][M0 - 8:M0]) & zvec))
        chunk_block(NKC, 0, False, True, ln_next)
        for t in range(SKEW):
            for sg in range(NG, 3 * NG):
                if t == 0:
                    halo = jnp.broadcast_to(p0_v[0, sg, KOFF:KOFF + 1, :], (HALO, 128))
                else:
                    halo = proj[(t - 1) % 2][(t - 1) // 2, sg, KOFF + T - HALO:KOFF + T, :]
                proj[t % 2][t // 2, sg, KOFF - HALO:KOFF, :] = halo
        copies["x2"].wait()

    def step(s, par, first=False, last=False):
        GS, GA, GL, LL, UG = GATES["first" if first else par]
        zvec = zv_v[...]
        t0 = s * T if first or last else pl.multiple_of(s * T, T)
        slot = (s >> 1) & 1
        dst = proj[1 - par].at[((s + SKEW) >> 1) & 1]
        prev = proj[par].at[1 - slot]
        w = jnp.concatenate([(wpe_v, wpo_v)[c % 2][c // 2, :, 0:3 * D] for c in range(NKC)], axis=0)
        tiles = _groups(_dot(h_v[:, 0:D], pltpu.bitcast(w, bf16)))
        for ct in range(3 * NG):
            dst[ct, KOFF:KOFF + T, :] = tiles[ct]
            if ct >= NG:
                dst[ct, KOFF - HALO:KOFF, :] = prev[ct, KOFF + T - HALO:KOFF + T, :]
        t1 = t0 + (SKEW + 1) * T
        src = proj[par].at[slot]
        links, rows = [], []

        def gate(pos):
            ct = int(pos)
            rb = min(T // 8 - 1, int((pos - ct) * (T // 8)))
            return _bits(tiles[ct][rb * 8:(rb + 1) * 8, :]) & zvec

        for pb in range(NP):
            halves = []
            for k in (2 * pb, 2 * pb + 1):
                d = gate(GA + GS * k / NRB)
                if k >= LL:
                    d = d | (links[k - LL] & zvec)
                halves.append(attn8(src, first, pb, k % 2, d))
            stage(pb, *halves)
            for rb in (2 * pb, 2 * pb + 1):
                d = gate(GA + GL + GS * rb / NRB)
                links.append(ln2_rows(0, rb * 8, d) if last else ln1_rows(x_v.at[pl.ds(t1, T), :], rb * 8, d))
            if (pb + 1) % UG == 0:
                rows.append(pltpu.bitcast(unstage((pb + 1 - UG) * 8, (pb + 1) * 8), bf16))

        def mods(a):
            links = {}
            ev = tiles[3 * NG - 2:] + a
            piece = jnp.minimum(s - 1, NLP - 1 - par)
            for k in range(LW // 256):
                part = [mod_vpu((wl0_v, wl1_v)[par], k, h, 2, _bits(ev[(7 * (2 * k + h)) // 4][T - 8:T]) & zvec)
                        for h in range(2)]
                m = jnp.sum(part[0] + part[1], axis=0, keepdims=True)
                m = jnp.broadcast_to(m + jnp.where(piece >> 1 == 2, 1.0, 0.0), (8, 256))
                modr_v[4 * piece + 2 * k] = m[:, 0:128]
                modr_v[4 * piece + 2 * k + 1] = m[:, 128:256]
                links[5 + 2 * k] = _bits(m[:, 0:128]) & zvec
            return links

        def handover(a):
            links = {}
            ev = tiles[3 * NG - 2:] + a
            for k in range(4):
                links[k + 3] = fill_window(0, range(6 * k, 6 * k + 6), _bits(ev[k + 2][T - 8:T]) & zvec) & zvec
            for k in range(6):
                seen = []
                for sg in range(4 * k, 4 * k + 4):
                    lo = KOFF if sg < NG else KOFF - HALO
                    for r in range(lo, KOFF + T, 8):
                        v = p0_v[1, sg, r:r + 8, :]
                        if not seen:
                            v = _after(v, _bits(ev[k + 1][T - 8:T]) & zvec)
                        p1_v[2, sg, r:r + 8, :] = v
                        seen.append(_bits(v))
                lk = functools.reduce(_or, seen) & zvec
                links[k + 2] = (links[k + 2] | lk) if k + 2 in links else lk
            return links
        if first:
            copies["wo"].wait()
            out_proj(jnp.concatenate(rows, axis=0), t0)
        elif last:
            out_proj(jnp.concatenate(rows, axis=0), t0, handover)
        else:
            out_proj(jnp.concatenate(rows, axis=0), t0, mods)

            @pl.when(s + 1 < NLP)
            def _():
                late_copy(s + 1, par).start()

    def phase_a(i):
        @pl.when(i == 0)
        def _():
            prologue()
            step(0, 0, first=True)

        @pl.when(i == 0)
        def _():
            copies["x3"].wait()

        @pl.when(2 * i < NLP)
        def _():
            late_copy(2 * i, 1).wait()
        step(2 * i + 1, 1)

        @pl.when(i < NA - 1)
        def _():
            @pl.when(i == 0)
            def _():
                copies["xr"].wait()

            @pl.when(2 * i + 1 < NLP)
            def _():
                late_copy(2 * i + 1, 0).wait()
            step(2 * i + 2, 0)

        @pl.when(i == NA - 1)
        def _():
            for n in ("w1", "w3", "w2"):
                copies[n].wait()
            step(NS - 1, 0, last=True)

    def fill_window(i, sgs, dep):
        row = (i % IPT) * 16 * PPI
        src = p1_v.at[(i // IPT) % 3, :, pl.ds(row if isinstance(i, int) else pl.multiple_of(row, 16 * PPI), WROWS), :]
        seen = []
        for sg in sgs:
            lo = KOFF if sg < NG else KOFF - HALO
            v = src[sg, lo:WROWS, :]
            if not seen:
                v = jnp.concatenate([_after(v[0:8], dep), v[8:]], axis=0)
            win_v[sg, lo:WROWS, :] = v
            seen += [_bits(v[r:r + 8]) for r in range(0, WROWS - lo, 8)]
        return functools.reduce(_or, seen)

    def phase_b(i):
        i = i - NA
        t1 = pl.multiple_of(jnp.minimum(i + 1, NT - 1) * T, T)
        zvec = zv_v[...]
        sl = (i // IPT) % 3
        orow = jnp.where(sl == 0, 0, jnp.where(sl == 1, T, T // 2)) + (i % IPT) * 8 * PPI

        def fin(dep):
            o = unstage(0, 8 * PPI)
            o_v[pl.ds(pl.multiple_of(orow, 8 * PPI), 8 * PPI), :] = o
            return o[8 * PPI - 8:8 * PPI, D - 128:D]
        halves = []

        def att(n):
            def run(d):
                halves.append(attn8(win_v, False, n // 2, n % 2, d))
                if n % 2:
                    stage(n // 2, *halves[-2:])
                return _bits(halves[-1][NG - 1])
            return run
        ln = lambda r: (lambda d: ln2_rows(t1, r * 8, d))
        fw = lambda k: (lambda d: fill_window(i + 1, range(6 * k, 6 * k + 6), d))
        code = {"a": att, "f": lambda n: fin, "l": ln, "w": fw}
        cnt = dict.fromkeys(code, 0)
        side = []
        for chunk in FPLAN.split("/"):
            side.append([])
            for c in chunk:
                side[-1].append(code[c](cnt[c]))
                cnt[c] += 1
        assert cnt == {"a": 2 * PPI, "f": 1, "l": NRB, "w": 4}, cnt
        h = h2_v[:, 0:D]
        gb = jnp.concatenate([mcol(5, g) for g in range(NG)], axis=1)
        scaled = lambda y: (y.reshape(NRB, 8, D) * gb).reshape(T, D)
        acc = act_prev = None
        links = []
        for fc in range(NFC + 1):
            ev = []
            if fc < NFC:
                g = _dot(h, w1_v[:, fc * FC:(fc + 1) * FC])
                u = _dot(h, w3_v[:, fc * FC:(fc + 1) * FC])
                ev = _groups(g) + _groups(u)
                if 1 <= fc <= len(side):
                    u0 = _after(u[T - 8:T, FC - 128:FC], functools.reduce(_or, links[fc - 1]) & zvec)
                    u = jnp.concatenate([u[0:T - 8, :], jnp.concatenate([u[T - 8:T, 0:FC - 128], u0], axis=1)], axis=0)
                hg = 0.5 * g
                act = (hg * (1.0 + jnp.tanh(hg)) * u).astype(bf16)
            if fc >= 1:
                y = _dot(act_prev, w2_v[(fc - 1) * FC:fc * FC, 0:D])
                ev = ev + _groups(y)
                acc = (x1_v[...] if acc is None else acc) + scaled(y)
            if fc < len(side):
                n = len(side[fc])
                pos = [4 + (k * 12) // n if fc else 3 + (k * 5) // n for k in range(n)]
                links.append([fn(_bits(ev[p][T - 16:T - 8]) & zvec) for p, fn in zip(pos, side[fc])])
            act_prev = act
        rows = pl.ds(pl.multiple_of(i * T, T), T)
        for half in range(2):
            cols = slice(half * (D // 2), (half + 1) * (D // 2))
            ob_v[rows, cols] = acc[:, cols].astype(bf16)
            pltpu.make_async_copy(ob_v.at[rows, cols], out_hbm.at[0, rows, cols], osem.at[0]).start()

        @pl.when(i == SKEW * IPT - 1)
        def _():
            out_proj(pltpu.bitcast(o_v[...], bf16), NS * T)

    def main(i, carry):
        lax.cond(i < NA, phase_a, phase_b, i)
        return carry
    lax.fori_loop(0, NA + NT, main, 0)
    pltpu.make_async_copy(ob_v, out_hbm.at[0], osem.at[0]).wait()


@jax.jit
def pallas_adaLN_cond__sliding_local_dilated__glu_gated_swiglu__prompt_kernel(
    A_x, A_wqkv, A_wo, B_x, B_w1, B_w3, B_w2, c, w_mod):
    del B_x
    any_spec = pl.BlockSpec(memory_space=pl.ANY)
    return pl.pallas_call(
        _kernel,
        out_shape=jax.ShapeDtypeStruct((1, S, D), bf16),
        in_specs=[any_spec] * 8,
        out_specs=any_spec,
        scratch_shapes=[
            pltpu.VMEM((S, D), bf16),
            pltpu.VMEM((1, D), bf16),
            pltpu.VMEM((D, 128), f32),
            pltpu.VMEM((NKC, D, 2 * KC), bf16),
            pltpu.VMEM((D, LW), bf16),
            pltpu.VMEM((D, LW), bf16),
            pltpu.VMEM((D, 3 * D), bf16),
            pltpu.VMEM((NKC // 2, KC // 2, 3 * D + PADW), u32),
            pltpu.VMEM((NKC // 2, KC // 2, 3 * D + PADW), u32),
            pltpu.VMEM((D, D + PADW), bf16),
            pltpu.VMEM((D, F + PADW), bf16),
            pltpu.VMEM((D, F + PADW), bf16),
            pltpu.VMEM((F, D + PADW), bf16),
            pltpu.VMEM((2 * NG, 8, 128), f32),
            pltpu.VMEM((4 * NG, 8, 128), f32),
            pltpu.VMEM((NG, M0, 128), f32),
            pltpu.VMEM((M0, KC), bf16),
            pltpu.VMEM((M0, KC), bf16),
            pltpu.VMEM((T, D + PADW), bf16),
            pltpu.VMEM((T, D + PADW), bf16),
            pltpu.VMEM((T, D), f32),
            pltpu.VMEM((3 * NG, WROWS + 8, 128), f32),
            pltpu.VMEM((T // 2, D), u32),
            pltpu.VMEM((M0 // 2, D), u32),
            pltpu.VMEM((2, 3 * NG, KROWS, 128), f32),
            pltpu.VMEM((3, 3 * NG, KROWS, 128), f32),
            pltpu.VMEM((NG, S + 8, 128), f32),
            pltpu.VMEM((S, D), bf16),
            pltpu.VMEM((8, 128), u32),
            pltpu.SemaphoreType.DMA((12 + 2 * NKC,)),
            pltpu.SemaphoreType.DMA((1,)),
        ],
        compiler_params=pltpu.CompilerParams(vmem_limit_bytes=110 * 2**20, disable_bounds_checks=True,
                                             disable_semaphore_checks=True),
        name="adaln_fused",
    )(A_x, A_wqkv, A_wo, B_w1, B_w3, B_w2, c, w_mod)
```

```python
import functools

import jax
import jax.numpy as jnp
from jax import lax
import jax.experimental.pallas as pl
import jax.experimental.pallas.tpu as pltpu

S, D, F = 2048, 1024, 3584
DH, W, DIL = 32, 8, 2
NG = D // 128
HALO = 16
T = 128
NT = S // T
NP = T // 16
NRB = T // 8
SKEW = 3
M0 = SKEW * T
NS = NT - SKEW
NA = NS // 2
PPI = 2
IPT = NP // PPI
WROWS = HALO + 16 * PPI
FC = 512
NFC = F // FC
KOFF = HALO
KROWS = KOFF + T + 8
LOG2E = 1.4426950408889634
QSCALE = (DH ** -0.5) * LOG2E
NEG = -1e9 * DH ** 0.5
KC = 128
NKC = D // KC
WR = 5
LW = 512
NLP = 4 * D // LW
PADW = 128
EPS = 1e-5
GATES = {"first": (19.5, 0.1, 0.6, 5, 8), 1: (19.5, 0.6, 0.6, 4, 2), 0: (20.5, 0.7, 0.75, 4, 2)}
FPLAN = "aaa/a/llfl/llllwll/llw/wllllwl"
f32, bf16, u32 = jnp.float32, jnp.bfloat16, jnp.uint32


def _lane_tables():
    lane = lax.broadcasted_iota(jnp.int32, (8, 128), 1)
    head = lane & 31
    masks = [(lane & (4 << s)) != 0 for s in range(3)]
    fwd = [((head & 3) << 5) | (((head >> 2) ^ g) << 2) | (lane >> 5) for g in range(NG)]
    inv = [((lane & 3) << 5) | ((((lane >> 2) & 7) ^ g) << 2) | (lane >> 5) for g in range(NG)]
    return masks, fwd, inv


def _butterfly(vs, masks):
    n = vs[0].shape[0] // 8
    vs = [v.reshape(n, 8, 128) for v in vs]
    for s in range(3):
        for g in range(NG):
            if g & (1 << s):
                continue
            a, b = vs[g], vs[g | (1 << s)]
            vs[g] = jnp.where(masks[s], b, a)
            vs[g | (1 << s)] = jnp.where(masks[s], a, b)
    return [v.reshape(n * 8, 128) for v in vs]


def _gather_lanes(v, idx):
    idx = jnp.concatenate([idx] * (v.shape[0] // 8), axis=0)
    return jnp.take_along_axis(v, idx, axis=1, mode="promise_in_bounds")


def _to_head_lanes(vs, tabs):
    return [_gather_lanes(y, i) for y, i in zip(_butterfly(vs, tabs[0]), tabs[1])]


def _from_head_lanes(zs, tabs):
    return _butterfly([_gather_lanes(z, i) for z, i in zip(zs, tabs[2])], tabs[0])


def _add(a, b):
    return a + b


def _or(a, b):
    return a | b


def _bits(x):
    return pltpu.bitcast(x, u32)


def _dot(a, b):
    return jnp.dot(a, b, preferred_element_type=f32)


def _after(x, dep):
    if dep is None:
        return x
    return pltpu.bitcast(_bits(x) | dep, x.dtype)


def _norm8(xs, dep=None):
    xs = [_after(xs[0], dep)] + list(xs[1:])
    m = jnp.sum(functools.reduce(_add, xs), axis=-1, keepdims=True) * (1.0 / D)
    xc = [v - m for v in xs]
    var = jnp.sum(functools.reduce(_add, [v * v for v in xc]), axis=-1, keepdims=True) * (1.0 / D)
    r = lax.rsqrt(var + EPS)
    return [v * r for v in xc]


def _groups(x):
    return [x[:, g * 128:(g + 1) * 128] for g in range(x.shape[1] // 128)]


def _kernel(x_hbm, wqkv_hbm, wo_hbm, w1_hbm, w3_hbm, w2_hbm, c_hbm, wmod_hbm, out_hbm,
            x_v, c_v, cb_v, wm_v, wl0_v, wl1_v, wraw_v, wpe_v, wpo_v, wo_v, w1_v, w3_v, w2_v, mod_v, modr_v,
            xn_v, he_v, ho_v, h_v, h2_v, x1_v, win_v, st_v, o_v, p0_v, p1_v, a_v, ob_v,
            zv_v, sem, osem):
    names = ["c", "x0", "x1", "x2", "x3", "xr", "wo", "w1", "w3", "w2", "wl0", "wl1"]
    srcdst = dict(
        c=(c_hbm, c_v),
        x0=(x_hbm.at[0, 0:M0, :], x_v.at[0:M0, :]),
        x1=(x_hbm.at[0, M0:M0 + T, :], x_v.at[M0:M0 + T, :]),
        x2=(x_hbm.at[0, M0 + T:M0 + 2 * T, :], x_v.at[M0 + T:M0 + 2 * T, :]),
        x3=(x_hbm.at[0, M0 + 2 * T:M0 + 3 * T, :], x_v.at[M0 + 2 * T:M0 + 3 * T, :]),
        xr=(x_hbm.at[0, M0 + 3 * T:S, :], x_v.at[M0 + 3 * T:S, :]),
        wo=(wo_hbm, wo_v.at[:, 0:D]),
        w1=(w1_hbm, w1_v.at[:, 0:F]), w3=(w3_hbm, w3_v.at[:, 0:F]), w2=(w2_hbm, w2_v.at[:, 0:D]),
    )
    copies = {n: pltpu.make_async_copy(*srcdst[n], sem.at[names.index(n)]) for n in srcdst}
    SEM_C = len(names)
    SEM_W = SEM_C + NKC

    def slab_copy(c, sec):
        cols = pl.ds(pl.multiple_of(sec * D + c * KC, KC), KC)
        return pltpu.make_async_copy(wmod_hbm.at[:, cols], wm_v.at[c, :, sec * KC:(sec + 1) * KC], sem.at[SEM_C + c])

    def chunk_copies(c):
        rows = pl.ds(pl.multiple_of(c * KC, KC), KC)
        return [slab_copy(c, 0), slab_copy(c, 1),
                pltpu.make_async_copy(wqkv_hbm.at[rows, :], wraw_v.at[rows, :], sem.at[SEM_W + c])]

    def late_copy(p, par):
        cols = pl.ds(pl.multiple_of(2 * D + p * LW, LW), LW)
        return pltpu.make_async_copy(wmod_hbm.at[:, cols], (wl0_v, wl1_v)[par], sem.at[names.index("wl0") + par])

    copies["c"].start()
    copies["x0"].start()
    for c in range(NKC):
        for cp in chunk_copies(c):
            cp.start()
    for n in ("x1", "x2", "wo", "x3"):
        copies[n].start()
    late_copy(0, 1).start()
    late_copy(1, 0).start()
    copies["xr"].start()
    zv_v[...] = jnp.zeros(zv_v.shape, u32)

    tabs = _lane_tables()
    proj = (p0_v, p1_v)
    mcol = lambda sec, g: mod_v[sec * NG + g] if sec < 2 else modr_v[(sec - 2) * NG + g]
    row8 = lax.broadcasted_iota(jnp.int32, (8, 128), 0)

    def ln1_rows(xt, drow, dep):
        xn = _norm8(_groups(xt[drow:drow + 8, :].astype(f32)), dep)
        ys = [xn[g] * mcol(1, g) + mcol(0, g) for g in range(NG)]
        h_v[drow:drow + 8, 0:D] = jnp.concatenate(ys, axis=1).astype(bf16)
        return _bits(ys[NG - 1])

    def ln2_rows(t, drow, dep):
        xt, at = x_v.at[pl.ds(t, T), :], a_v.at[:, pl.ds(t, T), :]
        x = _groups(xt[drow:drow + 8, :].astype(f32))
        x1 = [x[g] + mcol(2, g) * at[g, drow:drow + 8, :] for g in range(NG)]
        x1_v[drow:drow + 8, :] = jnp.concatenate(x1, axis=1)
        xn = _norm8(x1, dep)
        ys = [xn[g] * mcol(4, g) + mcol(3, g) for g in range(NG)]
        h2_v[drow:drow + 8, 0:D] = jnp.concatenate(ys, axis=1).astype(bf16)
        return _bits(ys[NG - 1])

    def attn8(src, masked, pb, par, dep):
        r0 = KOFF + 16 * pb + par
        rows = lambda j: pl.ds(r0 - DIL * j, 8, stride=DIL)
        zvec = zv_v[...]
        s = [None] * W
        for g in range(NG):
            q = src[g, rows(0), :]
            if g == 0:
                q = _after(q, dep)
            else:
                q = _after(q, _bits(s[W - 1]) & zvec)
            for j in range(W):
                p = q * src[NG + g, rows(j), :]
                s[j] = p if s[j] is None else s[j] + p
        for j in range(W):
            s[j] = s[j] + pltpu.roll(s[j], 64, 1)
            s[j] = s[j] + pltpu.roll(s[j], 32, 1)
            if masked and pb == 0 and j > 0:
                s[j] = jnp.where(par + DIL * row8 >= DIL * j, s[j], NEG)
        m = functools.reduce(jnp.maximum, s)
        e = [jnp.exp2((s[j] - m) * QSCALE) for j in range(W)]
        den = functools.reduce(_add, e)
        r = pl.reciprocal(den, approx=True)
        inv = r * (2.0 - den * r)
        og = [None] * NG
        for j in range(W):
            p = e[j] * inv
            if j:
                p = _after(p, _bits(og[NG - 1]) & zvec)
            for g in range(NG):
                t = p * src[2 * NG + g, rows(j), :]
                og[g] = t if og[g] is None else og[g] + t
        return og

    def stage(pb, even, odd):
        for g in range(NG):
            st_v[8 * pb:8 * pb + 8, g * 128:(g + 1) * 128] = _bits(
                jnp.concatenate([even[g], odd[g]], axis=0).astype(bf16))

    def unstage(r0, r1):
        return jnp.concatenate(_from_head_lanes(_groups(st_v[r0:r1, :]), tabs), axis=1)

    def out_proj(o, t0, side=None):
        a = _groups(_dot(o, wo_v[:, 0:D]))
        links = side(a) if side is not None else {}
        at = a_v.at[:, pl.ds(t0, o.shape[0] + 8), :]
        for g in range(NG):
            for rb in range(a[g].shape[0] // 8):
                v = a[g][rb * 8:(rb + 1) * 8]
                if rb == 0 and g in links:
                    v = _after(v, links[g])
                at[g, pl.ds((rb // 2) * 16 + rb % 2, 8, stride=2), :] = v

    def mod_vpu(wl, k, part, nparts, dep):
        n = D // nparts
        zvec = zv_v[...]
        acc = None
        for i in range(n // 8):
            rows = slice(part * n + i * 8, part * n + (i + 1) * 8)
            cb = cb_v[rows, :]
            if i % 4 == 0:
                cb = _after(cb, dep if i == 0 else _bits(acc[:, 0:128]) & zvec)
            t = wl[rows, k * 256:(k + 1) * 256].astype(f32) * jnp.concatenate([cb, cb], axis=1)
            acc = t if acc is None else acc + t
        return acc

    def chunk_block(c, par, do_prep, do_mm, extra=None):
        zvec = zv_v[...]
        links = {}

        def link(ct, v):
            links[ct] = (links[ct] | v) if ct in links else v

        def rounds(hc, wp, rs):
            res = {}
            for r in rs:
                out = _groups(_dot(hc, pltpu.bitcast(wp[:, r * 512:(r + 1) * 512], bf16)))
                for n in range(4):
                    res[4 * r + n] = out[n]
            return res

        def accumulate(res):
            for ct in res:
                for t in range(SKEW):
                    blk = res[ct][t * T:(t + 1) * T]
                    if t == SKEW - 1 and ct in links:
                        blk = jnp.concatenate([blk[0:T - 8], _after(blk[T - 8:T], links.pop(ct) & zvec)], axis=0)
                    proj[t % 2][t // 2, ct, KOFF:KOFF + T, :] += blk
        if do_prep:
            for cp in chunk_copies(c):
                cp.wait()
        if do_mm:
            res = rounds((he_v, ho_v)[1 - par][...], (wpe_v, wpo_v)[1 - par].at[(c - 1) >> 1], range(WR, 6))
        if do_prep:
            part = [mod_vpu(wm_v.at[c], 0, h, 4, None) for h in range(4)]
            m = jnp.broadcast_to(jnp.sum(functools.reduce(_add, part), axis=0, keepdims=True), (8, 256))
            sh = m[:, 0:128]
            s1 = m[:, 128:256] + 1.0
            mod_v[c] = sh
            mod_v[NG + c] = s1
            hc = (xn_v[c].reshape(M0 // 8, 8, 128) * s1 + sh).reshape(M0, 128).astype(bf16)
            (he_v, ho_v)[par][...] = hc
            wp = (wpe_v, wpo_v)[par].at[c >> 1]
            for b in range(6):
                sec, half = b // 2, b % 2
                r0 = pl.multiple_of(c * KC + half * 64, 64)
                vs = _groups(_bits(wraw_v[pl.ds(r0, 64), sec * D:(sec + 1) * D]))
                vs = _to_head_lanes(vs, tabs)
                wp[half * 32:(half + 1) * 32, sec * D:(sec + 1) * D] = jnp.concatenate(vs, axis=1)
        if extra is not None:
            extra(res, link, zvec)
        if do_mm:
            accumulate(res)
        if do_prep:
            accumulate(rounds(hc, wp, range(WR)))

    def prologue():
        def zero(ct, carry):
            for t in range(SKEW):
                proj[t % 2][t // 2, ct, KOFF:KOFF + T, :] = jnp.zeros((T, 128), f32)
            return carry
        lax.fori_loop(0, 3 * NG, zero, 0)
        copies["c"].wait()
        c32 = c_v[...].astype(f32)
        sc = (c32 * jax.nn.sigmoid(c32)).astype(bf16)
        diag = lax.broadcasted_iota(jnp.int32, (128, 128), 0) == lax.broadcasted_iota(jnp.int32, (128, 128), 1)
        for g, row in enumerate(_groups(sc.astype(f32))):
            col = jnp.sum(jnp.where(diag, row, 0.0), axis=1, keepdims=True)
            cb_v[g * 128:(g + 1) * 128, :] = jnp.broadcast_to(col, (128, 128))
        copies["x0"].wait()

        def stats(i, carry):
            for rb in range(12):
                rows = pl.ds(pl.multiple_of(i * 96, 32) + rb * 8, 8)
                xn = _norm8(_groups(x_v[rows, :].astype(f32)))
                for g in range(NG):
                    xn_v[g, rows, :] = xn[g]
            return carry
        lax.fori_loop(0, M0 // 96, stats, 0)
        chunk_block(0, 0, True, False)

        def kloop(i, carry):
            chunk_block(2 * i + 1, 1, True, True)

            @pl.when(2 * i + 2 < NKC)
            def _():
                chunk_block(2 * i + 2, 0, True, True)
            return carry
        lax.fori_loop(0, NKC // 2, kloop, 0)

        copies["x1"].wait()
        for n in ("w1", "w3", "w2"):
            copies[n].start(priority=1)

        def ln_next(res, link, zvec):
            for rb in range(T // 8):
                link(20 + rb % 4, ln1_rows(x_v.at[M0:M0 + T, :], rb * 8, _bits(res[4 * WR][0:8]) & zvec))
        chunk_block(NKC, 0, False, True, ln_next)
        for t in range(SKEW):
            for sg in range(NG, 3 * NG):
                if t == 0:
                    halo = jnp.broadcast_to(p0_v[0, sg, KOFF:KOFF + 1, :], (HALO, 128))
                else:
                    halo = proj[(t - 1) % 2][(t - 1) // 2, sg, KOFF + T - HALO:KOFF + T, :]
                proj[t % 2][t // 2, sg, KOFF - HALO:KOFF, :] = halo
        copies["x2"].wait()

    def step(s, par, first=False, last=False):
        GS, GA, GL, LL, UG = GATES["first" if first else par]
        zvec = zv_v[...]
        t0 = s * T if first or last else pl.multiple_of(s * T, T)
        slot = (s >> 1) & 1
        dst = proj[1 - par].at[((s + SKEW) >> 1) & 1]
        prev = proj[par].at[1 - slot]
        w = jnp.concatenate([(wpe_v, wpo_v)[c % 2][c // 2, :, 0:3 * D] for c in range(NKC)], axis=0)
        tiles = _groups(_dot(h_v[:, 0:D], pltpu.bitcast(w, bf16)))
        for ct in range(3 * NG):
            dst[ct, KOFF:KOFF + T, :] = tiles[ct]
            if ct >= NG:
                dst[ct, KOFF - HALO:KOFF, :] = prev[ct, KOFF + T - HALO:KOFF + T, :]
        t1 = t0 + (SKEW + 1) * T
        src = proj[par].at[slot]
        links, rows = [], []

        def gate(pos):
            ct = int(pos)
            rb = min(T // 8 - 1, int((pos - ct) * (T // 8)))
            return _bits(tiles[ct][rb * 8:(rb + 1) * 8, :]) & zvec

        for pb in range(NP):
            halves = []
            for k in (2 * pb, 2 * pb + 1):
                d = gate(GA + GS * k / NRB)
                if k >= LL:
                    d = d | (links[k - LL] & zvec)
                halves.append(attn8(src, first, pb, k % 2, d))
            stage(pb, *halves)
            for rb in (2 * pb, 2 * pb + 1):
                d = gate(GA + GL + GS * rb / NRB)
                links.append(ln2_rows(0, rb * 8, d) if last else ln1_rows(x_v.at[pl.ds(t1, T), :], rb * 8, d))
            if (pb + 1) % UG == 0:
                rows.append(pltpu.bitcast(unstage((pb + 1 - UG) * 8, (pb + 1) * 8), bf16))

        def mods(a):
            links = {}
            ev = tiles[3 * NG - 2:] + a
            piece = jnp.minimum(s - 1, NLP - 1 - par)
            for k in range(LW // 256):
                part = [mod_vpu((wl0_v, wl1_v)[par], k, h, 2, _bits(ev[(7 * (2 * k + h)) // 4][T - 8:T]) & zvec)
                        for h in range(2)]
                m = jnp.sum(part[0] + part[1], axis=0, keepdims=True)
                m = jnp.broadcast_to(m + jnp.where(piece >> 1 == 2, 1.0, 0.0), (8, 256))
                modr_v[4 * piece + 2 * k] = m[:, 0:128]
                modr_v[4 * piece + 2 * k + 1] = m[:, 128:256]
                links[5 + 2 * k] = _bits(m[:, 0:128]) & zvec
            return links

        def handover(a):
            links = {}
            ev = tiles[3 * NG - 2:] + a
            for k in range(4):
                links[k + 3] = fill_window(0, range(6 * k, 6 * k + 6), _bits(ev[k + 2][T - 8:T]) & zvec) & zvec
            for k in range(6):
                seen = []
                for sg in range(4 * k, 4 * k + 4):
                    lo = KOFF if sg < NG else KOFF - HALO
                    for r in range(lo, KOFF + T, 8):
                        v = p0_v[1, sg, r:r + 8, :]
                        if not seen:
                            v = _after(v, _bits(ev[k + 1][T - 8:T]) & zvec)
                        p1_v[2, sg, r:r + 8, :] = v
                        seen.append(_bits(v))
                lk = functools.reduce(_or, seen) & zvec
                links[k + 2] = (links[k + 2] | lk) if k + 2 in links else lk
            return links
        if first:
            copies["wo"].wait()
            out_proj(jnp.concatenate(rows, axis=0), t0)
        elif last:
            out_proj(jnp.concatenate(rows, axis=0), t0, handover)
        else:
            out_proj(jnp.concatenate(rows, axis=0), t0, mods)

            @pl.when(s + 1 < NLP)
            def _():
                late_copy(s + 1, par).start()

    def phase_a(i, carry):
        @pl.when(i == 0)
        def _():
            prologue()
            step(0, 0, first=True)

        @pl.when(i == 0)
        def _():
            copies["x3"].wait()

        @pl.when(2 * i < NLP)
        def _():
            late_copy(2 * i, 1).wait()
        step(2 * i + 1, 1)

        @pl.when(i < NA - 1)
        def _():
            @pl.when(i == 0)
            def _():
                copies["xr"].wait()

            @pl.when(2 * i + 1 < NLP)
            def _():
                late_copy(2 * i + 1, 0).wait()
            step(2 * i + 2, 0)

        @pl.when(i == NA - 1)
        def _():
            for n in ("w1", "w3", "w2"):
                copies[n].wait()
            step(NS - 1, 0, last=True)
            lax.fori_loop(0, NT, phase_b, 0)
        return carry

    def fill_window(i, sgs, dep):
        row = (i % IPT) * 16 * PPI
        src = p1_v.at[(i // IPT) % 3, :, pl.ds(row if isinstance(i, int) else pl.multiple_of(row, 16 * PPI), WROWS), :]
        seen = []
        for sg in sgs:
            lo = KOFF if sg < NG else KOFF - HALO
            v = src[sg, lo:WROWS, :]
            if not seen:
                v = jnp.concatenate([_after(v[0:8], dep), v[8:]], axis=0)
            win_v[sg, lo:WROWS, :] = v
            seen += [_bits(v[r:r + 8]) for r in range(0, WROWS - lo, 8)]
        return functools.reduce(_or, seen)

    def phase_b(i, carry):
        t1 = pl.multiple_of(jnp.minimum(i + 1, NT - 1) * T, T)
        zvec = zv_v[...]
        sl = (i // IPT) % 3
        orow = jnp.where(sl == 0, 0, jnp.where(sl == 1, T, T // 2)) + (i % IPT) * 8 * PPI

        def fin(dep):
            o = unstage(0, 8 * PPI)
            o_v[pl.ds(pl.multiple_of(orow, 8 * PPI), 8 * PPI), :] = o
            return o[8 * PPI - 8:8 * PPI, D - 128:D]
        halves = []

        def att(n):
            def run(d):
                halves.append(attn8(win_v, False, n // 2, n % 2, d))
                if n % 2:
                    stage(n // 2, *halves[-2:])
                return _bits(halves[-1][NG - 1])
            return run
        ln = lambda r: (lambda d: ln2_rows(t1, r * 8, d))
        fw = lambda k: (lambda d: fill_window(i + 1, range(6 * k, 6 * k + 6), d))
        code = {"a": att, "f": lambda n: fin, "l": ln, "w": fw}
        cnt = dict.fromkeys(code, 0)
        side = []
        for chunk in FPLAN.split("/"):
            side.append([])
            for c in chunk:
                side[-1].append(code[c](cnt[c]))
                cnt[c] += 1
        assert cnt == {"a": 2 * PPI, "f": 1, "l": NRB, "w": 4}, cnt
        h = h2_v[:, 0:D]
        gb = jnp.concatenate([mcol(5, g) for g in range(NG)], axis=1)
        scaled = lambda y: (y.reshape(NRB, 8, D) * gb).reshape(T, D)
        acc = act_prev = None
        links = []
        for fc in range(NFC + 1):
            ev = []
            if fc < NFC:
                g = _dot(h, w1_v[:, fc * FC:(fc + 1) * FC])
                u = _dot(h, w3_v[:, fc * FC:(fc + 1) * FC])
                ev = _groups(g) + _groups(u)
                if 1 <= fc <= len(side):
                    u0 = _after(u[T - 8:T, FC - 128:FC], functools.reduce(_or, links[fc - 1]) & zvec)
                    u = jnp.concatenate([u[0:T - 8, :], jnp.concatenate([u[T - 8:T, 0:FC - 128], u0], axis=1)], axis=0)
                hg = 0.5 * g
                act = (hg * (1.0 + jnp.tanh(hg)) * u).astype(bf16)
            if fc >= 1:
                y = _dot(act_prev, w2_v[(fc - 1) * FC:fc * FC, 0:D])
                ev = ev + _groups(y)
                acc = (x1_v[...] if acc is None else acc) + scaled(y)
            if fc < len(side):
                n = len(side[fc])
                pos = [4 + (k * 11) // n if fc else 3 + (k * 5) // n for k in range(n)]
                links.append([fn(_bits(ev[p][T - 16:T - 8]) & zvec) for p, fn in zip(pos, side[fc])])
            act_prev = act
        rows = pl.ds(pl.multiple_of(i * T, T), T)
        for half in range(2):
            cols = slice(half * (D // 2), (half + 1) * (D // 2))
            ob_v[rows, cols] = acc[:, cols].astype(bf16)
            pltpu.make_async_copy(ob_v.at[rows, cols], out_hbm.at[0, rows, cols], osem.at[0]).start()

        @pl.when(i == SKEW * IPT - 1)
        def _():
            out_proj(pltpu.bitcast(o_v[...], bf16), NS * T)
        return carry

    lax.fori_loop(0, NA, phase_a, 0)
    pltpu.make_async_copy(ob_v, out_hbm.at[0], osem.at[0]).wait()


@jax.jit
def pallas_adaLN_cond__sliding_local_dilated__glu_gated_swiglu__prompt_kernel(
    A_x, A_wqkv, A_wo, B_x, B_w1, B_w3, B_w2, c, w_mod):
    del B_x
    any_spec = pl.BlockSpec(memory_space=pl.ANY)
    return pl.pallas_call(
        _kernel,
        out_shape=jax.ShapeDtypeStruct((1, S, D), bf16),
        in_specs=[any_spec] * 8,
        out_specs=any_spec,
        scratch_shapes=[
            pltpu.VMEM((S, D), bf16),
            pltpu.VMEM((1, D), bf16),
            pltpu.VMEM((D, 128), f32),
            pltpu.VMEM((NKC, D, 2 * KC), bf16),
            pltpu.VMEM((D, LW), bf16),
            pltpu.VMEM((D, LW), bf16),
            pltpu.VMEM((D, 3 * D), bf16),
            pltpu.VMEM((NKC // 2, KC // 2, 3 * D + PADW), u32),
            pltpu.VMEM((NKC // 2, KC // 2, 3 * D + PADW), u32),
            pltpu.VMEM((D, D + PADW), bf16),
            pltpu.VMEM((D, F + PADW), bf16),
            pltpu.VMEM((D, F + PADW), bf16),
            pltpu.VMEM((F, D + PADW), bf16),
            pltpu.VMEM((2 * NG, 8, 128), f32),
            pltpu.VMEM((4 * NG, 8, 128), f32),
            pltpu.VMEM((NG, M0, 128), f32),
            pltpu.VMEM((M0, KC), bf16),
            pltpu.VMEM((M0, KC), bf16),
            pltpu.VMEM((T, D + PADW), bf16),
            pltpu.VMEM((T, D + PADW), bf16),
            pltpu.VMEM((T, D), f32),
            pltpu.VMEM((3 * NG, WROWS + 8, 128), f32),
            pltpu.VMEM((T // 2, D), u32),
            pltpu.VMEM((M0 // 2, D), u32),
            pltpu.VMEM((2, 3 * NG, KROWS, 128), f32),
            pltpu.VMEM((3, 3 * NG, KROWS, 128), f32),
            pltpu.VMEM((NG, S + 8, 128), f32),
            pltpu.VMEM((S, D), bf16),
            pltpu.VMEM((8, 128), u32),
            pltpu.SemaphoreType.DMA((12 + 2 * NKC,)),
            pltpu.SemaphoreType.DMA((1,)),
        ],
        compiler_params=pltpu.CompilerParams(vmem_limit_bytes=110 * 2**20, disable_bounds_checks=True,
                                             disable_semaphore_checks=True),
        name="adaln_fused",
    )(A_x, A_wqkv, A_wo, B_w1, B_w3, B_w2, c, w_mod)
```
